```python
import jax
import jax.numpy as jnp

def _softmax(x, axis=-1):
    return jax.nn.softmax(x, axis=axis)
def _gelu(x):
    return jax.nn.gelu(x, approximate=True)
def _silu(x):
    return jax.nn.silu(x)
def _sigmoid(x):
    return jax.nn.sigmoid(x)
def _layernorm(x, axis=-1, eps=1e-5):
    m = jnp.mean(x, axis=axis, keepdims=True)
    v = jnp.var(x, axis=axis, keepdims=True)
    return (x - m) / jnp.sqrt(v + eps)
def _scatter_add(tgt, idx, src, axis=0):
    return tgt.at[idx].add(src)
def _segment_sum(src, seg, n):
    return jax.ops.segment_sum(src, seg, n)
class _Rng:
    def __init__(self, key):
        self._k = key
    def _next(self):
        self._k, sub = jax.random.split(self._k)
        return sub
    def normal(self, shape):
        return jax.random.normal(self._next(), shape, dtype=jnp.bfloat16)
    def randint(self, lo, hi, shape):
        return jax.random.randint(self._next(), shape, lo, hi, dtype=jnp.int32)
    def uniform(self, shape, lo=0.0, hi=1.0):
        return jax.random.uniform(self._next(), shape, jnp.bfloat16, lo, hi)
    def permutation(self, n):
        return jax.random.permutation(self._next(), n)


kernel_name = 'gated_mix__linear_kernel_hedgehog__moe_arch_mod__prompt'

def setup_inputs():
    _rng = _Rng(jax.random.key(int.from_bytes(__import__("os").urandom(4), "little")))
    _w = (lambda a: (lambda t: t.astype(jnp.bfloat16) if jnp.issubdtype(t.dtype, jnp.floating) else t)(jnp.asarray(a)))
    def _A_setup():
        B, S, D, H = 1, 2048, 1024, 32
        Dh = D // H
        return {
            "x": _w((lambda *s: _rng.normal(s) * 0.05)(B, S, D)),
            "wqkv": _w((lambda *s: _rng.normal(s) * 0.05)(D, 3 * D)),
            "w_phi": _w((lambda *s: _rng.normal(s) * 0.05)(H, Dh, Dh) * (Dh ** -0.5)),
            "wo": _w((lambda *s: _rng.normal(s) * 0.05)(D, D)),
        }
    _A_in = _A_setup()

    def _B_setup():
        B, S, D, F, C = 1, 2048, 1024, 3584, 1
        return {
            "x": _w((lambda *s: _rng.normal(s) * 0.05)(B, S, D)),
            "w_r": _w((lambda *s: _rng.normal(s) * 0.05)(D)),
            "w_gate": _w((lambda *s: _rng.normal(s) * 0.05)(D, F)),
            "w_up": _w((lambda *s: _rng.normal(s) * 0.05)(D, F)),
            "w_down": _w((lambda *s: _rng.normal(s) * 0.05)(F, D)),
        }
    _B_in = _B_setup()

    return {
        "A_x": _A_in["x"],
        "A_wqkv": _A_in["wqkv"],
        "A_w_phi": _A_in["w_phi"],
        "A_wo": _A_in["wo"],
        "B_x": _B_in["x"],
        "B_w_r": _B_in["w_r"],
        "B_w_gate": _B_in["w_gate"],
        "B_w_up": _B_in["w_up"],
        "B_w_down": _B_in["w_down"],
        "gate_w": _w((lambda *s: _rng.normal(s) * 0.05)(1024)),
    }

def reference(A_x, A_wqkv, A_w_phi, A_wo, B_x, B_w_r, B_w_gate, B_w_up, B_w_down, gate_w):
    def _A_ref(x, wqkv, w_phi, wo):
        B, S, D = x.shape
        H = 32; Dh = D // H
        qkv = (lambda x, *d: x.transpose(*d))((x @ wqkv).reshape(B, S, 3, H, Dh), 2, 0, 3, 1, 4)
        q, k, v = qkv[0], qkv[1], qkv[2]
        pq = jnp.einsum("bhsd,hdf->bhsf", q, w_phi)
        pk = jnp.einsum("bhsd,hdf->bhsf", k, w_phi)
        phi_q = jnp.concatenate([_softmax(pq, axis=-1), _softmax(-pq, axis=-1)], axis=-1)
        phi_k = jnp.concatenate([_softmax(pk, axis=-1), _softmax(-pk, axis=-1)], axis=-1)
        kv = jnp.einsum("bhsf,bhsd->bhfd", phi_k, v)
        z  = jnp.einsum("bhsf->bhf", phi_k)
        num = jnp.einsum("bhqf,bhfd->bhqd", phi_q, kv)
        den = jnp.einsum("bhqf,bhf->bhq", phi_q, z)[..., None] + 1e-6
        o = num / den
        return (lambda x, *d: x.transpose(*d))(o, 0, 2, 1, 3).reshape(B, S, D) @ wo

    def _B_ref(x, w_r, w_gate, w_up, w_down):
        B, S, D = x.shape
        C = 1
        r = x @ w_r
        idx = jnp.argsort(-r, axis=-1)[:, :C]
        idx_e = jnp.repeat(idx.reshape(B, C, 1), D, axis=2)
        x_sel = jnp.take_along_axis(x, idx_e, axis=1)
        g = _silu(x_sel @ w_gate)
        u = x_sel @ w_up
        y = (g * u) @ w_down
        r_sel = _sigmoid(jnp.take_along_axis(r, idx, axis=1))
        y = y * r_sel.reshape(B, C, 1)
        b_off = (jnp.arange(B) * S).reshape(B, 1)
        flat_idx = (idx + b_off).reshape(B * C)
        zero = (x * 0.0).reshape(B * S, D)
        upd = _scatter_add(zero, flat_idx, y.reshape(B * C, D), axis=0)
        return x + upd.reshape(B, S, D)

    x = A_x
    g = _sigmoid((x * gate_w).sum(-1, keepdims=True))
    a = _A_ref(x, A_wqkv, A_w_phi, A_wo)
    b = _B_ref(x, B_w_r, B_w_gate, B_w_up, B_w_down)
    return g * a + (1 - g) * b
```

```python
import jax
import jax.numpy as jnp
from jax import lax
import jax.experimental.pallas as pl
import jax.experimental.pallas.tpu as pltpu

TS = 512
LOG2E = 1.4426950408889634

_NT = (((1,), (1,)), ((), ()))
_NN = (((1,), (0,)), ((), ()))
_TN = (((0,), (0,)), ((), ()))

f32 = jnp.float32
bf16 = jnp.bfloat16


def _dot(a, b, dims):
    return lax.dot_general(a, b, dims, preferred_element_type=f32)


def _tree(op, xs):
    xs = list(xs)
    while len(xs) > 1:
        nxt = [op(xs[i], xs[i + 1]) for i in range(0, len(xs) - 1, 2)]
        if len(xs) % 2:
            nxt.append(xs[-1])
        xs = nxt
    return xs[0]


def _head_reduce(op, tiles):
    r = _tree(op, tiles)
    r = op(r, pltpu.roll(r, 4, 0))
    return op(r, pltpu.roll(r, 2, 0))


def _phi_pair(p):
    tiles = [p[8 * j:8 * j + 8] for j in range(8)]
    hi = _head_reduce(jnp.maximum, tiles)
    lo = _head_reduce(jnp.minimum, tiles)
    ep = [jnp.exp2(t - hi) for t in tiles]
    en = [jnp.exp2(lo - t) for t in tiles]
    rp = 1.0 / _head_reduce(jnp.add, ep)
    rn = 1.0 / _head_reduce(jnp.add, en)
    return jnp.concatenate([e * rp for e in ep] + [e * rn for e in en], axis=0).astype(bf16)


def _lane_bcast_rows(row):
    return jnp.broadcast_to(row, (128, row.shape[1])).T


def _kernel(x_hbm, wqkv_hbm, wphi_ref, wo_hbm, wr_ref, wg_hbm, wu_hbm, wd_hbm, gw_ref,
            out_hbm,
            x_v, wqkv_v, wo_v, wg_v, wu_v, wd_v, wkv_t, wq_t, kv_acc, kv_t, rg_v, a_v,
            out_v, xcol_v, y_v, sem_x, sem_w, sem_f, sem_o):
    S, D = x_v.shape
    F = wd_v.shape[0]
    n_chunks = S // TS
    n_pairs = D // 64
    FS = F // n_chunks

    def x_copy(c):
        return pltpu.make_async_copy(x_hbm.at[pl.ds(c * TS, TS)], x_v.at[pl.ds(c * TS, TS)],
                                     sem_x.at[c])

    def w_copy(j):
        return pltpu.make_async_copy(wqkv_hbm.at[:, pl.ds(j * D, D)], wqkv_v.at[j], sem_w.at[j])

    wo_copy = pltpu.make_async_copy(wo_hbm, wo_v, sem_w.at[3])

    def f_copies(i):
        return (pltpu.make_async_copy(wg_hbm.at[:, pl.ds(i * FS, FS)], wg_v.at[i], sem_f.at[0, i]),
                pltpu.make_async_copy(wu_hbm.at[:, pl.ds(i * FS, FS)], wu_v.at[i], sem_f.at[1, i]),
                pltpu.make_async_copy(wd_hbm.at[pl.ds(i * FS, FS)], wd_v.at[pl.ds(i * FS, FS)],
                                      sem_f.at[2, i]))

    w_copy(1).start()
    w_copy(2).start()
    x_copy(0).start()

    c_i = lax.broadcasted_iota(jnp.int32, (128, 32), 0)
    f_i = lax.broadcasted_iota(jnp.int32, (128, 32), 1)
    sel = jnp.where((c_i % 64) // 2 == f_i, 1.0, 0.0).astype(bf16)
    r_i = lax.broadcasted_iota(jnp.int32, (128, 128), 0)
    l_i = lax.broadcasted_iota(jnp.int32, (128, 128), 1)
    same_head = (2 * (r_i // 64) + r_i % 2) == (l_i // 32)

    def fold(j, dst):
        for g in range(D // 128):
            phi_t = _dot(sel, wphi_ref[g * 128:(g + 1) * 128, :], _NT)
            phi_t = jnp.where(same_head, phi_t, 0.0).astype(bf16)
            w = _dot(phi_t, wqkv_v[j, :, g * 128:(g + 1) * 128], _NT)
            dst[g * 128:(g + 1) * 128, :] = (w * LOG2E).astype(bf16)

    w_copy(1).wait()
    for c in range(1, n_chunks):
        x_copy(c).start()
    w_copy(0).start()
    fold(1, wkv_t)
    w_copy(2).wait()
    wo_copy.start()
    wkv_t[D:2 * D, :] = wqkv_v[2].T
    row16 = lax.broadcasted_iota(jnp.int32, (16, D), 0)
    extra = jnp.where(row16 == 0, wr_ref[...].astype(f32),
                      jnp.where(row16 == 1, gw_ref[...].astype(f32), 0.0))
    wkv_t[2 * D:2 * D + 16, :] = extra.astype(bf16)
    kv_acc[...] = jnp.zeros(kv_acc.shape, f32)
    w_copy(0).wait()
    for i in range(n_chunks):
        for cp in f_copies(i):
            cp.start()
    fold(0, wq_t)

    ones = jnp.ones((16, TS), bf16)

    def phase1(c, _):
        x_copy(c).wait()
        s0 = pl.multiple_of(c * TS, TS)
        xc = x_v[pl.ds(s0, TS), :]
        res = _dot(wkv_t[...], xc, _NT)
        rg_v[c] = res[2 * D:2 * D + 8]
        for p in range(n_pairs):
            phi = _phi_pair(res[64 * p:64 * p + 64])
            vt = res[D + 64 * p:D + 64 * p + 64].astype(bf16)
            kv_acc[p] += _dot(jnp.concatenate([vt, ones], axis=0), phi, _NT)
        return 0

    lax.fori_loop(0, n_chunks, phase1, 0)

    kr = lax.broadcasted_iota(jnp.int32, (80, 128), 0)
    kl = lax.broadcasted_iota(jnp.int32, (80, 128), 1)
    keep = jnp.where(kr < 64, kr // 32, (kr - 64) // 8) == kl % 2
    for p in range(n_pairs):
        kv_t[p] = jnp.where(keep, kv_acc[p], 0.0).astype(bf16)

    r = jnp.concatenate([rg_v[c, 0:1, :] for c in range(n_chunks)], axis=1)
    r = r.astype(bf16).astype(f32)
    r_max = jnp.max(r, axis=1, keepdims=True)
    lane = lax.broadcasted_iota(jnp.int32, (1, S), 1)
    idx = jnp.min(jnp.where(r == r_max, lane, S - 1))
    r_gate = jax.nn.sigmoid(r_max)
    idx16 = pl.multiple_of((idx // 16) * 16, 16)
    is_sel = row16 == (idx - idx16)
    x_rows = x_v[pl.ds(idx16, 16), :].astype(f32)
    x_sel = jnp.sum(jnp.where(is_sel, x_rows, 0.0), axis=0, keepdims=True)
    xcol_v[...] = _lane_bcast_rows(x_sel)
    y_v[...] = jnp.zeros(y_v.shape, f32)
    last = idx // TS
    wo_copy.wait()

    def out_copy(c, slot):
        return pltpu.make_async_copy(out_v.at[slot], out_hbm.at[pl.ds(c * TS, TS)], sem_o.at[slot])

    def chunk_of(i):
        c = last + 1 + i
        return jnp.where(c >= n_chunks, c - n_chunks, c)

    def phase2(i, _):
        c = chunk_of(i)
        slot = i % 2
        s0 = pl.multiple_of(c * TS, TS)

        @pl.when(i >= 2)
        def _():
            out_copy(chunk_of(i - 2), slot).wait()

        for cp in f_copies(i):
            cp.wait()

        xc = x_v[pl.ds(s0, TS), :]
        pq = _dot(wq_t[...], xc, _NT)
        o_t = []
        for p in range(n_pairs):
            phi = _phi_pair(pq[64 * p:64 * p + 64])
            nd = _dot(kv_t[p], phi, _NN)
            for h in range(2):
                inv = 1.0 / (nd[64 + 8 * h:72 + 8 * h] + 1e-6)
                o_t += [nd[32 * h + 8 * j:32 * h + 8 * j + 8] * inv for j in range(4)]
        o_t = jnp.concatenate(o_t, axis=0).astype(bf16)
        a = _dot(o_t, wo_v[...], _TN)
        a_v[...] = a
        g = _lane_bcast_rows(jax.nn.sigmoid(rg_v[c, 1:2, :]))
        for j in range(D // 128):
            cols = slice(j * 128, (j + 1) * 128)
            xb = xc[:, cols].astype(f32)
            out_v[slot, :, cols] = (g * a[:, cols] + (1.0 - g) * xb).astype(bf16)

        acc_g = jnp.zeros((8, FS), f32)
        acc_u = jnp.zeros((8, FS), f32)
        for k in range(D // 16):
            xk = xcol_v[16 * k:16 * k + 16, :]
            xk = jnp.concatenate([xk] * (FS // 128), axis=1)
            pg = wg_v[i, 16 * k:16 * k + 16, :].astype(f32) * xk
            pu = wu_v[i, 16 * k:16 * k + 16, :].astype(f32) * xk
            acc_g += pg[:8] + pg[8:]
            acc_u += pu[:8] + pu[8:]
        gate = jnp.sum(acc_g, axis=0, keepdims=True)
        up = jnp.sum(acc_u, axis=0, keepdims=True)
        hcol = _lane_bcast_rows(gate * jax.nn.sigmoid(gate) * up)
        f0 = pl.multiple_of(i * FS, 128)
        acc_y = y_v[...]
        for k in range(FS // 16):
            hk = jnp.concatenate([hcol[16 * k:16 * k + 16]] * (D // 128), axis=1)
            py = wd_v[pl.ds(f0 + 16 * k, 16), :].astype(f32) * hk
            acc_y += py[:8] + py[8:]
        y_v[...] = acc_y

        @pl.when(i == n_chunks - 1)
        def _():
            l0 = pl.multiple_of(idx16 - s0, 16)
            y = jnp.sum(y_v[...], axis=0, keepdims=True) * r_gate
            b = x_rows + jnp.where(is_sel, y, 0.0)
            gl = _lane_bcast_rows(jax.nn.sigmoid(rg_v[c, 1:2, :]))
            xcol_v[0:TS, :] = gl
            g16 = xcol_v[pl.ds(l0, 16), :]
            g16 = jnp.concatenate([g16] * (D // 128), axis=1)
            out_v[slot, pl.ds(l0, 16), :] = (
                g16 * a_v[pl.ds(l0, 16), :] + (1.0 - g16) * b).astype(bf16)

        out_copy(c, slot).start()
        return 0

    lax.fori_loop(0, n_chunks, phase2, 0)
    out_copy(chunk_of(n_chunks - 2), n_chunks % 2).wait()
    out_copy(chunk_of(n_chunks - 1), (n_chunks - 1) % 2).wait()


@jax.jit
def pallas_gated_mix__linear_kernel_hedgehog__moe_arch_mod__prompt_kernel(
    A_x: jax.Array,
    A_wqkv: jax.Array,
    A_w_phi: jax.Array,
    A_wo: jax.Array,
    B_x: jax.Array,
    B_w_r: jax.Array,
    B_w_gate: jax.Array,
    B_w_up: jax.Array,
    B_w_down: jax.Array,
    gate_w: jax.Array,
):
    del B_x
    B, S, D = A_x.shape
    H, Dh, _ = A_w_phi.shape
    F = B_w_gate.shape[1]
    n_chunks = S // TS
    FS = F // n_chunks
    assert B == 1 and Dh == 32 and H * Dh == D and S % TS == 0 and FS % 128 == 0

    hbm = pl.BlockSpec(memory_space=pl.ANY)
    vmem = pl.BlockSpec(memory_space=pltpu.VMEM)
    out = pl.pallas_call(
        _kernel,
        out_shape=jax.ShapeDtypeStruct((S, D), A_x.dtype),
        in_specs=[hbm, hbm, vmem, hbm, vmem, hbm, hbm, hbm, vmem],
        out_specs=hbm,
        scratch_shapes=[
            pltpu.VMEM((S, D), bf16),
            pltpu.VMEM((3, D, D), bf16),
            pltpu.VMEM((D, D), bf16),
            pltpu.VMEM((n_chunks, D, FS), bf16),
            pltpu.VMEM((n_chunks, D, FS), bf16),
            pltpu.VMEM((F, D), bf16),
            pltpu.VMEM((2 * D + 16, D), bf16),
            pltpu.VMEM((D, D), bf16),
            pltpu.VMEM((H // 2, 80, 128), f32),
            pltpu.VMEM((H // 2, 80, 128), bf16),
            pltpu.VMEM((n_chunks, 8, TS), f32),
            pltpu.VMEM((TS, D), f32),
            pltpu.VMEM((2, TS, D), bf16),
            pltpu.VMEM((D, 128), f32),
            pltpu.VMEM((8, D), f32),
            pltpu.SemaphoreType.DMA((n_chunks,)),
            pltpu.SemaphoreType.DMA((4,)),
            pltpu.SemaphoreType.DMA((3, n_chunks)),
            pltpu.SemaphoreType.DMA((2,)),
        ],
        compiler_params=pltpu.CompilerParams(vmem_limit_bytes=110 * 1024 * 1024),
        name="gated_mix_hedgehog_mod",
    )(A_x.reshape(S, D), A_wqkv, A_w_phi.reshape(H * Dh, Dh), A_wo, B_w_r.reshape(1, D),
      B_w_gate, B_w_up, B_w_down, gate_w.reshape(1, D))
    return out.reshape(B, S, D)
```

```python
import jax
import jax.numpy as jnp
from jax import lax
import jax.experimental.pallas as pl
import jax.experimental.pallas.tpu as pltpu

TS = 512
LOG2E = 1.4426950408889634

_NT = (((1,), (1,)), ((), ()))
_NN = (((1,), (0,)), ((), ()))

f32 = jnp.float32
bf16 = jnp.bfloat16
i32 = jnp.int32
u32 = jnp.uint32


def _pack(even, odd):
    return pltpu.pack_elementwise([even, odd], packed_dtype=bf16)


def _unpack(words):
    return [pltpu.unpack_elementwise(words, index=p, packed_dtype=bf16, unpacked_dtype=f32)
            for p in range(2)]


def _dot(a, b, dims):
    a, b = (pltpu.bitcast(v, bf16) if v.dtype == u32 else v for v in (a, b))
    return lax.dot_general(a, b, dims, preferred_element_type=f32)


def _tree(op, xs):
    xs = list(xs)
    while len(xs) > 1:
        nxt = [op(xs[i], xs[i + 1]) for i in range(0, len(xs) - 1, 2)]
        if len(xs) % 2:
            nxt.append(xs[-1])
        xs = nxt
    return xs[0]


def _recip(x):
    return pl.reciprocal(x, full_range=False)


def _sigmoid(x):
    return 0.5 + 0.5 * jnp.tanh(0.5 * x)


def _head_reduce(op, tiles):
    r = _tree(op, tiles)
    r = op(r, pltpu.roll(r, 4, 0))
    return op(r, pltpu.roll(r, 2, 0))


def _phi(p):
    tiles = [p[8 * j:8 * j + 8] for j in range(8)]
    out = []
    for op, diff in ((jnp.maximum, lambda t, m: t - m), (jnp.minimum, lambda t, m: m - t)):
        m = _head_reduce(op, tiles)
        e = [jnp.exp2(diff(t, m)) for t in tiles]
        r = _recip(_head_reduce(jnp.add, e))
        out += [_pack(e[j] * r, e[j + 1] * r) for j in range(0, 8, 2)]
    return jnp.concatenate(out, axis=0)


def _lane_bcast_rows(row):
    return jnp.broadcast_to(row, (128, row.shape[1])).T


def _lhs_terms(a11, a12, a21, a22):
    return (a11 + a22, a21 + a22, a11, a22, a11 + a12, a21 - a11, a12 - a22)


def _rhs_terms(b11, b12, b21, b22):
    return (b11 + b22, b11, b12 - b22, b21 - b11, b22, b11 + b12, b21 + b22)


def _put_terms(dst, m, terms_fn, load):
    rows = pl.ds(8 * m, 8)
    for k in range(dst.shape[1]):
        quads = [load(i, j, k) for i in range(2) for j in range(2)]
        even, odd = (terms_fn(*[q[p] for q in quads]) for p in range(2))
        for n in range(7):
            dst[n, k, rows, :] = _pack(even[n], odd[n])
    return dst[dst.shape[0] - 1, dst.shape[1] - 1, rows, :]


def _get(ref):
    return jnp.concatenate([ref[k] for k in range(ref.shape[0])], axis=1)


def _after(lhs, row, vals, zero):
    bits = _tree(jnp.bitwise_or, [pltpu.bitcast(v, u32) for v in vals]) & zero
    mid = jnp.concatenate([lhs[row:row + 8, 0:128] | bits, lhs[row:row + 8, 128:]], axis=1)
    parts = ([lhs[:row]] if row else []) + [mid] + ([lhs[row + 8:]] if row + 8 < lhs.shape[0] else [])
    return jnp.concatenate(parts, axis=0)


def _paced_dot(lhs, rhs, dims, pieces, zero):
    if not pieces:
        return _dot(lhs, rhs, dims)
    cols = ([rhs[64 * j:64 * j + 64] for j in range(rhs.shape[0] // 64)] if dims == _NT else
            [rhs[:, 128 * j:128 * j + 128] for j in range(rhs.shape[1] // 128)])
    per = pl.cdiv(len(pieces), len(cols))
    out = []
    for j, col in enumerate(cols):
        a = lhs
        for m, piece in enumerate(pieces[j * per:(j + 1) * per]):
            vals = piece()
            if vals:
                a = _after(a, lhs.shape[0] * m // per // 8 * 8, vals, zero)
        out.append(_dot(a, col, dims))
    return jnp.concatenate(out, axis=1)


def _kernel(x_hbm, wqkv_hbm, wphi_hbm, wo_hbm, wr_hbm, wg_hbm, wu_hbm, wd_hbm, gw_hbm,
            out_hbm,
            x_v, wqkv_v, wphi_v, wr_v, gw_v, wo_v, wg_v, wu_v, wd_v, x0_v, wv_t, kv_s, q_s,
            wo_s, x_s, phi_s, kv_acc, kv_t, rmax_v, rarg_v, g_v, out_v, row_v, xcol_v, hcol_v, y_v,
            sem_x, sem_w, sem_s, sem_f, sem_o):
    S, D = x_v.shape
    F = wd_hbm.shape[0]
    n_chunks = S // TS
    n_pairs = D // 64
    FS = F // n_chunks
    HD, HT = D // 2, TS // 2
    n_wb = HD // 128
    HP = n_pairs // 2

    def x_copy(c):
        return pltpu.make_async_copy(x_hbm.at[pl.ds(c * TS, TS)], x_v.at[pl.ds(c * TS, TS)],
                                     sem_x.at[c])

    def w_copies(j, b):
        return [pltpu.make_async_copy(wqkv_hbm.at[:, pl.ds(j * D + g * 128, 128)],
                                      wqkv_v.at[j, g], sem_w.at[j, g]) for g in (b, b + n_wb)]

    small = (pltpu.make_async_copy(wphi_hbm, wphi_v, sem_s.at[0]),
             pltpu.make_async_copy(wr_hbm, wr_v, sem_s.at[1]),
             pltpu.make_async_copy(gw_hbm, gw_v, sem_s.at[2]))
    wo_copy = pltpu.make_async_copy(wo_hbm, wo_v, sem_s.at[3])

    def f_copies(i):
        return (pltpu.make_async_copy(wg_hbm.at[:, pl.ds(i * FS, FS)], wg_v.at[i], sem_f.at[0, i]),
                pltpu.make_async_copy(wu_hbm.at[:, pl.ds(i * FS, FS)], wu_v.at[i], sem_f.at[1, i]),
                pltpu.make_async_copy(wd_hbm.at[pl.ds(i * FS, FS)], wd_v.at[i], sem_f.at[2, i]))

    def start(copies):
        for cp in copies:
            cp.start()

    def wait(copies):
        for cp in copies:
            cp.wait()

    start([small[0]] + w_copies(1, 0) + [x_copy(0)] + w_copies(1, 1) + list(small[1:]))

    c_i = lax.broadcasted_iota(i32, (128, 32), 0)
    f_i = lax.broadcasted_iota(i32, (128, 32), 1)
    sel = jnp.where(8 * (c_i // 16 % 4) + c_i % 8 == f_i, 1.0, 0.0).astype(bf16)
    r_i = lax.broadcasted_iota(i32, (128, 128), 0)
    l_i = lax.broadcasted_iota(i32, (128, 128), 1)
    same_head = (2 * (r_i // 64) + r_i // 8 % 2) == (l_i // 32)

    def fold(j, g):
        phi_t = _dot(sel, wphi_v[128 * g:128 * g + 128, :], _NT)
        phi_t = jnp.where(same_head, phi_t, 0.0).astype(bf16)
        return _dot(phi_t, wqkv_v[j, g], _NT) * LOG2E

    def put_lhs(dst, r0, top, bot):
        for m in range(top.shape[0] // 16):
            _put_terms(dst, r0 // 16 + m, _lhs_terms, lambda i, j, k: [(top, bot)[i][
                16 * m + 8 * p:16 * m + 8 * p + 8, j * HD + 128 * k:j * HD + 128 * k + 128]
                for p in range(2)])

    def prep_x(c, m, best):
        w_r = wr_v[...].astype(f32)
        w_g = gw_v[...].astype(f32)
        first = [c * TS + t * HT + 16 * m for t in range(2)]
        rows = [pl.ds(pl.multiple_of(s0, 16), 16) for s0 in first]
        dots = {}

        def load(i, j, k):
            col = i * n_wb + k
            xt = _unpack(pltpu.bitcast(x_v[rows[j], 128 * col:128 * col + 128], u32))
            for p in range(2):
                for name, w in (("r", w_r), ("g", w_g)):
                    v = xt[p] * w[col:col + 1]
                    dots[name, j, p] = v + dots[name, j, p] if (name, j, p) in dots else v
            return xt

        done = _put_terms(x_s.at[c], m, _rhs_terms, load)
        for t in range(2):
            for p in range(2):
                g = jnp.broadcast_to(jnp.sum(dots["g", t, p], axis=1, keepdims=True), (8, 128))
                g_v[pl.ds(first[t] + p, 8, stride=2), :] = _sigmoid(g)
                r = jnp.broadcast_to(jnp.sum(dots["r", t, p], axis=1, keepdims=True), (8, 128))
                r = r.astype(bf16).astype(f32)
                tok = first[t] + p + 2 * lax.broadcasted_iota(i32, (8, 128), 0)
                if m:
                    better = r > best[t, p][0]
                    r = jnp.where(better, r, best[t, p][0])
                    tok = jnp.where(better, tok, best[t, p][1])
                best[t, p] = (r, tok)
                if m == HT // 16 - 1:
                    rmax_v[c, 2 * t + p], rarg_v[c, 2 * t + p] = r, tok
        return done

    def prep_wo(m):
        r0 = pl.multiple_of(16 * m, 16)
        return _put_terms(wo_s, m, _rhs_terms, lambda i, j, k: _unpack(pltpu.bitcast(wo_v[
            pl.ds(i * HD + r0, 16), j * HD + 128 * k:j * HD + 128 * k + 128], u32)))

    def prep_v(b):
        halves = [pltpu.bitcast(wqkv_v[2, g].T, u32) for g in (b, b + n_wb)]
        for k in range(D // 128):
            for g, half in zip((b, b + n_wb), halves):
                wv_t[k, 64 * g:64 * g + 64, :] = half[:, 128 * k:128 * k + 128]
        for m in range(8):
            _put_terms(kv_s, (HD + 128 * b) // 16 + m, _lhs_terms, lambda i, j, k: _unpack(
                halves[i][8 * m:8 * m + 8, j * HD + 128 * k:j * HD + 128 * k + 128]))

    def put_phi(p, j, logits):
        phi_s[p, j] = _phi(logits)
        return phi_s[p, j, 56:64, :]

    def with_ones(vt):
        return jnp.concatenate([vt, jnp.ones((16, vt.shape[1]), f32)], axis=0).astype(bf16)

    small[0].wait()
    bits = jnp.concatenate([pltpu.bitcast(wphi_v[0:16, :], u32)] * 4, axis=1)
    zero = (bits & 1) * ((bits + 1) & 1)
    wq_copies = [cp for b in range(n_wb) for cp in w_copies(0, b)]
    for b in range(n_wb):
        wait(w_copies(1, b))
        if b + 2 < n_wb:
            start(w_copies(1, b + 2))
        else:
            start(w_copies(2, 2 * (b + 2 - n_wb)) + w_copies(2, 2 * (b + 2 - n_wb) + 1))
        top, bot = fold(1, b), fold(1, b + n_wb)
        put_lhs(kv_s, 128 * b, top, bot)
        lhs = jnp.concatenate([_pack(w[r:r + 8], w[r + 8:r + 16])
                               for w in (top, bot) for r in range(0, 128, 16)], axis=0)
        if b == 0:
            x_copy(0).wait()
            for k in range(D // 128):
                x0_v[k] = pltpu.bitcast(x_v[0:TS, 128 * k:128 * k + 128], u32)
        if b == n_wb - 1:
            wait(w_copies(2, 0) + w_copies(2, 1))
            start([x_copy(1)] + wq_copies)
            prep_v(0)
            prep_v(1)
        pk = _dot(lhs, _get(x0_v), _NT)
        for j in range(TS // 128):
            for q in range(4):
                put_phi(2 * b + q % 2 + (q // 2) * HP, j, pk[64 * q:64 * q + 64, 128 * j:128 * j + 128])
    wait(w_copies(2, 2) + w_copies(2, 3) + list(small[1:]))
    prep_v(2)
    prep_v(3)

    def v_block(b, pieces):
        lhs = jnp.concatenate([wv_t[k, 128 * b:128 * b + 128, :] for k in range(D // 128)], axis=1)
        vt = _paced_dot(lhs, _get(x0_v), _NT, pieces, zero)
        for q in range(4):
            kv_acc[4 * b + q] = _dot(with_ones(vt[64 * q:64 * q + 64]), _get(phi_s.at[4 * b + q]), _NT)

    best = {}
    v_block(0, [])
    v_block(2, [])
    wait([x_copy(1)] + wq_copies)
    start([x_copy(c) for c in range(2, n_chunks)] + [wo_copy])
    v_block(1, [lambda m=m: [prep_x(1, m, best)] for m in range(16)])
    for b in range(n_wb):
        put_lhs(q_s, 128 * b, fold(0, b), fold(0, b + n_wb))
    v_block(3, [])
    wait([x_copy(c) for c in range(2, n_chunks)] + [wo_copy])
    for i in range(n_chunks):
        start(f_copies(i))

    def phase1(c, _):
        nxt = jnp.where(c + 1 < n_chunks, c + 1, 0)
        best = {}
        wo_pieces = HD // 16
        wo_per = pl.cdiv(wo_pieces, n_chunks - 1)

        def product(n, pieces=()):
            return _paced_dot(_get(kv_s.at[n]), _get(x_s.at[c, n]), _NT, pieces, zero)

        def features(half, t, res, tiles=range(2 * HP)):
            return [lambda q=n // 2, j=n % 2: [put_phi(
                half * HP + q, 2 * t + j, res[64 * q:64 * q + 64, 128 * j:128 * j + 128])]
                for n in tiles]

        def kv_update(half, t, res):
            for q in range(HP):
                p = half * HP + q
                kv_acc[p] += _dot(with_ones(res[HD + 64 * q:HD + 64 * q + 64]),
                                  _get(phi_s.at[p, 2 * t:2 * t + 2]), _NT)

        m3 = product(2)
        for m in range(0, 8):
            prep_x(nxt, m, best)
        m5 = product(4)
        for m in range(8, 16):
            prep_x(nxt, m, best)
        c12 = m3 + m5
        m4 = product(3, features(0, 1, c12))
        t = m4 - m5
        kv_update(0, 1, c12)
        m2 = product(1, [lambda j=j: [prep_wo(jnp.minimum((c - 1) * wo_per + j, wo_pieces - 1))]
                         for j in range(wo_per)])
        c21 = m2 + m4
        u = m3 - m2
        m1 = product(0, features(1, 0, c21))
        t = t + m1
        u = u + m1
        kv_update(1, 0, c21)
        m7 = product(6)
        c11 = t + m7
        m6 = product(5, features(0, 0, c11))
        c22 = u + m6
        kv_update(0, 0, c11)
        for piece in features(1, 1, c22):
            piece()
        kv_update(1, 1, c22)
        return 0

    lax.fori_loop(1, n_chunks, phase1, 0)

    kr = lax.broadcasted_iota(i32, (80, 128), 0)
    kl = lax.broadcasted_iota(i32, (80, 128), 1)
    keep = jnp.where(kr < 64, kr // 32, (kr - 64) // 8) == kl // 2 % 2
    for p in range(n_pairs):
        kv_t[p] = jnp.where(keep, kv_acc[p], 0.0).astype(bf16)

    r = rmax_v[...].reshape(n_chunks * 32, 128)
    r_max = jnp.max(r, axis=0, keepdims=True)
    tok = rarg_v[...].reshape(n_chunks * 32, 128)
    idx = jnp.min(jnp.where(r == r_max, tok, S - 1))
    r_gate = _sigmoid(r_max[:, 0:1])
    idx16 = pl.multiple_of((idx // 16) * 16, 16)
    is_sel = lax.broadcasted_iota(i32, (16, D), 0) == (idx - idx16)
    x_rows = x_v[pl.ds(idx16, 16), :].astype(f32)
    x_sel = jnp.sum(jnp.where(is_sel, x_rows, 0.0), axis=0, keepdims=True)
    xcol_v[...] = _lane_bcast_rows(x_sel)
    y_v[...] = jnp.zeros(y_v.shape, f32)
    routed = idx // TS

    def chunk_of(i):
        c = routed + i
        return jnp.where(c >= n_chunks, c - n_chunks, c)

    def out_copy(i, t, h):
        return pltpu.make_async_copy(
            out_v.at[i, t, h],
            out_hbm.at[pl.ds(chunk_of(i) * TS + t * HT, HT), pl.ds(h * HD, HD)], sem_o.at[i, 2 * t + h])

    def phase2(i, _):
        c = chunk_of(i)
        wait(f_copies(i))

        def mat_vec(acc, col_ref, w_refs, k0, k1):
            for k in range(k0, k1):
                col = col_ref[8 * k:8 * k + 8, :]
                for a, w_ref in enumerate(w_refs):
                    n = w_ref.shape[2] // 128
                    for j0 in range(0, n, 2):
                        j1 = min(j0 + 2, n)
                        w = w_ref[i, 8 * k:8 * k + 8, 128 * j0:128 * j1].astype(f32)
                        for j in range(j0, j1):
                            p = w[:, 128 * (j - j0):128 * (j - j0) + 128] * col
                            acc[a * n + j] = p if acc[a * n + j] is None else acc[a * n + j] + p
            return list(acc)

        gu = [None] * (2 * FS // 128)
        y = [y_v[:, 128 * j:128 * j + 128] for j in range(D // 128)]

        def spread(fn, k0, k1, n):
            cuts = [k0 + (k1 - k0) * m // n for m in range(n + 1)]
            return [lambda a=a, b=b: fn(a, b) for a, b in zip(cuts[:-1], cuts[1:])]

        def gate_up(k0, k1, n):
            return spread(lambda a, b: mat_vec(gu, xcol_v, (wg_v, wu_v), a, b), k0, k1, n)

        def down(k0, k1, n):
            return spread(lambda a, b: mat_vec(y, hcol_v, (wd_v,), a, b), k0, k1, n)

        def q_product(n, pieces=()):
            return _paced_dot(_get(q_s.at[n]), _get(x_s.at[c, n]), _NT, pieces, zero)

        def features(half, t, res, n0, n1):
            return [lambda q=n // 2, j=n % 2: [put_phi(
                half * HP + q, 2 * t + j, res[64 * q:64 * q + 64, 128 * j:128 * j + 128])]
                for n in range(n0, n1)]

        def attend(half, t):
            o_t = []
            for q in range(HP):
                p = half * HP + q
                nd = _dot(kv_t[p], _get(phi_s.at[p, 2 * t:2 * t + 2]), _NN)
                for h in range(2):
                    inv = _recip(nd[64 + 8 * h:72 + 8 * h] + 1e-6)
                    o_t += [nd[32 * h + 8 * j:32 * h + 8 * j + 8] * inv for j in range(4)]
            return jnp.concatenate(o_t, axis=0)

        def o_product(n, o_t, pieces=()):
            lhs = pltpu.bitcast(o_t.astype(bf16).T, u32)
            return _paced_dot(lhs, _get(wo_s.at[n]), _NN, pieces, zero)

        def mix(t, h, a):
            for m in range(HT // 16):
                rows = pl.ds(pl.multiple_of(c * TS + t * HT + 16 * m, 16), 16)
                g = g_v[rows, :]
                for k in range(HD // 128):
                    xb = x_v[rows, h * HD + 128 * k:h * HD + 128 * k + 128].astype(f32)
                    out_v[i, t, h, 16 * m:16 * m + 16, 128 * k:128 * k + 128] = (
                        g * a[16 * m:16 * m + 16, 128 * k:128 * k + 128] + (1.0 - g) * xb).astype(bf16)
            out_copy(i, t, h).start()

        m3 = q_product(2, gate_up(0, 22, 8))
        m5 = q_product(4, gate_up(22, 48, 8))
        c12 = m3 + m5
        m4 = q_product(3, features(0, 1, c12, 0, 8))
        t = m4 - m5
        m2 = q_product(1, features(0, 1, c12, 8, 16))
        c21 = m2 + m4
        u = m3 - m2
        a11 = attend(0, 1)
        m1 = q_product(0, features(1, 0, c21, 0, 8))
        t = t + m1
        u = u + m1
        m7 = q_product(6, features(1, 0, c21, 8, 16))
        c11 = t + m7
        a22 = attend(1, 0)
        m6 = q_product(5, features(0, 0, c11, 0, 8))
        c22 = u + m6
        m3 = o_product(2, a11, features(0, 0, c11, 8, 16))
        a21 = attend(0, 0)
        m4 = o_product(3, a22, features(1, 1, c22, 0, 8))
        m1 = o_product(0, a11 + a22, features(1, 1, c22, 8, 16))
        a12 = attend(1, 1)
        t = m1 + m4
        u = m1 + m3
        m2 = o_product(1, a21 + a22, gate_up(48, 88, 8))
        mix(0, 0, m2 + m4)
        u = u - m2
        m6 = o_product(5, a21 - a11, gate_up(88, 128, 8))
        mix(0, 1, u + m6)
        n = FS // 128
        gate = jnp.sum(jnp.concatenate(gu[:n], axis=1), axis=0, keepdims=True)
        up = jnp.sum(jnp.concatenate(gu[n:], axis=1), axis=0, keepdims=True)
        hcol_v[...] = _lane_bcast_rows(gate * _sigmoid(gate) * up)
        m5 = o_product(4, a11 + a12, [list] * 2 + down(0, 48, 6))
        mix(1, 1, m3 + m5)
        t = t - m5
        m7 = o_product(6, a12 - a22, down(48, FS // 8, 8))
        mix(1, 0, t + m7)
        y_v[...] = jnp.concatenate(y, axis=1)
        return 0

    lax.fori_loop(0, n_chunks, phase2, 0)

    wait([out_copy(0, t, h) for t in range(2) for h in range(2)])
    t_sel = (idx16 - routed * TS) // HT
    rows = pl.ds(pl.multiple_of(idx16 - routed * TS - t_sel * HT, 16), 16)
    staged = jnp.concatenate([out_v[0, t_sel, h, rows, :] for h in range(2)], axis=1).astype(f32)
    g = jnp.concatenate([g_v[pl.ds(idx16, 16), :]] * (D // 128), axis=1)
    y = jnp.sum(y_v[...], axis=0, keepdims=True) * r_gate
    row_v[...] = (staged + jnp.where(is_sel, (1.0 - g) * y, 0.0)).astype(bf16)
    row_copy = pltpu.make_async_copy(row_v, out_hbm.at[pl.ds(idx16, 16)], sem_s.at[4])
    row_copy.start()
    wait([out_copy(i, t, h) for i in range(1, n_chunks) for t in range(2) for h in range(2)])
    row_copy.wait()


@jax.jit
def pallas_gated_mix__linear_kernel_hedgehog__moe_arch_mod__prompt_kernel(
    A_x: jax.Array,
    A_wqkv: jax.Array,
    A_w_phi: jax.Array,
    A_wo: jax.Array,
    B_x: jax.Array,
    B_w_r: jax.Array,
    B_w_gate: jax.Array,
    B_w_up: jax.Array,
    B_w_down: jax.Array,
    gate_w: jax.Array,
):
    del B_x
    B, S, D = A_x.shape
    H, Dh, _ = A_w_phi.shape
    F = B_w_gate.shape[1]
    n_chunks = S // TS
    FS = F // n_chunks
    HD, HT = D // 2, TS // 2
    assert B == 1 and Dh == 32 and D == 1024 and H * Dh == D and S % TS == 0 and FS % 128 == 0

    hbm = pl.BlockSpec(memory_space=pl.ANY)
    out = pl.pallas_call(
        _kernel,
        out_shape=jax.ShapeDtypeStruct((S, D), A_x.dtype),
        in_specs=[hbm] * 9,
        out_specs=hbm,
        scratch_shapes=[
            pltpu.VMEM((S, D), bf16),
            pltpu.VMEM((3, D // 128, D, 128), bf16),
            pltpu.VMEM((H * Dh, Dh), bf16),
            pltpu.VMEM((8, 128), bf16),
            pltpu.VMEM((8, 128), bf16),
            pltpu.VMEM((D, D), bf16),
            pltpu.VMEM((n_chunks, D, FS), bf16),
            pltpu.VMEM((n_chunks, D, FS), bf16),
            pltpu.VMEM((n_chunks, FS, D), bf16),
            pltpu.VMEM((D // 128, TS // 2, 128), u32),
            pltpu.VMEM((D // 128, D // 2, 128), u32),
            pltpu.VMEM((7, HD // 128, D // 2, 128), u32),
            pltpu.VMEM((7, HD // 128, HD // 2, 128), u32),
            pltpu.VMEM((7, HD // 128, HD // 2, 128), u32),
            pltpu.VMEM((n_chunks, 7, HD // 128, HT // 2, 128), u32),
            pltpu.VMEM((H // 2, TS // 128, 64, 128), u32),
            pltpu.VMEM((H // 2, 80, 128), f32),
            pltpu.VMEM((H // 2, 80, 128), bf16),
            pltpu.VMEM((n_chunks, 4, 8, 128), f32),
            pltpu.VMEM((n_chunks, 4, 8, 128), i32),
            pltpu.VMEM((S, 128), f32),
            pltpu.VMEM((n_chunks, 2, 2, HT, HD), bf16),
            pltpu.VMEM((16, D), bf16),
            pltpu.VMEM((D, 128), f32),
            pltpu.VMEM((FS, 128), f32),
            pltpu.VMEM((8, D), f32),
            pltpu.SemaphoreType.DMA((n_chunks,)),
            pltpu.SemaphoreType.DMA((3, D // 128)),
            pltpu.SemaphoreType.DMA((5,)),
            pltpu.SemaphoreType.DMA((3, n_chunks)),
            pltpu.SemaphoreType.DMA((n_chunks, 4)),
        ],
        compiler_params=pltpu.CompilerParams(vmem_limit_bytes=110 * 1024 * 1024),
        name="gated_mix_hedgehog_mod",
    )(A_x.reshape(S, D), A_wqkv, A_w_phi.reshape(H * Dh, Dh), A_wo, B_w_r.reshape(8, 128),
      B_w_gate, B_w_up, B_w_down, gate_w.reshape(8, 128))
    return out.reshape(B, S, D)
```

```python
import functools

import jax
import jax.numpy as jnp
from jax import lax
import jax.experimental.pallas as pl
import jax.experimental.pallas.tpu as pltpu

TS = 512
LOG2E = 1.4426950408889634
KS = 2
RATE = 1.3

_NT = (((1,), (1,)), ((), ()))
_NN = (((1,), (0,)), ((), ()))

f32 = jnp.float32
bf16 = jnp.bfloat16
i32 = jnp.int32
u32 = jnp.uint32


def _pack(even, odd):
    return pltpu.pack_elementwise([even, odd], packed_dtype=bf16)


def _unpack(words):
    return [pltpu.unpack_elementwise(words, index=p, packed_dtype=bf16, unpacked_dtype=f32)
            for p in range(2)]


def _dot(a, b, dims):
    a, b = (pltpu.bitcast(v, bf16) if v.dtype == u32 else v for v in (a, b))
    return lax.dot_general(a, b, dims, preferred_element_type=f32)


def _tree(op, xs):
    xs = list(xs)
    while len(xs) > 1:
        nxt = [op(xs[i], xs[i + 1]) for i in range(0, len(xs) - 1, 2)]
        if len(xs) % 2:
            nxt.append(xs[-1])
        xs = nxt
    return xs[0]


def _recip(x):
    return pl.reciprocal(x, full_range=False)


def _sigmoid(x):
    return 0.5 + 0.5 * jnp.tanh(0.5 * x)


def _head_reduce(op, tiles):
    r = _tree(op, tiles)
    r = op(r, pltpu.roll(r, 4, 0))
    return op(r, pltpu.roll(r, 2, 0))


def _phi(p, hold):
    tiles = [p[8 * j:8 * j + 8] for j in range(8)]
    out = []
    for op, diff in ((jnp.maximum, lambda t, m: t - m), (jnp.minimum, lambda t, m: m - t)):
        m = hold(_head_reduce(op, tiles))
        e = [jnp.exp2(diff(t, m)) for t in tiles]
        r = _recip(_head_reduce(jnp.add, e))
        out += [_pack(e[j] * r, e[j + 1] * r) for j in range(0, 8, 2)]
    return jnp.concatenate(out, axis=0)


def _lane_bcast_rows(row):
    return jnp.broadcast_to(row, (128, row.shape[1])).T


def _lhs_terms(a11, a12, a21, a22):
    return (a11 + a22, a21 + a22, a11, a22, a11 + a12, a21 - a11, a12 - a22)


def _rhs_terms(b11, b12, b21, b22):
    return (b11 + b22, b11, b12 - b22, b21 - b11, b22, b11 + b12, b21 + b22)


def _put_terms(dst, m, terms_fn, load):
    rows = pl.ds(8 * m, 8)
    for k in range(dst.shape[1]):
        quads = [load(i, j, k) for i in range(2) for j in range(2)]
        even, odd = (terms_fn(*[q[p] for q in quads]) for p in range(2))
        for n in range(7):
            dst[n, k, rows, :] = _pack(even[n], odd[n])
    return dst[dst.shape[0] - 1, dst.shape[1] - 1, rows, :]


def _get(ref):
    return jnp.concatenate([ref[k] for k in range(ref.shape[0])], axis=1)


class _Pacer:
    def __init__(self, zero):
        self.zero = zero
        self.previous = None
        self.tick = 0
        self.queues = ([], [])

    def add(self, tag, cost, pieces, urgent=False):
        self.queues[0 if urgent else 1].extend(
            (tag, cost, max(self.tick + urgent, 1), p) for p in pieces)

    def flush(self, tag):
        for queue in self.queues:
            for item in [q for q in queue if q[0] == tag]:
                queue[:] = [q for q in queue if q is not item]
                item[3](lambda v: v)

    def _take(self, budget):
        taken = ([], [])
        for queue, out in zip(self.queues, taken):
            while queue and queue[0][2] <= self.tick and budget >= queue[0][1] / 2:
                budget -= queue[0][1]
                out.append(queue.pop(0)[3])
        return taken

    def _hold(self, where):
        rows = self.previous.shape[0] // 8
        start = pltpu.bitcast(self.previous[int(where * rows) * 8:][:8], u32) & self.zero
        return lambda v: pltpu.bitcast(pltpu.bitcast(v, u32) | start, v.dtype)

    def dot(self, lhs, rhs, dims):
        n = rhs.shape[0] // 64 if dims == _NT else rhs.shape[1] // 128
        out = []
        for j in range(n):
            marks = {}
            urgent, chain = self._take(RATE * lhs.shape[0] * lhs.shape[1] / 256)
            for pieces, shift in ((urgent, 0.0), (chain, 0.5)):
                for m, piece in enumerate(pieces):
                    where = (m + shift) / len(pieces)
                    done = piece(self._hold(where))
                    if done and (pieces is urgent or m == len(pieces) - 1):
                        marks.setdefault(int(where * lhs.shape[0] / 8) * 8, []).extend(done)
            parts, at = [], 0
            for row, done in sorted(marks.items()):
                bits = _tree(jnp.bitwise_or, [pltpu.bitcast(v, u32) for v in done]) & self.zero
                parts += [lhs[at:row]] if row > at else []
                parts.append(jnp.concatenate(
                    [lhs[row:row + 8, 0:128] | bits, lhs[row:row + 8, 128:]], axis=1))
                at = row + 8
            a = jnp.concatenate(parts + ([lhs[at:]] if at < lhs.shape[0] else []), axis=0)
            out.append(_dot(a, rhs[64 * j:64 * j + 64] if dims == _NT else
                            rhs[:, 128 * j:128 * j + 128], dims))
            self.previous = out[-1]
            self.tick += 1
        return jnp.concatenate(out, axis=1)


def _kernel(x_hbm, wqkv_hbm, wphi_hbm, wo_hbm, wr_hbm, wg_hbm, wu_hbm, wd_hbm, gw_hbm,
            out_hbm,
            x_v, wqkv_v, wphi_v, wr_v, gw_v, wo_v, wg_v, wu_v, wd_v, wrg_v, fold_v, phi_t, x0_v, wv_t, kv_s, q_s,
            wo_s, x_s, xn_s, phi_s, kv_acc, kv_t, rmax_v, rarg_v, g_v, out_v, row_v, xcol_v, hcol_v, y_v,
            sem_x, sem_w, sem_s, sem_o):
    S, D = x_v.shape
    F = wd_hbm.shape[0]
    n_chunks = S // TS
    n_pairs = D // 64
    FS = hcol_v.shape[0]
    HD, HT = D // 2, TS // 2
    n_wb = HD // 128
    HP = n_pairs // 2

    def x_copy(h0, h1):
        rows = pl.ds(h0 * HT, (h1 - h0) * HT)
        return pltpu.make_async_copy(x_hbm.at[rows], x_v.at[rows], sem_x.at[h0])

    def w_copies(j, b):
        return [pltpu.make_async_copy(wqkv_hbm.at[:, pl.ds(j * D + g * 128, 128)],
                                      wqkv_v.at[j, g], sem_w.at[j, g]) for g in (b, b + n_wb)]

    whole = [pltpu.make_async_copy(src, dst, sem_s.at[n]) for n, (src, dst) in enumerate(
        [(wphi_hbm, wphi_v), (wr_hbm, wr_v), (gw_hbm, gw_v), (wo_hbm, wo_v)]
        + [pair for i in range(n_chunks) for pair in (
            (wg_hbm.at[:, pl.ds(i * FS, FS)], wg_v.at[i]),
            (wu_hbm.at[:, pl.ds(i * FS, FS)], wu_v.at[i]),
            (wd_hbm.at[pl.ds(i * FS, FS)], wd_v.at[i]))])]

    def start(copies):
        for cp in copies:
            cp.start()

    def wait(copies):
        for cp in copies:
            cp.wait()

    start(whole[0:1] + w_copies(1, 0) + [x_copy(0, 1)] + whole[1:3])

    c_i = lax.broadcasted_iota(i32, (128, 32), 0)
    f_i = lax.broadcasted_iota(i32, (128, 32), 1)
    sel = jnp.where(8 * (c_i // 16 % 4) + c_i % 8 == f_i, 1.0, 0.0).astype(bf16)
    r_i = lax.broadcasted_iota(i32, (128, 128), 0)
    l_i = lax.broadcasted_iota(i32, (128, 128), 1)
    same_head = (2 * (r_i // 64) + r_i // 8 % 2) == (l_i // 32)

    def fold(j, b, dst, tag):
        for i in range(2):
            g = b + i * n_wb
            fold_v[j, b, i] = _dot(phi_t[g], pltpu.bitcast(wqkv_v[j, g], u32), _NT) * LOG2E
        pacer.add(tag, 70, [lambda hold, m=m: [_put_terms(
            dst, 8 * b + m, _lhs_terms, lambda i, jj, k: [hold(fold_v[
                j, b, i, 16 * m + 8 * p:16 * m + 8 * p + 8, jj * HD + 128 * k:jj * HD + 128 * k + 128])
                for p in range(2)])] for m in range(8)])

    def prep_x(c, dst, m, best, hold):
        first = [pl.multiple_of(c * TS + t * HT + 16 * m, 16) for t in range(2)]
        dots = {}

        def load(i, j, k):
            col = i * n_wb + k
            xt = _unpack(hold(pltpu.bitcast(x_v[pl.ds(first[j], 16), 128 * col:128 * col + 128], u32)))
            for p in range(2):
                for name, w in (("r", wrg_v[0, col]), ("g", wrg_v[1, col])):
                    v = xt[p] * w
                    dots[name, j, p] = v + dots[name, j, p] if (name, j, p) in dots else v
            return xt

        done = [_put_terms(dst, m, _rhs_terms, load)]
        for t in range(2):
            for p in range(2):
                g = jnp.broadcast_to(jnp.sum(dots["g", t, p], axis=1, keepdims=True), (8, 128))
                g = _sigmoid(g)
                g_v[pl.ds(first[t] + p, 8, stride=2), :] = g
                r = jnp.broadcast_to(jnp.sum(dots["r", t, p], axis=1, keepdims=True), (8, 128))
                r = r.astype(bf16).astype(f32)
                tok = first[t] + p + 2 * lax.broadcasted_iota(i32, (8, 128), 0)
                if m:
                    better = r > best[t, p][0]
                    r = jnp.where(better, r, best[t, p][0])
                    tok = jnp.where(better, tok, best[t, p][1])
                best[t, p] = (r, tok)
                done += [g, tok]
                if m == HT // 16 - 1:
                    rmax_v[c, 2 * t + p], rarg_v[c, 2 * t + p] = r, tok
        return done

    def prep_wo(m, hold):
        r0 = pl.multiple_of(16 * m, 16)
        return [_put_terms(wo_s, m, _rhs_terms, lambda i, j, k: _unpack(hold(pltpu.bitcast(
            wo_v[pl.ds(i * HD + r0, 16), j * HD + 128 * k:j * HD + 128 * k + 128], u32))))]

    def prep_v(b):
        halves = [pltpu.bitcast(wqkv_v[2, g].T, u32) for g in (b, b + n_wb)]
        for k in range(D // 128):
            for g, half in zip((b, b + n_wb), halves):
                wv_t[k, 64 * g:64 * g + 64, :] = half[:, 128 * k:128 * k + 128]
        return [lambda hold, m=m: [_put_terms(
            kv_s, (HD + 128 * b) // 16 + m, _lhs_terms, lambda i, j, k: _unpack(hold(
                wv_t[j * n_wb + k, 64 * (b + i * n_wb) + 8 * m:64 * (b + i * n_wb) + 8 * m + 8, :])))]
            for m in range(8)]

    def put_phi(p, j, logits, hold):
        phi_s[p, j] = _phi(logits, hold)
        return [phi_s[p, j, 56:64, :]]

    def features(pacer, tag, pairs, j0, res):
        pacer.add(tag, 100, [lambda hold, q=q, p=p, j=j: put_phi(
            p, j0 + j, res[64 * q:64 * q + 64, 128 * j:128 * j + 128], hold)
            for q, p in enumerate(pairs) for j in range(res.shape[1] // 128)], urgent=True)

    def with_ones(vt):
        return jnp.concatenate([vt, jnp.ones((16, vt.shape[1]), f32)], axis=0).astype(bf16)

    wait(whole[0:1])
    bits = jnp.concatenate([pltpu.bitcast(wphi_v[0:16, :], u32)] * 4, axis=1)
    zero = (bits & 1) * ((bits + 1) & 1)
    pacer = _Pacer(zero)
    for g in range(D // 128):
        spread = _dot(sel, wphi_v[128 * g:128 * g + 128, :], _NT)
        phi_t[g] = pltpu.bitcast(jnp.where(same_head, spread, 0.0).astype(bf16), u32)
    rmax_v[...] = jnp.full(rmax_v.shape, -jnp.inf, f32)
    rarg_v[...] = jnp.zeros(rarg_v.shape, i32)

    def stage_x(t):
        for k in range(D // 128):
            x0_v[k, t * HT // 2:(t + 1) * HT // 2, :] = pltpu.bitcast(
                x_v[t * HT:(t + 1) * HT, 128 * k:128 * k + 128], u32)

    def k_block(b, t0, t1):
        lhs = jnp.concatenate([_pack(fold_v[1, b, i, r:r + 8, :], fold_v[1, b, i, r + 8:r + 16, :])
                               for i in range(2) for r in range(0, 128, 16)], axis=0)
        pk = pacer.dot(lhs, _get(x0_v.at[:, t0 * HT // 2:t1 * HT // 2]), _NT)
        features(pacer, "k", [2 * b, 2 * b + 1, HP + 2 * b, HP + 2 * b + 1], 2 * t0, pk)

    def v_block(b):
        lhs = jnp.concatenate([wv_t[k, 128 * b:128 * b + 128, :] for k in range(D // 128)], axis=1)
        vt = pacer.dot(lhs, _get(x0_v), _NT)
        pacer.flush("k")
        for q in range(4):
            kv_acc[4 * b + q] = _dot(with_ones(vt[64 * q:64 * q + 64]), _get(phi_s.at[4 * b + q]), _NT)

    def queue_x(pacer, c, dst):
        best = {}
        pacer.add("x", 280, [lambda hold, m=m: prep_x(c, dst, m, best, hold) for m in range(HT // 16)])

    strips = lambda j, b0, b1: [cp for b in range(b0, b1) for cp in w_copies(j, b)]
    wait(strips(1, 0, 1))
    start(strips(1, 1, 2))
    fold(1, 0, kv_s, "kv")
    wait([x_copy(0, 1)])
    start([x_copy(1, 2)])
    stage_x(0)
    k_block(0, 0, 1)
    wait(strips(1, 1, 2))
    start(strips(1, 2, 4))
    fold(1, 1, kv_s, "kv")
    k_block(1, 0, 1)
    wait([x_copy(1, 2)] + strips(1, 2, 3))
    start(strips(2, 0, 4))
    stage_x(1)
    k_block(0, 1, 2)
    fold(1, 2, kv_s, "kv")
    k_block(1, 1, 2)
    wait(strips(1, 3, 4))
    fold(1, 3, kv_s, "kv")
    k_block(2, 0, 2)
    wait(strips(2, 0, 4) + whole[1:3])
    start(strips(0, 0, 4) + [x_copy(2, 4)])
    for n, w in enumerate((wr_v, gw_v)):
        w = w[...].astype(f32)
        for col in range(D // 128):
            wrg_v[n, col] = jnp.broadcast_to(w[col:col + 1], (8, 128))
    pacer.add("kv", 90, prep_v(0) + prep_v(1))
    k_block(3, 0, 2)
    pacer.add("kv", 90, prep_v(2) + prep_v(3))
    v_block(0)
    wait(strips(0, 0, 4) + [x_copy(2, 4)])
    start([x_copy(4, 8)] + whole[3:4])
    queue_x(pacer, 1, x_s.at[1])
    fold(0, 0, q_s, "q")
    v_block(2)
    fold(0, 1, q_s, "q")
    fold(0, 2, q_s, "q")
    v_block(1)
    fold(0, 3, q_s, "q")
    v_block(3)
    for tag in ("kv", "x", "q"):
        pacer.flush(tag)
    wait([x_copy(4, 8)] + whole[3:4])
    start(whole[4:])

    def project(pacer, lhs_s, c, finish):
        product = lambda n: pacer.dot(_get(lhs_s.at[n]), _get(x_s.at[c, n]), _NT)
        m3 = product(2)
        m5 = product(4)
        s12 = finish(0, 1, m3 + m5)
        m4 = product(3)
        t = m4 - m5
        m2 = product(1)
        s12()
        s21 = finish(1, 0, m2 + m4)
        u = m3 - m2
        m1 = product(0)
        t = t + m1
        u = u + m1
        m7 = product(6)
        s21()
        s11 = finish(0, 0, t + m7)
        m6 = product(5)
        return s11, finish(1, 1, u + m6)

    def phase1(c, _):
        pacer = _Pacer(zero)
        nxt = jnp.where(c + 1 < n_chunks, c + 1, 0)
        wo_per = pl.cdiv(HD // 16, n_chunks - 1)
        queue_x(pacer, nxt, xn_s)
        pacer.add("wo", 120, [lambda hold, j=j: prep_wo(
            jnp.minimum((c - 1) * wo_per + j, HD // 16 - 1), hold) for j in range(wo_per)])
        kr = lax.broadcasted_iota(i32, (80, 128), 0)
        kl = lax.broadcasted_iota(i32, (80, 128), 1)
        keep = jnp.where(kr < 64, kr // 32, (kr - 64) // 8) == kl // 2 % 2

        def kv_finish(half, t, res):
            features(pacer, (half, t), range(half * HP, half * HP + HP), 2 * t, res)

            def update():
                pacer.flush((half, t))
                for q in range(HP):
                    p = half * HP + q
                    acc = kv_acc[p] + _dot(with_ones(res[HD + 64 * q:HD + 64 * q + 64]),
                                           _get(phi_s.at[p, 2 * t:2 * t + 2]), _NT)
                    kv_acc[p] = acc
                    if half == t:
                        kv_t[p] = jnp.where(keep, acc, 0.0).astype(bf16)
            return update

        s11, s22 = project(pacer, kv_s, c, kv_finish)
        pacer.flush("x")
        x_s[nxt] = xn_s[...]

        r = rmax_v[...].reshape(n_chunks * 32, 128)
        tok = rarg_v[...].reshape(n_chunks * 32, 128)
        r_max = jnp.max(r, axis=0, keepdims=True)
        idx = jnp.min(jnp.where(r == r_max, tok, S - 1))
        rows = x_v[pl.ds(pl.multiple_of((idx // 16) * 16, 16), 16), :].astype(f32)
        is_sel = lax.broadcasted_iota(i32, (16, D), 0) == idx % 16
        xcol_v[...] = _lane_bcast_rows(jnp.sum(jnp.where(is_sel, rows, 0.0), axis=0, keepdims=True))
        s11()
        s22()
        pacer.flush("wo")
        return idx, r_max

    idx, r_max = lax.fori_loop(1, n_chunks, phase1, (jnp.int32(0), jnp.zeros((1, 128), f32)))
    y_v[...] = jnp.zeros(y_v.shape, f32)
    routed = idx // TS
    wait(whole[4:])

    def chunk_of(i):
        c = routed + i
        return jnp.where(c >= n_chunks, c - n_chunks, c)

    def out_copy(i, t, h):
        return pltpu.make_async_copy(
            out_v.at[i, t, h],
            out_hbm.at[pl.ds(chunk_of(i) * TS + t * HT, HT), pl.ds(h * HD, HD)],
            sem_o.at[jnp.minimum(i, 1)])

    def phase2(i, _):
        pacer = _Pacer(zero)
        c = chunk_of(i)

        def mat_vec(acc, col_ref, blocks, k0, hold):
            for k in range(k0, k0 + KS):
                col = hold(col_ref[8 * k:8 * k + 8, :])
                for a, block in enumerate(blocks):
                    n = block.shape[1] // 128
                    for j0 in range(0, n, 2):
                        j1 = min(j0 + 2, n)
                        w = block[8 * k:8 * k + 8, 128 * j0:128 * j1].astype(f32)
                        for j in range(j0, j1):
                            p = w[:, 128 * (j - j0):128 * (j - j0) + 128] * col
                            acc[a * n + j] = p if acc[a * n + j] is None else acc[a * n + j] + p
            return list(acc)

        def hidden(hold):
            gate, up = (jnp.sum(jnp.concatenate(v, axis=1), axis=0, keepdims=True)
                        for v in (gu[:FS // 128], gu[FS // 128:]))
            hcol_v[...] = _lane_bcast_rows(gate * _sigmoid(gate) * up)
            return [hcol_v[FS - 8:FS, :]]

        gu = [None] * (2 * FS // 128)
        y = [y_v[:, 128 * j:128 * j + 128] for j in range(D // 128)]
        pacer.add("ffn", KS * 43, [lambda hold, k=k: mat_vec(gu, xcol_v, (wg_v.at[i], wu_v.at[i]), k, hold)
                                  for k in range(0, D // 8, KS)])
        pacer.add("ffn", 400, [hidden])
        pacer.add("ffn", KS * 25, [lambda hold, k=k: mat_vec(y, hcol_v, (wd_v.at[i],), k, hold)
                                  for k in range(0, FS // 8, KS)])
        o = {}

        def q_finish(half, t, res):
            features(pacer, (half, t), range(half * HP, half * HP + HP), 2 * t, res)

            def attend():
                pacer.flush((half, t))
                o_t = []
                for p in range(half * HP, half * HP + HP):
                    nd = _dot(kv_t[p], _get(phi_s.at[p, 2 * t:2 * t + 2]), _NN)
                    for h in range(2):
                        inv = _recip(nd[64 + 8 * h:72 + 8 * h] + 1e-6)
                        o_t += [nd[32 * h + 8 * j:32 * h + 8 * j + 8] * inv for j in range(4)]
                o[t, half] = jnp.concatenate(o_t, axis=0)
            return attend

        def o_product(n, o_t):
            return pacer.dot(pltpu.bitcast(o_t.astype(bf16).T, u32), _get(wo_s.at[n]), _NN)

        def mix(t, h, a):
            def piece(m, hold):
                rows = pl.ds(pl.multiple_of(c * TS + t * HT + 16 * m, 16), 16)
                g = g_v[rows, :]
                g = jnp.concatenate([hold(g[:8]), hold(g[8:])], axis=0)
                for k in range(HD // 128):
                    xb = x_v[rows, h * HD + 128 * k:h * HD + 128 * k + 128].astype(f32)
                    out_v[i, t, h, 16 * m:16 * m + 16, 128 * k:128 * k + 128] = (
                        g * a[16 * m:16 * m + 16, 128 * k:128 * k + 128] + (1.0 - g) * xb).astype(bf16)
                return [out_v[i, t, h, 16 * m:16 * m + 16, HD - 128:HD]]

            pacer.add(("mix", t, h), 60, [functools.partial(piece, m) for m in range(HT // 16)], True)

            def send():
                pacer.flush(("mix", t, h))
                out_copy(i, t, h).start()
            return send

        s11, s22 = project(pacer, q_s, c, q_finish)
        m3 = o_product(2, o[1, 0])
        s11()
        m4 = o_product(3, o[0, 1])
        m1 = o_product(0, o[1, 0] + o[0, 1])
        s22()
        t = m1 + m4
        u = m1 + m3
        m2 = o_product(1, o[0, 0] + o[0, 1])
        send = mix(0, 0, m2 + m4)
        u = u - m2
        m6 = o_product(5, o[0, 0] - o[1, 0])
        send()
        send = mix(0, 1, u + m6)
        m5 = o_product(4, o[1, 0] + o[1, 1])
        send()
        send = mix(1, 1, m3 + m5)
        t = t - m5
        m7 = o_product(6, o[1, 1] - o[0, 1])
        send()
        mix(1, 0, t + m7)()
        pacer.flush("ffn")
        y_v[...] = jnp.concatenate(y, axis=1)
        return 0

    lax.fori_loop(0, n_chunks, phase2, 0)

    pacer.flush("ffn")
    sent = lambda rows, n: pltpu.make_async_copy(out_v.at[rows], out_v.at[rows], sem_o.at[n])
    sent(slice(0, 1), 0).wait()
    idx16 = pl.multiple_of((idx // 16) * 16, 16)
    t_sel = idx % TS // HT
    rows = pl.ds(pl.multiple_of(idx16 % HT, 16), 16)
    staged = jnp.concatenate([out_v[0, t_sel, h, rows, :] for h in range(2)], axis=1).astype(f32)
    g = jnp.concatenate([g_v[pl.ds(idx16, 16), :]] * (D // 128), axis=1)
    y = jnp.sum(y_v[...], axis=0, keepdims=True) * _sigmoid(r_max[:, 0:1])
    is_sel = lax.broadcasted_iota(i32, (16, D), 0) == idx % 16
    row_v[...] = (staged + jnp.where(is_sel, (1.0 - g) * y, 0.0)).astype(bf16)
    row_copy = pltpu.make_async_copy(row_v, out_hbm.at[pl.ds(idx16, 16)], sem_o.at[0])
    row_copy.start()
    sent(slice(1, n_chunks), 1).wait()
    row_copy.wait()


@jax.jit
def pallas_gated_mix__linear_kernel_hedgehog__moe_arch_mod__prompt_kernel(
    A_x: jax.Array,
    A_wqkv: jax.Array,
    A_w_phi: jax.Array,
    A_wo: jax.Array,
    B_x: jax.Array,
    B_w_r: jax.Array,
    B_w_gate: jax.Array,
    B_w_up: jax.Array,
    B_w_down: jax.Array,
    gate_w: jax.Array,
):
    del B_x
    B, S, D = A_x.shape
    H, Dh, _ = A_w_phi.shape
    F = B_w_gate.shape[1]
    n_chunks = S // TS
    FS = F // n_chunks
    HD, HT = D // 2, TS // 2
    assert B == 1 and Dh == 32 and D == 1024 and H * Dh == D and S == 4 * TS and FS % 128 == 0

    hbm = pl.BlockSpec(memory_space=pl.ANY)
    out = pl.pallas_call(
        _kernel,
        out_shape=jax.ShapeDtypeStruct((S, D), A_x.dtype),
        in_specs=[hbm] * 9,
        out_specs=hbm,
        scratch_shapes=[
            pltpu.VMEM((S, D), bf16),
            pltpu.VMEM((3, D // 128, D, 128), bf16),
            pltpu.VMEM((H * Dh, Dh), bf16),
            pltpu.VMEM((8, 128), bf16),
            pltpu.VMEM((8, 128), bf16),
            pltpu.VMEM((D, D), bf16),
            pltpu.VMEM((n_chunks, D, FS), bf16),
            pltpu.VMEM((n_chunks, D, FS), bf16),
            pltpu.VMEM((n_chunks, FS, D), bf16),
            pltpu.VMEM((2, D // 128, 8, 128), f32),
            pltpu.VMEM((2, HD // 128, 2, 128, D), f32),
            pltpu.VMEM((D // 128, 64, 128), u32),
            pltpu.VMEM((D // 128, TS // 2, 128), u32),
            pltpu.VMEM((D // 128, D // 2, 128), u32),
            pltpu.VMEM((7, HD // 128, D // 2, 128), u32),
            pltpu.VMEM((7, HD // 128, HD // 2, 128), u32),
            pltpu.VMEM((7, HD // 128, HD // 2, 128), u32),
            pltpu.VMEM((n_chunks, 7, HD // 128, HT // 2, 128), u32),
            pltpu.VMEM((7, HD // 128, HT // 2, 128), u32),
            pltpu.VMEM((H // 2, TS // 128, 64, 128), u32),
            pltpu.VMEM((H // 2, 80, 128), f32),
            pltpu.VMEM((H // 2, 80, 128), bf16),
            pltpu.VMEM((n_chunks, 4, 8, 128), f32),
            pltpu.VMEM((n_chunks, 4, 8, 128), i32),
            pltpu.VMEM((S, 128), f32),
            pltpu.VMEM((n_chunks, 2, 2, HT, HD), bf16),
            pltpu.VMEM((16, D), bf16),
            pltpu.VMEM((D, 128), f32),
            pltpu.VMEM((FS, 128), f32),
            pltpu.VMEM((8, D), f32),
            pltpu.SemaphoreType.DMA((5,)),
            pltpu.SemaphoreType.DMA((3, D // 128)),
            pltpu.SemaphoreType.DMA((4 + 3 * n_chunks,)),
            pltpu.SemaphoreType.DMA((2,)),
        ],
        compiler_params=pltpu.CompilerParams(vmem_limit_bytes=110 * 1024 * 1024),
        name="gated_mix_hedgehog_mod",
    )(A_x.reshape(S, D), A_wqkv, A_w_phi.reshape(H * Dh, Dh), A_wo, B_w_r.reshape(8, 128),
      B_w_gate, B_w_up, B_w_down, gate_w.reshape(8, 128))
    return out.reshape(B, S, D)
```

```python
import functools

import jax
import jax.numpy as jnp
from jax import lax
import jax.experimental.pallas as pl
import jax.experimental.pallas.tpu as pltpu

TS = 512
LOG2E = 1.4426950408889634
RATE0 = 1.8
KS = 2
RATE = 1.3

_NT = (((1,), (1,)), ((), ()))
_NN = (((1,), (0,)), ((), ()))

f32 = jnp.float32
bf16 = jnp.bfloat16
i32 = jnp.int32
u32 = jnp.uint32


def _pack(even, odd):
    return pltpu.pack_elementwise([even, odd], packed_dtype=bf16)


def _unpack(words):
    return [pltpu.unpack_elementwise(words, index=p, packed_dtype=bf16, unpacked_dtype=f32)
            for p in range(2)]


def _dot(a, b, dims):
    a, b = (pltpu.bitcast(v, bf16) if v.dtype == u32 else v for v in (a, b))
    return lax.dot_general(a, b, dims, preferred_element_type=f32)


def _tree(op, xs):
    xs = list(xs)
    while len(xs) > 1:
        nxt = [op(xs[i], xs[i + 1]) for i in range(0, len(xs) - 1, 2)]
        if len(xs) % 2:
            nxt.append(xs[-1])
        xs = nxt
    return xs[0]


def _recip(x):
    return pl.reciprocal(x, full_range=False)


def _sigmoid(x):
    return 0.5 + 0.5 * jnp.tanh(0.5 * x)


def _head_reduce(op, tiles):
    r = _tree(op, tiles)
    r = op(r, pltpu.roll(r, 4, 0))
    return op(r, pltpu.roll(r, 2, 0))


def _phi(p, hold):
    tiles = [p[8 * j:8 * j + 8] for j in range(8)]
    out = []
    for op, diff in ((jnp.maximum, lambda t, m: t - m), (jnp.minimum, lambda t, m: m - t)):
        m = hold(_head_reduce(op, tiles))
        e = [jnp.exp2(diff(t, m)) for t in tiles]
        r = _recip(_head_reduce(jnp.add, e))
        out += [_pack(e[j] * r, e[j + 1] * r) for j in range(0, 8, 2)]
    return jnp.concatenate(out, axis=0)


def _lane_bcast_rows(row):
    return jnp.broadcast_to(row, (128, row.shape[1])).T


def _lhs_terms(a11, a12, a21, a22):
    return (a11 + a22, a21 + a22, a11, a22, a11 + a12, a21 - a11, a12 - a22)


def _rhs_terms(b11, b12, b21, b22):
    return (b11 + b22, b11, b12 - b22, b21 - b11, b22, b11 + b12, b21 + b22)


def _put_terms(dst, m, terms_fn, load):
    rows = pl.ds(8 * m, 8)
    for k in range(dst.shape[1]):
        quads = [load(i, j, k) for i in range(2) for j in range(2)]
        even, odd = (terms_fn(*[q[p] for q in quads]) for p in range(2))
        for n in range(7):
            dst[n, k, rows, :] = _pack(even[n], odd[n])
    return dst[dst.shape[0] - 1, dst.shape[1] - 1, rows, :]


def _get(ref):
    return jnp.concatenate([ref[k] for k in range(ref.shape[0])], axis=1)


class _Pacer:
    def __init__(self, zero):
        self.zero = zero
        self.previous = None
        self.tick = 0
        self.rate = RATE
        self.queues = ([], [])

    def add(self, tag, cost, pieces, urgent=False):
        self.queues[0 if urgent else 1].extend(
            (tag, cost, max(self.tick + urgent, 1), p) for p in pieces)

    def flush(self, tag):
        for queue in self.queues:
            for item in [q for q in queue if q[0] == tag]:
                queue[:] = [q for q in queue if q is not item]
                item[3](lambda v: v)

    def _take(self, budget):
        taken = ([], [])
        for queue, out in zip(self.queues, taken):
            while queue and queue[0][2] <= self.tick and budget >= queue[0][1] / 2:
                budget -= queue[0][1]
                out.append(queue.pop(0)[3])
        return taken

    def _hold(self, where):
        rows = self.previous.shape[0] // 8
        start = pltpu.bitcast(self.previous[int(where * rows) * 8:][:8], u32) & self.zero
        return lambda v: pltpu.bitcast(pltpu.bitcast(v, u32) | start, v.dtype)

    def dot(self, lhs, rhs, dims):
        n = rhs.shape[0] // 64 if dims == _NT else rhs.shape[1] // 128
        out = []
        for j in range(n):
            marks = {}
            urgent, chain = self._take(self.rate * lhs.shape[0] * lhs.shape[1] / 256)
            for pieces, shift in ((urgent, 0.0), (chain, 0.5)):
                for m, piece in enumerate(pieces):
                    where = (m + shift) / len(pieces)
                    done = piece(self._hold(where))
                    if done and (pieces is urgent or m == len(pieces) - 1):
                        marks.setdefault(int(where * lhs.shape[0] / 8) * 8, []).extend(done)
            parts, at = [], 0
            for row, done in sorted(marks.items()):
                bits = _tree(jnp.bitwise_or, [pltpu.bitcast(v, u32) for v in done]) & self.zero
                parts += [lhs[at:row]] if row > at else []
                parts.append(jnp.concatenate(
                    [lhs[row:row + 8, 0:128] | bits, lhs[row:row + 8, 128:]], axis=1))
                at = row + 8
            a = jnp.concatenate(parts + ([lhs[at:]] if at < lhs.shape[0] else []), axis=0)
            out.append(_dot(a, rhs[64 * j:64 * j + 64] if dims == _NT else
                            rhs[:, 128 * j:128 * j + 128], dims))
            self.previous = out[-1]
            self.tick += 1
        return jnp.concatenate(out, axis=1)


def _kernel(x_hbm, wqkv_hbm, wphi_hbm, wo_hbm, wr_hbm, wg_hbm, wu_hbm, wd_hbm, gw_hbm,
            out_hbm,
            x_v, wqkv_v, wphi_v, wr_v, gw_v, wo_v, wg_v, wu_v, wd_v, wrg_v, fold_v, phi_t, x0_v, wv_t, kv_s, q_s,
            wo_s, x_s, xn_s, phi_s, kv_acc, kv_t, rmax_v, rarg_v, g_v, out_v, row_v, xcol_v, hcol_v, y_v,
            sem_x, sem_w, sem_s, sem_o):
    S, D = x_v.shape
    F = wd_hbm.shape[0]
    n_chunks = S // TS
    n_pairs = D // 64
    FS = hcol_v.shape[0]
    HD, HT = D // 2, TS // 2
    n_wb = HD // 128
    HP = n_pairs // 2

    def x_copy(h0, h1):
        rows = pl.ds(h0 * HT, (h1 - h0) * HT)
        return pltpu.make_async_copy(x_hbm.at[rows], x_v.at[rows], sem_x.at[h0])

    def w_copies(j, b):
        return [pltpu.make_async_copy(wqkv_hbm.at[:, pl.ds(j * D + g * 128, 128)],
                                      wqkv_v.at[j, g], sem_w.at[j, g]) for g in (b, b + n_wb)]

    whole = [pltpu.make_async_copy(src, dst, sem_s.at[n]) for n, (src, dst) in enumerate(
        [(wphi_hbm, wphi_v), (wr_hbm, wr_v), (gw_hbm, gw_v), (wo_hbm, wo_v)]
        + [pair for i in range(n_chunks) for pair in (
            (wg_hbm.at[:, pl.ds(i * FS, FS)], wg_v.at[i]),
            (wu_hbm.at[:, pl.ds(i * FS, FS)], wu_v.at[i]),
            (wd_hbm.at[pl.ds(i * FS, FS)], wd_v.at[i]))])]

    def start(copies):
        for cp in copies:
            cp.start()

    def wait(copies):
        for cp in copies:
            cp.wait()

    start(whole[0:1] + w_copies(1, 0) + [x_copy(0, 1)] + whole[1:3])

    c_i = lax.broadcasted_iota(i32, (128, 32), 0)
    f_i = lax.broadcasted_iota(i32, (128, 32), 1)
    sel = jnp.where(8 * (c_i // 16 % 4) + c_i % 8 == f_i, 1.0, 0.0).astype(bf16)
    r_i = lax.broadcasted_iota(i32, (128, 128), 0)
    l_i = lax.broadcasted_iota(i32, (128, 128), 1)
    same_head = (2 * (r_i // 64) + r_i // 8 % 2) == (l_i // 32)

    def fold(j, b, dst, tag):
        for i in range(2):
            g = b + i * n_wb
            fold_v[j, b, i] = _dot(phi_t[g], pltpu.bitcast(wqkv_v[j, g], u32), _NT) * LOG2E
        pacer.add(tag, 70, [lambda hold, m=m: [_put_terms(
            dst, 8 * b + m, _lhs_terms, lambda i, jj, k: [hold(fold_v[
                j, b, i, 16 * m + 8 * p:16 * m + 8 * p + 8, jj * HD + 128 * k:jj * HD + 128 * k + 128])
                for p in range(2)])] for m in range(8)])

    def prep_x(c, dst, m, best, hold):
        first = [pl.multiple_of(c * TS + t * HT + 16 * m, 16) for t in range(2)]
        dots = {}

        def load(i, j, k):
            col = i * n_wb + k
            xt = _unpack(hold(pltpu.bitcast(x_v[pl.ds(first[j], 16), 128 * col:128 * col + 128], u32)))
            for p in range(2):
                for name, w in (("r", wrg_v[0, col]), ("g", wrg_v[1, col])):
                    v = xt[p] * w
                    dots[name, j, p] = v + dots[name, j, p] if (name, j, p) in dots else v
            return xt

        done = [_put_terms(dst, m, _rhs_terms, load)]
        for t in range(2):
            for p in range(2):
                g = jnp.broadcast_to(jnp.sum(dots["g", t, p], axis=1, keepdims=True), (8, 128))
                g = _sigmoid(g)
                g_v[pl.ds(first[t] + p, 8, stride=2), :] = g
                r = jnp.broadcast_to(jnp.sum(dots["r", t, p], axis=1, keepdims=True), (8, 128))
                r = r.astype(bf16).astype(f32)
                tok = first[t] + p + 2 * lax.broadcasted_iota(i32, (8, 128), 0)
                if m:
                    better = r > best[t, p][0]
                    r = jnp.where(better, r, best[t, p][0])
                    tok = jnp.where(better, tok, best[t, p][1])
                best[t, p] = (r, tok)
                done += [g, tok]
                if m == HT // 16 - 1:
                    rmax_v[c, 2 * t + p], rarg_v[c, 2 * t + p] = r, tok
        return done

    def prep_wo(m, hold):
        r0 = pl.multiple_of(16 * m, 16)
        return [_put_terms(wo_s, m, _rhs_terms, lambda i, j, k: _unpack(hold(pltpu.bitcast(
            wo_v[pl.ds(i * HD + r0, 16), j * HD + 128 * k:j * HD + 128 * k + 128], u32))))]

    def prep_v(b):
        halves = [pltpu.bitcast(wqkv_v[2, g].T, u32) for g in (b, b + n_wb)]
        for k in range(D // 128):
            for g, half in zip((b, b + n_wb), halves):
                wv_t[k, 64 * g:64 * g + 64, :] = half[:, 128 * k:128 * k + 128]
        return [lambda hold, m=m: [_put_terms(
            kv_s, (HD + 128 * b) // 16 + m, _lhs_terms, lambda i, j, k: _unpack(hold(
                wv_t[j * n_wb + k, 64 * (b + i * n_wb) + 8 * m:64 * (b + i * n_wb) + 8 * m + 8, :])))]
            for m in range(8)]

    def put_phi(p, j, logits, hold):
        phi_s[p, j] = _phi(logits, hold)
        return [phi_s[p, j, 56:64, :]]

    def features(pacer, tag, pairs, j0, res):
        pacer.add(tag, 100, [lambda hold, q=q, p=p, j=j: put_phi(
            p, j0 + j, res[64 * q:64 * q + 64, 128 * j:128 * j + 128], hold)
            for q, p in enumerate(pairs) for j in range(res.shape[1] // 128)], urgent=True)

    def with_ones(vt):
        return jnp.concatenate([vt, jnp.ones((16, vt.shape[1]), f32)], axis=0).astype(bf16)

    wait(whole[0:1])
    bits = jnp.concatenate([pltpu.bitcast(wphi_v[0:16, :], u32)] * 4, axis=1)
    zero = (bits & 1) * ((bits + 1) & 1)
    pacer = _Pacer(zero)
    for g in range(D // 128):
        spread = _dot(sel, wphi_v[128 * g:128 * g + 128, :], _NT)
        phi_t[g] = pltpu.bitcast(jnp.where(same_head, spread, 0.0).astype(bf16), u32)
    rmax_v[...] = jnp.full(rmax_v.shape, -jnp.inf, f32)
    rarg_v[...] = jnp.zeros(rarg_v.shape, i32)

    def stage_x(t):
        for k in range(D // 128):
            x0_v[k, t * HT // 2:(t + 1) * HT // 2, :] = pltpu.bitcast(
                x_v[t * HT:(t + 1) * HT, 128 * k:128 * k + 128], u32)

    def k_block(b, t0, t1):
        lhs = jnp.concatenate([_pack(fold_v[1, b, i, r:r + 8, :], fold_v[1, b, i, r + 8:r + 16, :])
                               for i in range(2) for r in range(0, 128, 16)], axis=0)
        pk = pacer.dot(lhs, _get(x0_v.at[:, t0 * HT // 2:t1 * HT // 2]), _NT)
        features(pacer, "k", [2 * b, 2 * b + 1, HP + 2 * b, HP + 2 * b + 1], 2 * t0, pk)

    def v_block(b):
        lhs = jnp.concatenate([wv_t[k, 128 * b:128 * b + 128, :] for k in range(D // 128)], axis=1)
        vt = pacer.dot(lhs, _get(x0_v), _NT)
        pacer.flush("k")
        for q in range(4):
            kv_acc[4 * b + q] = _dot(with_ones(vt[64 * q:64 * q + 64]), _get(phi_s.at[4 * b + q]), _NT)

    def queue_x(pacer, c, dst):
        best = {}
        pacer.add("x", 280, [lambda hold, m=m: prep_x(c, dst, m, best, hold) for m in range(HT // 16)])

    strips = lambda j, b0, b1: [cp for b in range(b0, b1) for cp in w_copies(j, b)]
    wait(strips(1, 0, 1))
    start(strips(1, 1, 2))
    fold(1, 0, kv_s, "kv")
    wait([x_copy(0, 1)])
    start([x_copy(1, 2)])
    stage_x(0)
    k_block(0, 0, 1)
    wait(strips(1, 1, 2))
    start(strips(1, 2, 4))
    fold(1, 1, kv_s, "kv")
    k_block(1, 0, 1)
    wait([x_copy(1, 2)] + strips(1, 2, 3))
    start(strips(2, 0, 4))
    stage_x(1)
    k_block(0, 1, 2)
    fold(1, 2, kv_s, "kv")
    k_block(1, 1, 2)
    wait(strips(1, 3, 4))
    fold(1, 3, kv_s, "kv")
    k_block(2, 0, 2)
    wait(strips(2, 0, 4) + whole[1:3])
    start(strips(0, 0, 4) + [x_copy(2, 4)])
    for n, w in enumerate((wr_v, gw_v)):
        w = w[...].astype(f32)
        for col in range(D // 128):
            wrg_v[n, col] = jnp.broadcast_to(w[col:col + 1], (8, 128))
    pacer.add("kv", 90, prep_v(0) + prep_v(1))
    k_block(3, 0, 2)
    pacer.add("kv", 90, prep_v(2) + prep_v(3))
    v_block(0)
    v_block(2)
    pacer.flush("kv")
    wait(strips(0, 0, 4) + [x_copy(2, 4)])
    start([x_copy(4, 8)] + whole[3:4])
    for b in range(n_wb):
        fold(0, b, q_s, "q")
    queue_x(pacer, 1, x_s.at[1])
    pacer.rate = RATE0
    v_block(1)
    v_block(3)
    for tag in ("kv", "x", "q"):
        pacer.flush(tag)
    wait([x_copy(4, 8)] + whole[3:4])
    start(whole[4:])

    def project(pacer, lhs_s, c, finish):
        product = lambda n: pacer.dot(_get(lhs_s.at[n]), _get(x_s.at[c, n]), _NT)
        m3 = product(2)
        m5 = product(4)
        s12 = finish(0, 1, m3 + m5)
        m4 = product(3)
        t = m4 - m5
        m2 = product(1)
        s12()
        s21 = finish(1, 0, m2 + m4)
        u = m3 - m2
        m1 = product(0)
        t = t + m1
        u = u + m1
        m7 = product(6)
        s21()
        s11 = finish(0, 0, t + m7)
        m6 = product(5)
        return s11, finish(1, 1, u + m6)

    def phase1(c, _):
        pacer = _Pacer(zero)
        nxt = jnp.where(c + 1 < n_chunks, c + 1, 0)
        wo_per = pl.cdiv(HD // 16, n_chunks - 1)
        queue_x(pacer, nxt, xn_s)
        pacer.add("wo", 120, [lambda hold, j=j: prep_wo(
            jnp.minimum((c - 1) * wo_per + j, HD // 16 - 1), hold) for j in range(wo_per)])
        kr = lax.broadcasted_iota(i32, (80, 128), 0)
        kl = lax.broadcasted_iota(i32, (80, 128), 1)
        keep = jnp.where(kr < 64, kr // 32, (kr - 64) // 8) == kl // 2 % 2

        def kv_finish(half, t, res):
            features(pacer, (half, t), range(half * HP, half * HP + HP), 2 * t, res)

            def update():
                pacer.flush((half, t))
                for q in range(HP):
                    p = half * HP + q
                    acc = kv_acc[p] + _dot(with_ones(res[HD + 64 * q:HD + 64 * q + 64]),
                                           _get(phi_s.at[p, 2 * t:2 * t + 2]), _NT)
                    kv_acc[p] = acc
                    if half == t:
                        kv_t[p] = jnp.where(keep, acc, 0.0).astype(bf16)
            return update

        s11, s22 = project(pacer, kv_s, c, kv_finish)
        pacer.flush("x")
        x_s[nxt] = xn_s[...]

        r = rmax_v[...].reshape(n_chunks * 32, 128)
        tok = rarg_v[...].reshape(n_chunks * 32, 128)
        r_max = jnp.max(r, axis=0, keepdims=True)
        idx = jnp.min(jnp.where(r == r_max, tok, S - 1))
        rows = x_v[pl.ds(pl.multiple_of((idx // 16) * 16, 16), 16), :].astype(f32)
        is_sel = lax.broadcasted_iota(i32, (16, D), 0) == idx % 16
        xcol_v[...] = _lane_bcast_rows(jnp.sum(jnp.where(is_sel, rows, 0.0), axis=0, keepdims=True))
        s11()
        s22()
        pacer.flush("wo")
        return idx, r_max

    idx, r_max = lax.fori_loop(1, n_chunks, phase1, (jnp.int32(0), jnp.zeros((1, 128), f32)))
    y_v[...] = jnp.zeros(y_v.shape, f32)
    routed = idx // TS
    wait(whole[4:])

    def chunk_of(i):
        c = routed + i
        return jnp.where(c >= n_chunks, c - n_chunks, c)

    def out_copy(i, t, h):
        return pltpu.make_async_copy(
            out_v.at[i, t, h],
            out_hbm.at[pl.ds(chunk_of(i) * TS + t * HT, HT), pl.ds(h * HD, HD)],
            sem_o.at[jnp.minimum(i, 1)])

    def phase2(i, _):
        pacer = _Pacer(zero)
        c = chunk_of(i)

        def mat_vec(acc, col_ref, blocks, k0, hold):
            for k in range(k0, k0 + KS):
                col = hold(col_ref[8 * k:8 * k + 8, :])
                for a, block in enumerate(blocks):
                    n = block.shape[1] // 128
                    for j0 in range(0, n, 2):
                        j1 = min(j0 + 2, n)
                        w = block[8 * k:8 * k + 8, 128 * j0:128 * j1].astype(f32)
                        for j in range(j0, j1):
                            p = w[:, 128 * (j - j0):128 * (j - j0) + 128] * col
                            acc[a * n + j] = p if acc[a * n + j] is None else acc[a * n + j] + p
            return list(acc)

        def hidden(hold):
            gate, up = (jnp.sum(jnp.concatenate(v, axis=1), axis=0, keepdims=True)
                        for v in (gu[:FS // 128], gu[FS // 128:]))
            hcol_v[...] = _lane_bcast_rows(gate * _sigmoid(gate) * up)
            return [hcol_v[FS - 8:FS, :]]

        gu = [None] * (2 * FS // 128)
        y = [y_v[:, 128 * j:128 * j + 128] for j in range(D // 128)]
        pacer.add("ffn", KS * 43, [lambda hold, k=k: mat_vec(gu, xcol_v, (wg_v.at[i], wu_v.at[i]), k, hold)
                                  for k in range(0, D // 8, KS)])
        pacer.add("ffn", 400, [hidden])
        pacer.add("ffn", KS * 25, [lambda hold, k=k: mat_vec(y, hcol_v, (wd_v.at[i],), k, hold)
                                  for k in range(0, FS // 8, KS)])
        o = {}

        def q_finish(half, t, res):
            features(pacer, (half, t), range(half * HP, half * HP + HP), 2 * t, res)

            def attend():
                pacer.flush((half, t))
                o_t = []
                for p in range(half * HP, half * HP + HP):
                    nd = _dot(kv_t[p], _get(phi_s.at[p, 2 * t:2 * t + 2]), _NN)
                    for h in range(2):
                        inv = _recip(nd[64 + 8 * h:72 + 8 * h] + 1e-6)
                        o_t += [nd[32 * h + 8 * j:32 * h + 8 * j + 8] * inv for j in range(4)]
                o[t, half] = jnp.concatenate(o_t, axis=0)
            return attend

        def o_product(n, o_t):
            return pacer.dot(pltpu.bitcast(o_t.astype(bf16).T, u32), _get(wo_s.at[n]), _NN)

        def mix(t, h, a):
            def piece(m, hold):
                rows = pl.ds(pl.multiple_of(c * TS + t * HT + 16 * m, 16), 16)
                g = g_v[rows, :]
                g = jnp.concatenate([hold(g[:8]), hold(g[8:])], axis=0)
                for k in range(HD // 128):
                    xb = x_v[rows, h * HD + 128 * k:h * HD + 128 * k + 128].astype(f32)
                    out_v[i, t, h, 16 * m:16 * m + 16, 128 * k:128 * k + 128] = (
                        g * a[16 * m:16 * m + 16, 128 * k:128 * k + 128] + (1.0 - g) * xb).astype(bf16)
                return [out_v[i, t, h, 16 * m:16 * m + 16, HD - 128:HD]]

            pacer.add(("mix", t, h), 60, [functools.partial(piece, m) for m in range(HT // 16)], True)

            def send():
                pacer.flush(("mix", t, h))
                out_copy(i, t, h).start()
            return send

        s11, s22 = project(pacer, q_s, c, q_finish)
        m3 = o_product(2, o[1, 0])
        s11()
        m4 = o_product(3, o[0, 1])
        m1 = o_product(0, o[1, 0] + o[0, 1])
        s22()
        t = m1 + m4
        u = m1 + m3
        m2 = o_product(1, o[0, 0] + o[0, 1])
        send = mix(0, 0, m2 + m4)
        u = u - m2
        m6 = o_product(5, o[0, 0] - o[1, 0])
        send()
        send = mix(0, 1, u + m6)
        m5 = o_product(4, o[1, 0] + o[1, 1])
        send()
        send = mix(1, 1, m3 + m5)
        t = t - m5
        m7 = o_product(6, o[1, 1] - o[0, 1])
        send()
        mix(1, 0, t + m7)()
        pacer.flush("ffn")
        y_v[...] = jnp.concatenate(y, axis=1)
        return 0

    lax.fori_loop(0, n_chunks, phase2, 0)

    pacer.flush("ffn")
    sent = lambda rows, n: pltpu.make_async_copy(out_v.at[rows], out_v.at[rows], sem_o.at[n])
    sent(slice(0, 1), 0).wait()
    idx16 = pl.multiple_of((idx // 16) * 16, 16)
    t_sel = idx % TS // HT
    rows = pl.ds(pl.multiple_of(idx16 % HT, 16), 16)
    staged = jnp.concatenate([out_v[0, t_sel, h, rows, :] for h in range(2)], axis=1).astype(f32)
    g = jnp.concatenate([g_v[pl.ds(idx16, 16), :]] * (D // 128), axis=1)
    y = jnp.sum(y_v[...], axis=0, keepdims=True) * _sigmoid(r_max[:, 0:1])
    is_sel = lax.broadcasted_iota(i32, (16, D), 0) == idx % 16
    row_v[...] = (staged + jnp.where(is_sel, (1.0 - g) * y, 0.0)).astype(bf16)
    row_copy = pltpu.make_async_copy(row_v, out_hbm.at[pl.ds(idx16, 16)], sem_o.at[0])
    row_copy.start()
    sent(slice(1, n_chunks), 1).wait()
    row_copy.wait()


@jax.jit
def pallas_gated_mix__linear_kernel_hedgehog__moe_arch_mod__prompt_kernel(
    A_x: jax.Array,
    A_wqkv: jax.Array,
    A_w_phi: jax.Array,
    A_wo: jax.Array,
    B_x: jax.Array,
    B_w_r: jax.Array,
    B_w_gate: jax.Array,
    B_w_up: jax.Array,
    B_w_down: jax.Array,
    gate_w: jax.Array,
):
    del B_x
    B, S, D = A_x.shape
    H, Dh, _ = A_w_phi.shape
    F = B_w_gate.shape[1]
    n_chunks = S // TS
    FS = F // n_chunks
    HD, HT = D // 2, TS // 2
    assert B == 1 and Dh == 32 and D == 1024 and H * Dh == D and S == 4 * TS and FS % 128 == 0

    hbm = pl.BlockSpec(memory_space=pl.ANY)
    out = pl.pallas_call(
        _kernel,
        out_shape=jax.ShapeDtypeStruct((S, D), A_x.dtype),
        in_specs=[hbm] * 9,
        out_specs=hbm,
        scratch_shapes=[
            pltpu.VMEM((S, D), bf16),
            pltpu.VMEM((3, D // 128, D, 128), bf16),
            pltpu.VMEM((H * Dh, Dh), bf16),
            pltpu.VMEM((8, 128), bf16),
            pltpu.VMEM((8, 128), bf16),
            pltpu.VMEM((D, D), bf16),
            pltpu.VMEM((n_chunks, D, FS), bf16),
            pltpu.VMEM((n_chunks, D, FS), bf16),
            pltpu.VMEM((n_chunks, FS, D), bf16),
            pltpu.VMEM((2, D // 128, 8, 128), f32),
            pltpu.VMEM((2, HD // 128, 2, 128, D), f32),
            pltpu.VMEM((D // 128, 64, 128), u32),
            pltpu.VMEM((D // 128, TS // 2, 128), u32),
            pltpu.VMEM((D // 128, D // 2, 128), u32),
            pltpu.VMEM((7, HD // 128, D // 2, 128), u32),
            pltpu.VMEM((7, HD // 128, HD // 2, 128), u32),
            pltpu.VMEM((7, HD // 128, HD // 2, 128), u32),
            pltpu.VMEM((n_chunks, 7, HD // 128, HT // 2, 128), u32),
            pltpu.VMEM((7, HD // 128, HT // 2, 128), u32),
            pltpu.VMEM((H // 2, TS // 128, 64, 128), u32),
            pltpu.VMEM((H // 2, 80, 128), f32),
            pltpu.VMEM((H // 2, 80, 128), bf16),
            pltpu.VMEM((n_chunks, 4, 8, 128), f32),
            pltpu.VMEM((n_chunks, 4, 8, 128), i32),
            pltpu.VMEM((S, 128), f32),
            pltpu.VMEM((n_chunks, 2, 2, HT, HD), bf16),
            pltpu.VMEM((16, D), bf16),
            pltpu.VMEM((D, 128), f32),
            pltpu.VMEM((FS, 128), f32),
            pltpu.VMEM((8, D), f32),
            pltpu.SemaphoreType.DMA((5,)),
            pltpu.SemaphoreType.DMA((3, D // 128)),
            pltpu.SemaphoreType.DMA((4 + 3 * n_chunks,)),
            pltpu.SemaphoreType.DMA((2,)),
        ],
        compiler_params=pltpu.CompilerParams(vmem_limit_bytes=110 * 1024 * 1024),
        name="gated_mix_hedgehog_mod",
    )(A_x.reshape(S, D), A_wqkv, A_w_phi.reshape(H * Dh, Dh), A_wo, B_w_r.reshape(8, 128),
      B_w_gate, B_w_up, B_w_down, gate_w.reshape(8, 128))
    return out.reshape(B, S, D)
```

```python
import functools

import jax
import jax.numpy as jnp
from jax import lax
import jax.experimental.pallas as pl
import jax.experimental.pallas.tpu as pltpu

TS = 512
LOG2E = 1.4426950408889634
RATE0 = 1.1
RATE1 = 1.0
RATEK = 1.3
KS = 2
RATE = 1.3

_NT = (((1,), (1,)), ((), ()))
_NN = (((1,), (0,)), ((), ()))

f32 = jnp.float32
bf16 = jnp.bfloat16
i32 = jnp.int32
u32 = jnp.uint32


def _pack(even, odd):
    return pltpu.pack_elementwise([even, odd], packed_dtype=bf16)


def _unpack(words):
    return [pltpu.unpack_elementwise(words, index=p, packed_dtype=bf16, unpacked_dtype=f32)
            for p in range(2)]


def _dot(a, b, dims):
    a, b = (pltpu.bitcast(v, bf16) if v.dtype == u32 else v for v in (a, b))
    return lax.dot_general(a, b, dims, preferred_element_type=f32)


def _tree(op, xs):
    xs = list(xs)
    while len(xs) > 1:
        nxt = [op(xs[i], xs[i + 1]) for i in range(0, len(xs) - 1, 2)]
        if len(xs) % 2:
            nxt.append(xs[-1])
        xs = nxt
    return xs[0]


def _recip(x):
    return pl.reciprocal(x, full_range=False)


def _sigmoid(x):
    return 0.5 + 0.5 * jnp.tanh(0.5 * x)


def _head_reduce(op, tiles):
    r = _tree(op, tiles)
    r = op(r, pltpu.roll(r, 4, 0))
    return op(r, pltpu.roll(r, 2, 0))


def _phi(p, hold):
    tiles = [p[8 * j:8 * j + 8] for j in range(8)]
    out = []
    for op, diff in ((jnp.maximum, lambda t, m: t - m), (jnp.minimum, lambda t, m: m - t)):
        m = hold(_head_reduce(op, tiles))
        e = [jnp.exp2(diff(t, m)) for t in tiles]
        r = _recip(_head_reduce(jnp.add, e))
        out += [_pack(e[j] * r, e[j + 1] * r) for j in range(0, 8, 2)]
    return jnp.concatenate(out, axis=0)


def _lane_bcast_rows(row):
    return jnp.broadcast_to(row, (128, row.shape[1])).T


def _lhs_terms(a11, a12, a21, a22):
    return (a11 + a22, a21 + a22, a11, a22, a11 + a12, a21 - a11, a12 - a22)


def _rhs_terms(b11, b12, b21, b22):
    return (b11 + b22, b11, b12 - b22, b21 - b11, b22, b11 + b12, b21 + b22)


def _put_terms(dst, m, terms_fn, load):
    rows = pl.ds(8 * m, 8)
    for k in range(dst.shape[1]):
        quads = [load(i, j, k) for i in range(2) for j in range(2)]
        even, odd = (terms_fn(*[q[p] for q in quads]) for p in range(2))
        for n in range(7):
            dst[n, k, rows, :] = _pack(even[n], odd[n])
    return dst[dst.shape[0] - 1, dst.shape[1] - 1, rows, :]


def _get(ref):
    return jnp.concatenate([ref[k] for k in range(ref.shape[0])], axis=1)


class _Pacer:
    def __init__(self, zero):
        self.zero = zero
        self.previous = None
        self.tick = 0
        self.rate = RATE
        self.queues = ([], [])

    def add(self, tag, cost, pieces, urgent=False):
        self.queues[0 if urgent else 1].extend(
            (tag, cost, max(self.tick + urgent, 1), p) for p in pieces)

    def flush(self, tag):
        for queue in self.queues:
            for item in [q for q in queue if q[0] == tag]:
                queue[:] = [q for q in queue if q is not item]
                item[3](lambda v: v)

    def _take(self, budget):
        taken = ([], [])
        for queue, out in zip(self.queues, taken):
            while queue and queue[0][2] <= self.tick and budget >= queue[0][1] / 2:
                budget -= queue[0][1]
                out.append(queue.pop(0)[3])
        return taken

    def hold(self, where):
        rows = self.previous.shape[0] // 8
        start = pltpu.bitcast(self.previous[int(where * rows) * 8:][:8], u32) & self.zero
        return lambda v: pltpu.bitcast(pltpu.bitcast(v, u32) | start, v.dtype)

    def dot(self, lhs, rhs, dims):
        n = rhs.shape[0] // 64 if dims == _NT else rhs.shape[1] // 128
        out = []
        for j in range(n):
            marks = {}
            urgent, chain = self._take(self.rate * lhs.shape[0] * lhs.shape[1] / 256)
            for pieces, shift in ((urgent, 0.0), (chain, 0.5)):
                for m, piece in enumerate(pieces):
                    where = (m + shift) / len(pieces)
                    done = piece(self.hold(where))
                    if done and (pieces is urgent or m == len(pieces) - 1):
                        marks.setdefault(int(where * lhs.shape[0] / 8) * 8, []).extend(done)
            parts, at = [], 0
            for row, done in sorted(marks.items()):
                bits = _tree(jnp.bitwise_or, [pltpu.bitcast(v, u32) for v in done]) & self.zero
                parts += [lhs[at:row]] if row > at else []
                parts.append(jnp.concatenate(
                    [lhs[row:row + 8, 0:128] | bits, lhs[row:row + 8, 128:]], axis=1))
                at = row + 8
            a = jnp.concatenate(parts + ([lhs[at:]] if at < lhs.shape[0] else []), axis=0)
            out.append(_dot(a, rhs[64 * j:64 * j + 64] if dims == _NT else
                            rhs[:, 128 * j:128 * j + 128], dims))
            self.previous = out[-1]
            self.tick += 1
        return jnp.concatenate(out, axis=1)


def _kernel(x_hbm, wqkv_hbm, wphi_hbm, wo_hbm, wr_hbm, wg_hbm, wu_hbm, wd_hbm, gw_hbm,
            out_hbm,
            x_v, wqkv_v, wphi_v, wr_v, gw_v, wo_v, wg_v, wu_v, wd_v, wrg_v, fold_v, phi_t, x0_v, wv_t, kv_s, q_s,
            wo_s, x_s, phi_s, kv_acc, kv_t, rmax_v, rarg_v, g_v, out_v, row_v, xcol_v, hcol_v, y_v,
            sem_x, sem_w, sem_s, sem_o):
    S, D = x_v.shape
    F = wd_hbm.shape[0]
    n_chunks = S // TS
    n_pairs = D // 64
    FS = hcol_v.shape[0]
    HD, HT = D // 2, TS // 2
    n_wb = HD // 128
    HP = n_pairs // 2

    def x_copy(h0, h1):
        rows = pl.ds(h0 * HT, (h1 - h0) * HT)
        return pltpu.make_async_copy(x_hbm.at[rows], x_v.at[rows], sem_x.at[h0])

    def w_copies(j, b):
        return [pltpu.make_async_copy(wqkv_hbm.at[:, pl.ds(j * D + g * 128, 128)],
                                      wqkv_v.at[j, g], sem_w.at[j, g]) for g in (b, b + n_wb)]

    whole = [pltpu.make_async_copy(src, dst, sem_s.at[n]) for n, (src, dst) in enumerate(
        [(wphi_hbm, wphi_v), (wr_hbm, wr_v), (gw_hbm, gw_v), (wo_hbm, wo_v)]
        + [pair for i in range(n_chunks) for pair in (
            (wg_hbm.at[:, pl.ds(i * FS, FS)], wg_v.at[i]),
            (wu_hbm.at[:, pl.ds(i * FS, FS)], wu_v.at[i]),
            (wd_hbm.at[pl.ds(i * FS, FS)], wd_v.at[i]))])]

    def start(copies):
        for cp in copies:
            cp.start()

    def wait(copies):
        for cp in copies:
            cp.wait()

    start(whole[0:1] + w_copies(1, 0) + [x_copy(0, 1)] + whole[1:3])

    c_i = lax.broadcasted_iota(i32, (128, 32), 0)
    f_i = lax.broadcasted_iota(i32, (128, 32), 1)
    sel = jnp.where(8 * (c_i // 16 % 4) + c_i % 8 == f_i, 1.0, 0.0).astype(bf16)
    r_i = lax.broadcasted_iota(i32, (128, 128), 0)
    l_i = lax.broadcasted_iota(i32, (128, 128), 1)
    same_head = (2 * (r_i // 64) + r_i // 8 % 2) == (l_i // 32)

    def fold(j, b):
        for i in range(2):
            g = b + i * n_wb
            fold_v[j, i, 128 * b:128 * b + 128, :] = _dot(
                phi_t[g], pltpu.bitcast(wqkv_v[j, g], u32), _NT) * LOG2E

    def prep_folded(j, dst, m, hold):
        r0 = pl.multiple_of(16 * m, 16)
        return [_put_terms(dst, m, _lhs_terms, lambda i, jj, k: [hold(fold_v[
            j, i, pl.ds(r0 + 8 * p, 8), jj * HD + 128 * k:jj * HD + 128 * k + 128]) for p in range(2)])]

    def fold_k(b):
        fold(1, b)
        pacer.add("kv", 100, [functools.partial(prep_folded, 1, kv_s, 8 * b + m) for m in range(8)])

    def prep_x(c, terms, m, best, hold):
        first = [pl.multiple_of(c * TS + t * HT + 16 * m, 16) for t in range(2)]
        dots, done = {}, []
        for k in range(n_wb):
            words, quads = [], []
            for col in (k, n_wb + k):
                for t in range(2):
                    words.append(hold(pltpu.bitcast(
                        x_v[pl.ds(first[t], 16), 128 * col:128 * col + 128], u32)))
                    quads.append(_unpack(words[-1]))
                    for p in range(2):
                        for n in range(2):
                            v = quads[-1][p] * wrg_v[n, col]
                            dots[n, t, p] = v + dots[n, t, p] if (n, t, p) in dots else v
            even, odd = (_rhs_terms(*[q[p] for q in quads]) for p in range(2))
            for n in range(7):
                terms[m, n, k] = {1: words[0], 4: words[3]}.get(n)
                if terms[m, n, k] is None:
                    terms[m, n, k] = _pack(even[n], odd[n])
                    done.append(terms[m, n, k])
        for t in range(2):
            for p in range(2):
                g = jnp.broadcast_to(jnp.sum(dots[1, t, p], axis=1, keepdims=True), (8, 128))
                g = _sigmoid(g)
                g_v[pl.ds(first[t] + p, 8, stride=2), :] = g
                r = jnp.broadcast_to(jnp.sum(dots[0, t, p], axis=1, keepdims=True), (8, 128))
                r = r.astype(bf16).astype(f32)
                tok = first[t] + p + 2 * lax.broadcasted_iota(i32, (8, 128), 0)
                if m:
                    better = r > best[t, p][0]
                    r = jnp.where(better, r, best[t, p][0])
                    tok = jnp.where(better, tok, best[t, p][1])
                best[t, p] = (r, tok)
                done += [g, tok]
                if m == HT // 16 - 1:
                    rmax_v[c, 2 * t + p], rarg_v[c, 2 * t + p] = r, tok
        return done

    def prep_wo(m, hold):
        r0 = pl.multiple_of(16 * m, 16)
        return [_put_terms(wo_s, m, _rhs_terms, lambda i, j, k: _unpack(hold(pltpu.bitcast(
            wo_v[pl.ds(i * HD + r0, 16), j * HD + 128 * k:j * HD + 128 * k + 128], u32))))]

    def prep_v(b):
        halves = [pltpu.bitcast(wqkv_v[2, g].T, u32) for g in (b, b + n_wb)]
        for k in range(D // 128):
            for g, half in zip((b, b + n_wb), halves):
                wv_t[k, 64 * g:64 * g + 64, :] = half[:, 128 * k:128 * k + 128]
        return [lambda hold, m=m: [_put_terms(
            kv_s, (HD + 128 * b) // 16 + m, _lhs_terms, lambda i, j, k: _unpack(hold(
                wv_t[j * n_wb + k, 64 * (b + i * n_wb) + 8 * m:64 * (b + i * n_wb) + 8 * m + 8, :])))]
            for m in range(8)]

    def put_phi(p, j, logits, hold):
        phi_s[p, j] = _phi(logits, hold)
        return [phi_s[p, j, 56:64, :]]

    def features(pacer, tag, pairs, j0, res):
        pacer.add(tag, 100, [lambda hold, q=q, p=p, j=j: put_phi(
            p, j0 + j, res[64 * q:64 * q + 64, 128 * j:128 * j + 128], hold)
            for q, p in enumerate(pairs) for j in range(res.shape[1] // 128)], urgent=True)

    def with_ones(vt):
        return jnp.concatenate([vt, jnp.ones((16, vt.shape[1]), f32)], axis=0).astype(bf16)

    wait(whole[0:1])
    bits = jnp.concatenate([pltpu.bitcast(wphi_v[0:16, :], u32)] * 4, axis=1)
    zero = (bits & 1) * ((bits + 1) & 1)
    pacer = _Pacer(zero)
    pacer.rate = RATEK
    for g in range(D // 128):
        spread = _dot(sel, wphi_v[128 * g:128 * g + 128, :], _NT)
        phi_t[g] = pltpu.bitcast(jnp.where(same_head, spread, 0.0).astype(bf16), u32)
    rmax_v[...] = jnp.full(rmax_v.shape, -jnp.inf, f32)
    rarg_v[...] = jnp.zeros(rarg_v.shape, i32)

    def stage_x(t):
        for k in range(D // 128):
            x0_v[k, t * HT // 2:(t + 1) * HT // 2, :] = pltpu.bitcast(
                x_v[t * HT:(t + 1) * HT, 128 * k:128 * k + 128], u32)

    def k_block(b, t0, t1):
        lhs = jnp.concatenate([_pack(fold_v[1, i, r:r + 8, :], fold_v[1, i, r + 8:r + 16, :])
                               for i in range(2) for r in range(128 * b, 128 * b + 128, 16)], axis=0)
        pk = pacer.dot(lhs, _get(x0_v.at[:, t0 * HT // 2:t1 * HT // 2]), _NT)
        features(pacer, "k", [2 * b, 2 * b + 1, HP + 2 * b, HP + 2 * b + 1], 2 * t0, pk)

    def v_block(b):
        lhs = jnp.concatenate([wv_t[k, 128 * b:128 * b + 128, :] for k in range(D // 128)], axis=1)
        vt = pacer.dot(lhs, _get(x0_v), _NT)
        pacer.flush("k")
        for q in range(4):
            kv_acc[4 * b + q] = _dot(with_ones(vt[64 * q:64 * q + 64]), _get(phi_s.at[4 * b + q]), _NT)

    def put_x(c, terms, hold):
        for (m, n, k), term in sorted(terms.items(), key=lambda item: item[0]):
            x_s[c, n, k, 8 * m:8 * m + 8, :] = hold(m)(term)

    strips = lambda j, b0, b1: [cp for b in range(b0, b1) for cp in w_copies(j, b)]
    wait(strips(1, 0, 1))
    start(strips(1, 1, 2))
    fold_k(0)
    wait([x_copy(0, 1)])
    start([x_copy(1, 2)])
    stage_x(0)
    k_block(0, 0, 1)
    wait(strips(1, 1, 2))
    start(strips(1, 2, 4))
    fold_k(1)
    k_block(1, 0, 1)
    wait([x_copy(1, 2)] + strips(1, 2, 3))
    start(strips(2, 0, 4))
    stage_x(1)
    k_block(0, 1, 2)
    fold_k(2)
    k_block(1, 1, 2)
    wait(strips(1, 3, 4))
    fold_k(3)
    k_block(2, 0, 2)
    wait(strips(2, 0, 4) + whole[1:3])
    start(strips(0, 0, 4) + [x_copy(2, 4)])
    for n, w in enumerate((wr_v, gw_v)):
        w = w[...].astype(f32)
        for col in range(D // 128):
            wrg_v[n, col] = jnp.broadcast_to(w[col:col + 1], (8, 128))
    pacer.add("kv", 90, prep_v(0) + prep_v(1))
    k_block(3, 0, 2)
    pacer.add("kv", 90, prep_v(2) + prep_v(3))
    v_block(0)
    v_block(2)
    pacer.flush("kv")
    wait(strips(0, 0, 4) + [x_copy(2, 4)])
    start([x_copy(4, 8)] + whole[3:4])
    for b in range(n_wb):
        fold(0, b)
    best = {}

    def first_x(m, hold):
        terms = {}
        done = prep_x(1, terms, m, best, hold)
        put_x(1, terms, lambda m: lambda v: v)
        return done[-8:] + [x_s[1, 6, n_wb - 1, 8 * m:8 * m + 8, :]]

    pacer.add("x", 270, [functools.partial(first_x, m) for m in range(HT // 16)])
    pacer.rate = RATE0
    v_block(1)
    v_block(3)
    pacer.flush("x")
    wait([x_copy(4, 8)] + whole[3:4])
    start(whole[4:])

    def project(pacer, lhs_s, c, finish):
        product = lambda n: pacer.dot(_get(lhs_s.at[n]), _get(x_s.at[c, n]), _NT)
        m3 = product(2)
        m5 = product(4)
        s12 = finish(0, 1, m3 + m5)
        m4 = product(3)
        t = m4 - m5
        m2 = product(1)
        s12()
        s21 = finish(1, 0, m2 + m4)
        u = m3 - m2
        m1 = product(0)
        t = t + m1
        u = u + m1
        m7 = product(6)
        s21()
        s11 = finish(0, 0, t + m7)
        m6 = product(5)
        return s11, finish(1, 1, u + m6)

    def phase1(c, _):
        pacer = _Pacer(zero)
        pacer.rate = RATE1
        nxt = jnp.where(c + 1 < n_chunks, c + 1, 0)
        best, terms = {}, {}
        pacer.add("x", 290, [functools.partial(prep_x, nxt, terms, m, best) for m in range(HT // 16)])
        share = pl.cdiv(HD // 16, n_chunks - 1)
        for prep in (prep_wo, functools.partial(prep_folded, 0, q_s)):
            pacer.add("w", 120, [functools.partial(
                prep, jnp.minimum((c - 1) * share + j, HD // 16 - 1)) for j in range(share)])
        kr = lax.broadcasted_iota(i32, (80, 128), 0)
        kl = lax.broadcasted_iota(i32, (80, 128), 1)
        keep = jnp.where(kr < 64, kr // 32, (kr - 64) // 8) == kl // 2 % 2

        def kv_finish(half, t, res):
            features(pacer, (half, t), range(half * HP, half * HP + HP), 2 * t, res)

            def update():
                pacer.flush((half, t))
                for q in range(HP):
                    p = half * HP + q
                    acc = kv_acc[p] + _dot(with_ones(res[HD + 64 * q:HD + 64 * q + 64]),
                                           _get(phi_s.at[p, 2 * t:2 * t + 2]), _NT)
                    kv_acc[p] = acc
                    if half == t:
                        kv_t[p] = jnp.where(keep, acc, 0.0).astype(bf16)
            return update

        s11, s22 = project(pacer, kv_s, c, kv_finish)
        pacer.flush("x")
        put_x(nxt, terms, functools.cache(lambda m: pacer.hold(m / (HT // 16))))

        r = rmax_v[...].reshape(n_chunks * 32, 128)
        tok = rarg_v[...].reshape(n_chunks * 32, 128)
        r_max = jnp.max(r, axis=0, keepdims=True)
        idx = jnp.min(jnp.where(r == r_max, tok, S - 1))
        rows = x_v[pl.ds(pl.multiple_of((idx // 16) * 16, 16), 16), :].astype(f32)
        is_sel = lax.broadcasted_iota(i32, (16, D), 0) == idx % 16
        xcol_v[...] = _lane_bcast_rows(jnp.sum(jnp.where(is_sel, rows, 0.0), axis=0, keepdims=True))
        s11()
        s22()
        pacer.flush("w")
        return idx, r_max

    idx, r_max = lax.fori_loop(1, n_chunks, phase1, (jnp.int32(0), jnp.zeros((1, 128), f32)))
    y_v[...] = jnp.zeros(y_v.shape, f32)
    routed = idx // TS
    wait(whole[4:])

    def chunk_of(i):
        c = routed + i
        return jnp.where(c >= n_chunks, c - n_chunks, c)

    def out_copy(i, t, h):
        return pltpu.make_async_copy(
            out_v.at[i, t, h],
            out_hbm.at[pl.ds(chunk_of(i) * TS + t * HT, HT), pl.ds(h * HD, HD)],
            sem_o.at[jnp.minimum(i, 1)])

    def phase2(i, _):
        pacer = _Pacer(zero)
        c = chunk_of(i)

        def mat_vec(acc, col_ref, blocks, k0, hold):
            for k in range(k0, k0 + KS):
                col = hold(col_ref[8 * k:8 * k + 8, :])
                for a, block in enumerate(blocks):
                    n = block.shape[1] // 128
                    for j0 in range(0, n, 2):
                        j1 = min(j0 + 2, n)
                        w = block[8 * k:8 * k + 8, 128 * j0:128 * j1].astype(f32)
                        for j in range(j0, j1):
                            p = w[:, 128 * (j - j0):128 * (j - j0) + 128] * col
                            acc[a * n + j] = p if acc[a * n + j] is None else acc[a * n + j] + p
            return list(acc)

        def hidden(hold):
            gate, up = (jnp.sum(jnp.concatenate(v, axis=1), axis=0, keepdims=True)
                        for v in (gu[:FS // 128], gu[FS // 128:]))
            hcol_v[...] = _lane_bcast_rows(gate * _sigmoid(gate) * up)
            return [hcol_v[FS - 8:FS, :]]

        gu = [None] * (2 * FS // 128)
        y = [y_v[:, 128 * j:128 * j + 128] for j in range(D // 128)]
        pacer.add("ffn", KS * 43, [lambda hold, k=k: mat_vec(gu, xcol_v, (wg_v.at[i], wu_v.at[i]), k, hold)
                                  for k in range(0, D // 8, KS)])
        pacer.add("ffn", 400, [hidden])
        pacer.add("ffn", KS * 25, [lambda hold, k=k: mat_vec(y, hcol_v, (wd_v.at[i],), k, hold)
                                  for k in range(0, FS // 8, KS)])
        o = {}

        def q_finish(half, t, res):
            features(pacer, (half, t), range(half * HP, half * HP + HP), 2 * t, res)

            def attend():
                pacer.flush((half, t))
                o_t = []
                for p in range(half * HP, half * HP + HP):
                    nd = _dot(kv_t[p], _get(phi_s.at[p, 2 * t:2 * t + 2]), _NN)
                    for h in range(2):
                        inv = _recip(nd[64 + 8 * h:72 + 8 * h] + 1e-6)
                        o_t += [nd[32 * h + 8 * j:32 * h + 8 * j + 8] * inv for j in range(4)]
                o[t, half] = jnp.concatenate(o_t, axis=0)
            return attend

        def o_product(n, o_t):
            return pacer.dot(pltpu.bitcast(o_t.astype(bf16).T, u32), _get(wo_s.at[n]), _NN)

        def mix(t, h, a):
            def piece(m, hold):
                rows = pl.ds(pl.multiple_of(c * TS + t * HT + 16 * m, 16), 16)
                g = g_v[rows, :]
                g = jnp.concatenate([hold(g[:8]), hold(g[8:])], axis=0)
                for k in range(HD // 128):
                    xb = x_v[rows, h * HD + 128 * k:h * HD + 128 * k + 128].astype(f32)
                    out_v[i, t, h, 16 * m:16 * m + 16, 128 * k:128 * k + 128] = (
                        g * a[16 * m:16 * m + 16, 128 * k:128 * k + 128] + (1.0 - g) * xb).astype(bf16)
                return [out_v[i, t, h, 16 * m:16 * m + 16, HD - 128:HD]]

            pacer.add(("mix", t, h), 60, [functools.partial(piece, m) for m in range(HT // 16)], True)

            def send():
                pacer.flush(("mix", t, h))
                out_copy(i, t, h).start()
            return send

        s11, s22 = project(pacer, q_s, c, q_finish)
        m3 = o_product(2, o[1, 0])
        s11()
        m4 = o_product(3, o[0, 1])
        m1 = o_product(0, o[1, 0] + o[0, 1])
        s22()
        t = m1 + m4
        u = m1 + m3
        m2 = o_product(1, o[0, 0] + o[0, 1])
        send = mix(0, 0, m2 + m4)
        u = u - m2
        m6 = o_product(5, o[0, 0] - o[1, 0])
        send()
        send = mix(0, 1, u + m6)
        m5 = o_product(4, o[1, 0] + o[1, 1])
        send()
        send = mix(1, 1, m3 + m5)
        t = t - m5
        m7 = o_product(6, o[1, 1] - o[0, 1])
        send()
        mix(1, 0, t + m7)()
        pacer.flush("ffn")
        y_v[...] = jnp.concatenate(y, axis=1)
        return 0

    lax.fori_loop(0, n_chunks, phase2, 0)

    pacer.flush("ffn")
    sent = lambda rows, n: pltpu.make_async_copy(out_v.at[rows], out_v.at[rows], sem_o.at[n])
    sent(slice(0, 1), 0).wait()
    idx16 = pl.multiple_of((idx // 16) * 16, 16)
    t_sel = idx % TS // HT
    rows = pl.ds(pl.multiple_of(idx16 % HT, 16), 16)
    staged = jnp.concatenate([out_v[0, t_sel, h, rows, :] for h in range(2)], axis=1).astype(f32)
    g = jnp.concatenate([g_v[pl.ds(idx16, 16), :]] * (D // 128), axis=1)
    y = jnp.sum(y_v[...], axis=0, keepdims=True) * _sigmoid(r_max[:, 0:1])
    is_sel = lax.broadcasted_iota(i32, (16, D), 0) == idx % 16
    row_v[...] = (staged + jnp.where(is_sel, (1.0 - g) * y, 0.0)).astype(bf16)
    row_copy = pltpu.make_async_copy(row_v, out_hbm.at[pl.ds(idx16, 16)], sem_o.at[0])
    row_copy.start()
    sent(slice(1, n_chunks), 1).wait()
    row_copy.wait()


@jax.jit
def pallas_gated_mix__linear_kernel_hedgehog__moe_arch_mod__prompt_kernel(
    A_x: jax.Array,
    A_wqkv: jax.Array,
    A_w_phi: jax.Array,
    A_wo: jax.Array,
    B_x: jax.Array,
    B_w_r: jax.Array,
    B_w_gate: jax.Array,
    B_w_up: jax.Array,
    B_w_down: jax.Array,
    gate_w: jax.Array,
):
    del B_x
    B, S, D = A_x.shape
    H, Dh, _ = A_w_phi.shape
    F = B_w_gate.shape[1]
    n_chunks = S // TS
    FS = F // n_chunks
    HD, HT = D // 2, TS // 2
    assert B == 1 and Dh == 32 and D == 1024 and H * Dh == D and S == 4 * TS and FS % 128 == 0

    hbm = pl.BlockSpec(memory_space=pl.ANY)
    out = pl.pallas_call(
        _kernel,
        out_shape=jax.ShapeDtypeStruct((S, D), A_x.dtype),
        in_specs=[hbm] * 9,
        out_specs=hbm,
        scratch_shapes=[
            pltpu.VMEM((S, D), bf16),
            pltpu.VMEM((3, D // 128, D, 128), bf16),
            pltpu.VMEM((H * Dh, Dh), bf16),
            pltpu.VMEM((8, 128), bf16),
            pltpu.VMEM((8, 128), bf16),
            pltpu.VMEM((D, D), bf16),
            pltpu.VMEM((n_chunks, D, FS), bf16),
            pltpu.VMEM((n_chunks, D, FS), bf16),
            pltpu.VMEM((n_chunks, FS, D), bf16),
            pltpu.VMEM((2, D // 128, 8, 128), f32),
            pltpu.VMEM((2, 2, HD, D), f32),
            pltpu.VMEM((D // 128, 64, 128), u32),
            pltpu.VMEM((D // 128, TS // 2, 128), u32),
            pltpu.VMEM((D // 128, D // 2, 128), u32),
            pltpu.VMEM((7, HD // 128, D // 2, 128), u32),
            pltpu.VMEM((7, HD // 128, HD // 2, 128), u32),
            pltpu.VMEM((7, HD // 128, HD // 2, 128), u32),
            pltpu.VMEM((n_chunks, 7, HD // 128, HT // 2, 128), u32),
            pltpu.VMEM((H // 2, TS // 128, 64, 128), u32),
            pltpu.VMEM((H // 2, 80, 128), f32),
            pltpu.VMEM((H // 2, 80, 128), bf16),
            pltpu.VMEM((n_chunks, 4, 8, 128), f32),
            pltpu.VMEM((n_chunks, 4, 8, 128), i32),
            pltpu.VMEM((S, 128), f32),
            pltpu.VMEM((n_chunks, 2, 2, HT, HD), bf16),
            pltpu.VMEM((16, D), bf16),
            pltpu.VMEM((D, 128), f32),
            pltpu.VMEM((FS, 128), f32),
            pltpu.VMEM((8, D), f32),
            pltpu.SemaphoreType.DMA((5,)),
            pltpu.SemaphoreType.DMA((3, D // 128)),
            pltpu.SemaphoreType.DMA((4 + 3 * n_chunks,)),
            pltpu.SemaphoreType.DMA((2,)),
        ],
        compiler_params=pltpu.CompilerParams(vmem_limit_bytes=110 * 1024 * 1024),
        name="gated_mix_hedgehog_mod",
    )(A_x.reshape(S, D), A_wqkv, A_w_phi.reshape(H * Dh, Dh), A_wo, B_w_r.reshape(8, 128),
      B_w_gate, B_w_up, B_w_down, gate_w.reshape(8, 128))
    return out.reshape(B, S, D)
```

```python
import functools

import jax
import jax.numpy as jnp
from jax import lax
import jax.experimental.pallas as pl
import jax.experimental.pallas.tpu as pltpu

TS = 512
LOG2E = 1.4426950408889634
RATE0 = 1.1
RATE1 = 1.0
RATEK = 1.3
KS = 2
RATE = 1.35

_NT = (((1,), (1,)), ((), ()))
_NN = (((1,), (0,)), ((), ()))

f32 = jnp.float32
bf16 = jnp.bfloat16
i32 = jnp.int32
u32 = jnp.uint32


def _pack(even, odd):
    return pltpu.pack_elementwise([even, odd], packed_dtype=bf16)


def _unpack(words):
    return [pltpu.unpack_elementwise(words, index=p, packed_dtype=bf16, unpacked_dtype=f32)
            for p in range(2)]


def _dot(a, b, dims):
    a, b = (pltpu.bitcast(v, bf16) if v.dtype == u32 else v for v in (a, b))
    return lax.dot_general(a, b, dims, preferred_element_type=f32)


def _tree(op, xs):
    xs = list(xs)
    while len(xs) > 1:
        nxt = [op(xs[i], xs[i + 1]) for i in range(0, len(xs) - 1, 2)]
        if len(xs) % 2:
            nxt.append(xs[-1])
        xs = nxt
    return xs[0]


def _recip(x):
    return pl.reciprocal(x, full_range=False)


def _sigmoid(x):
    return 0.5 + 0.5 * jnp.tanh(0.5 * x)


def _head_reduce(op, tiles):
    r = _tree(op, tiles)
    r = op(r, pltpu.roll(r, 4, 0))
    return op(r, pltpu.roll(r, 2, 0))


def _phi(p, hold):
    tiles = [p[8 * j:8 * j + 8] for j in range(8)]
    out = []
    for op, diff in ((jnp.maximum, lambda t, m: t - m), (jnp.minimum, lambda t, m: m - t)):
        m = hold(_head_reduce(op, tiles))
        e = [jnp.exp2(diff(t, m)) for t in tiles]
        r = _recip(_head_reduce(jnp.add, e))
        out += [_pack(e[j] * r, e[j + 1] * r) for j in range(0, 8, 2)]
    return jnp.concatenate(out, axis=0)


def _lane_bcast_rows(row):
    return jnp.broadcast_to(row, (128, row.shape[1])).T


def _lhs_terms(a11, a12, a21, a22):
    return (a11 + a22, a21 + a22, a11, a22, a11 + a12, a21 - a11, a12 - a22)


def _rhs_terms(b11, b12, b21, b22):
    return (b11 + b22, b11, b12 - b22, b21 - b11, b22, b11 + b12, b21 + b22)


def _put_terms(dst, m, terms_fn, load):
    rows = pl.ds(8 * m, 8)
    for k in range(dst.shape[1]):
        quads = [load(i, j, k) for i in range(2) for j in range(2)]
        even, odd = (terms_fn(*[q[p] for q in quads]) for p in range(2))
        for n in range(7):
            dst[n, k, rows, :] = _pack(even[n], odd[n])
    return dst[dst.shape[0] - 1, dst.shape[1] - 1, rows, :]


def _get(ref):
    return jnp.concatenate([ref[k] for k in range(ref.shape[0])], axis=1)


class _Pacer:
    def __init__(self, zero):
        self.zero = zero
        self.previous = None
        self.tick = 0
        self.rate = RATE
        self.queues = ([], [])

    def add(self, tag, cost, pieces, urgent=False):
        self.queues[0 if urgent else 1].extend(
            (tag, cost, max(self.tick + urgent, 1), p) for p in pieces)

    def flush(self, tag, run=True):
        for queue in self.queues:
            for item in [q for q in queue if q[0] == tag]:
                queue[:] = [q for q in queue if q is not item]
                if run:
                    item[3](lambda v: v)

    def _take(self, budget):
        taken = ([], [])
        for queue, out in zip(self.queues, taken):
            while queue and queue[0][2] <= self.tick and budget >= queue[0][1] / 2:
                budget -= queue[0][1]
                out.append(queue.pop(0)[3])
        return taken

    def hold(self, where):
        rows = self.previous.shape[0] // 8
        start = pltpu.bitcast(self.previous[int(where * rows) * 8:][:8], u32) & self.zero
        return lambda v: pltpu.bitcast(pltpu.bitcast(v, u32) | start, v.dtype)

    def dot(self, lhs, rhs, dims):
        n = rhs.shape[0] // 64 if dims == _NT else rhs.shape[1] // 128
        out = []
        for j in range(n):
            marks = {}
            urgent, chain = self._take(self.rate * lhs.shape[0] * lhs.shape[1] / 256)
            for pieces, shift in ((urgent, 0.0), (chain, 0.5)):
                for m, piece in enumerate(pieces):
                    where = (m + shift) / len(pieces)
                    done = piece(self.hold(where))
                    if done and (pieces is urgent or m == len(pieces) - 1):
                        marks.setdefault(int(where * lhs.shape[0] / 8) * 8, []).extend(done)
            parts, at = [], 0
            for row, done in sorted(marks.items()):
                bits = _tree(jnp.bitwise_or, [pltpu.bitcast(v, u32) for v in done]) & self.zero
                parts += [lhs[at:row]] if row > at else []
                parts.append(jnp.concatenate(
                    [lhs[row:row + 8, 0:128] | bits, lhs[row:row + 8, 128:]], axis=1))
                at = row + 8
            a = jnp.concatenate(parts + ([lhs[at:]] if at < lhs.shape[0] else []), axis=0)
            out.append(_dot(a, rhs[64 * j:64 * j + 64] if dims == _NT else
                            rhs[:, 128 * j:128 * j + 128], dims))
            self.previous = out[-1]
            self.tick += 1
        return jnp.concatenate(out, axis=1)


def _kernel(x_hbm, wqkv_hbm, wphi_hbm, wo_hbm, wr_hbm, wg_hbm, wu_hbm, wd_hbm, gw_hbm,
            out_hbm,
            x_v, wqkv_v, wphi_v, wr_v, gw_v, wo_v, wg_v, wu_v, wd_v, wrg_v, fold_v, phi_t, x0_v, wv_t, kv_s, q_s,
            wo_s, x_s, phi_s, kv_acc, kv_t, rmax_v, rarg_v, g_v, out_v, row_v, xcol_v, hcol_v, y_v,
            sem_x, sem_w, sem_s, sem_o):
    S, D = x_v.shape
    F = wd_hbm.shape[0]
    n_chunks = S // TS
    n_pairs = D // 64
    FS = hcol_v.shape[0]
    HD, HT = D // 2, TS // 2
    n_wb = HD // 128
    HP = n_pairs // 2

    def x_copy(h0, h1):
        rows = pl.ds(h0 * HT, (h1 - h0) * HT)
        return pltpu.make_async_copy(x_hbm.at[rows], x_v.at[rows], sem_x.at[h0])

    def w_copies(j, b):
        return [pltpu.make_async_copy(wqkv_hbm.at[:, pl.ds(j * D + g * 128, 128)],
                                      wqkv_v.at[j, g], sem_w.at[j, g]) for g in (b, b + n_wb)]

    whole = [pltpu.make_async_copy(src, dst, sem_s.at[n]) for n, (src, dst) in enumerate(
        [(wphi_hbm, wphi_v), (wr_hbm, wr_v), (gw_hbm, gw_v), (wo_hbm, wo_v)]
        + [pair for i in range(n_chunks) for pair in (
            (wg_hbm.at[:, pl.ds(i * FS, FS)], wg_v.at[i]),
            (wu_hbm.at[:, pl.ds(i * FS, FS)], wu_v.at[i]),
            (wd_hbm.at[pl.ds(i * FS, FS)], wd_v.at[i]))])]

    def start(copies):
        for cp in copies:
            cp.start()

    def wait(copies):
        for cp in copies:
            cp.wait()

    start(whole[0:1] + w_copies(1, 0) + [x_copy(0, 1)] + whole[1:3])

    c_i = lax.broadcasted_iota(i32, (128, 32), 0)
    f_i = lax.broadcasted_iota(i32, (128, 32), 1)
    sel = jnp.where(8 * (c_i // 16 % 4) + c_i % 8 == f_i, 1.0, 0.0).astype(bf16)
    r_i = lax.broadcasted_iota(i32, (128, 128), 0)
    l_i = lax.broadcasted_iota(i32, (128, 128), 1)
    same_head = (2 * (r_i // 64) + r_i // 8 % 2) == (l_i // 32)

    def fold(j, b):
        for i in range(2):
            g = b + i * n_wb
            fold_v[j, i, 128 * b:128 * b + 128, :] = _dot(
                phi_t[g], pltpu.bitcast(wqkv_v[j, g], u32), _NT) * LOG2E

    def prep_folded(j, dst, m, hold):
        r0 = pl.multiple_of(16 * m, 16)
        return [_put_terms(dst, m, _lhs_terms, lambda i, jj, k: [hold(fold_v[
            j, i, pl.ds(r0 + 8 * p, 8), jj * HD + 128 * k:jj * HD + 128 * k + 128]) for p in range(2)])]

    def fold_k(b):
        fold(1, b)
        pacer.add("kv", 100, [functools.partial(prep_folded, 1, kv_s, 8 * b + m) for m in range(8)])

    def prep_x(c, terms, m, best, hold):
        first = [pl.multiple_of(c * TS + t * HT + 16 * m, 16) for t in range(2)]
        dots, done = {}, []
        for k in range(n_wb):
            words, quads = [], []
            for col in (k, n_wb + k):
                for t in range(2):
                    words.append(hold(pltpu.bitcast(
                        x_v[pl.ds(first[t], 16), 128 * col:128 * col + 128], u32)))
                    quads.append(_unpack(words[-1]))
                    for p in range(2):
                        for n in range(2):
                            v = quads[-1][p] * wrg_v[n, col]
                            dots[n, t, p] = v + dots[n, t, p] if (n, t, p) in dots else v
            even, odd = (_rhs_terms(*[q[p] for q in quads]) for p in range(2))
            for n in range(7):
                terms[m, n, k] = {1: words[0], 4: words[3]}.get(n)
                if terms[m, n, k] is None:
                    terms[m, n, k] = _pack(even[n], odd[n])
                    done.append(terms[m, n, k])
        for t in range(2):
            for p in range(2):
                g = jnp.broadcast_to(jnp.sum(dots[1, t, p], axis=1, keepdims=True), (8, 128))
                g = _sigmoid(g)
                g_v[pl.ds(first[t] + p, 8, stride=2), :] = g
                r = jnp.broadcast_to(jnp.sum(dots[0, t, p], axis=1, keepdims=True), (8, 128))
                r = r.astype(bf16).astype(f32)
                tok = first[t] + p + 2 * lax.broadcasted_iota(i32, (8, 128), 0)
                if m:
                    better = r > best[t, p][0]
                    r = jnp.where(better, r, best[t, p][0])
                    tok = jnp.where(better, tok, best[t, p][1])
                best[t, p] = (r, tok)
                done += [g, tok]
                if m == HT // 16 - 1:
                    rmax_v[c, 2 * t + p], rarg_v[c, 2 * t + p] = r, tok
        return done

    def prep_wo(m, hold):
        r0 = pl.multiple_of(16 * m, 16)
        return [_put_terms(wo_s, m, _rhs_terms, lambda i, j, k: _unpack(hold(pltpu.bitcast(
            wo_v[pl.ds(i * HD + r0, 16), j * HD + 128 * k:j * HD + 128 * k + 128], u32))))]

    def prep_v(b):
        halves = [pltpu.bitcast(wqkv_v[2, g].T, u32) for g in (b, b + n_wb)]
        for k in range(D // 128):
            for g, half in zip((b, b + n_wb), halves):
                wv_t[k, 64 * g:64 * g + 64, :] = half[:, 128 * k:128 * k + 128]
        return [lambda hold, m=m: [_put_terms(
            kv_s, (HD + 128 * b) // 16 + m, _lhs_terms, lambda i, j, k: _unpack(hold(
                wv_t[j * n_wb + k, 64 * (b + i * n_wb) + 8 * m:64 * (b + i * n_wb) + 8 * m + 8, :])))]
            for m in range(8)]

    def put_phi(p, j, logits, hold):
        phi_s[p, j] = _phi(logits, hold)
        return [phi_s[p, j, 56:64, :]]

    def features(pacer, tag, pairs, j0, res):
        pacer.add(tag, 100, [lambda hold, q=q, p=p, j=j: put_phi(
            p, j0 + j, res[64 * q:64 * q + 64, 128 * j:128 * j + 128], hold)
            for q, p in enumerate(pairs) for j in range(res.shape[1] // 128)], urgent=True)

    def with_ones(vt):
        return jnp.concatenate([vt, jnp.ones((16, vt.shape[1]), f32)], axis=0).astype(bf16)

    wait(whole[0:1])
    start(w_copies(1, 1))
    bits = jnp.concatenate([pltpu.bitcast(wphi_v[0:16, :], u32)] * 4, axis=1)
    zero = (bits & 1) * ((bits + 1) & 1)
    pacer = _Pacer(zero)
    pacer.rate = RATEK
    for g in range(D // 128):
        spread = _dot(sel, wphi_v[128 * g:128 * g + 128, :], _NT)
        phi_t[g] = pltpu.bitcast(jnp.where(same_head, spread, 0.0).astype(bf16), u32)
    rmax_v[...] = jnp.full(rmax_v.shape, -jnp.inf, f32)
    rarg_v[...] = jnp.zeros(rarg_v.shape, i32)

    def stage_x(t):
        for k in range(D // 128):
            x0_v[k, t * HT // 2:(t + 1) * HT // 2, :] = pltpu.bitcast(
                x_v[t * HT:(t + 1) * HT, 128 * k:128 * k + 128], u32)

    def k_block(b, t0, t1):
        lhs = jnp.concatenate([_pack(fold_v[1, i, r:r + 8, :], fold_v[1, i, r + 8:r + 16, :])
                               for i in range(2) for r in range(128 * b, 128 * b + 128, 16)], axis=0)
        pk = pacer.dot(lhs, _get(x0_v.at[:, t0 * HT // 2:t1 * HT // 2]), _NT)
        features(pacer, "k", [2 * b, 2 * b + 1, HP + 2 * b, HP + 2 * b + 1], 2 * t0, pk)

    def v_block(b):
        lhs = jnp.concatenate([wv_t[k, 128 * b:128 * b + 128, :] for k in range(D // 128)], axis=1)
        vt = pacer.dot(lhs, _get(x0_v), _NT)
        pacer.flush("k")
        for q in range(4):
            kv_acc[4 * b + q] = _dot(with_ones(vt[64 * q:64 * q + 64]), _get(phi_s.at[4 * b + q]), _NT)

    def put_x(c, terms, hold):
        for (m, n, k), term in sorted(terms.items(), key=lambda item: item[0]):
            x_s[c, n, k, 8 * m:8 * m + 8, :] = hold(m)(term)

    strips = lambda j, b0, b1: [cp for b in range(b0, b1) for cp in w_copies(j, b)]
    wait(strips(1, 0, 1))
    start([x_copy(1, 2)])
    fold_k(0)
    wait([x_copy(0, 1)])
    start(strips(1, 2, 4))
    stage_x(0)
    k_block(0, 0, 1)
    wait(strips(1, 1, 2))
    start(strips(2, 0, 4))
    fold_k(1)
    k_block(1, 0, 1)
    wait([x_copy(1, 2)])
    start(strips(0, 0, 4) + [x_copy(2, 4)])
    stage_x(1)
    k_block(0, 1, 2)
    k_block(1, 1, 2)
    wait(strips(1, 2, 4))
    start([x_copy(4, 8), whole[3]])
    fold_k(2)
    k_block(2, 0, 2)
    fold_k(3)
    wait(strips(2, 0, 4) + whole[1:3])
    start(whole[4:])
    for n, w in enumerate((wr_v, gw_v)):
        w = w[...].astype(f32)
        for col in range(D // 128):
            wrg_v[n, col] = jnp.broadcast_to(w[col:col + 1], (8, 128))
    pacer.add("kv", 90, prep_v(0) + prep_v(1))
    k_block(3, 0, 2)
    pacer.add("kv", 90, prep_v(2) + prep_v(3))
    v_block(0)
    v_block(2)
    pacer.flush("kv")
    wait(strips(0, 0, 4) + [x_copy(2, 4)])
    for b in range(n_wb):
        fold(0, b)
    best = {}

    def first_x(m, hold):
        terms = {}
        done = prep_x(1, terms, m, best, hold)
        put_x(1, terms, lambda m: lambda v: v)
        return done[-8:] + [x_s[1, 6, n_wb - 1, 8 * m:8 * m + 8, :]]

    pacer.add("x", 270, [functools.partial(first_x, m) for m in range(HT // 16)])
    pacer.rate = RATE0
    v_block(1)
    v_block(3)
    pacer.flush("x")
    wait([x_copy(4, 8), whole[3]])

    def project(pacer, lhs_s, c, finish):
        product = lambda n: pacer.dot(_get(lhs_s.at[n]), _get(x_s.at[c, n]), _NT)
        m3 = product(2)
        m5 = product(4)
        s12 = finish(0, 1, m3 + m5)
        m4 = product(3)
        t = m4 - m5
        m2 = product(1)
        s12()
        s21 = finish(1, 0, m2 + m4)
        u = m3 - m2
        m1 = product(0)
        t = t + m1
        u = u + m1
        m7 = product(6)
        s21()
        s11 = finish(0, 0, t + m7)
        m6 = product(5)
        return s11, finish(1, 1, u + m6)

    def phase1(c, _):
        pacer = _Pacer(zero)
        pacer.rate = RATE1
        nxt = jnp.where(c + 1 < n_chunks, c + 1, 0)
        best, terms = {}, {}
        pacer.add("x", 290, [functools.partial(prep_x, nxt, terms, m, best) for m in range(HT // 16)])
        share = pl.cdiv(HD // 16, n_chunks - 1)
        for prep in (prep_wo, functools.partial(prep_folded, 0, q_s)):
            pacer.add("w", 120, [functools.partial(
                prep, jnp.minimum((c - 1) * share + j, HD // 16 - 1)) for j in range(share)])
        kr = lax.broadcasted_iota(i32, (80, 128), 0)
        kl = lax.broadcasted_iota(i32, (80, 128), 1)
        keep = jnp.where(kr < 64, kr // 32, (kr - 64) // 8) == kl // 2 % 2

        def kv_finish(half, t, res):
            features(pacer, (half, t), range(half * HP, half * HP + HP), 2 * t, res)

            def update():
                pacer.flush((half, t))
                for q in range(HP):
                    p = half * HP + q
                    acc = kv_acc[p] + _dot(with_ones(res[HD + 64 * q:HD + 64 * q + 64]),
                                           _get(phi_s.at[p, 2 * t:2 * t + 2]), _NT)
                    kv_acc[p] = acc
                    if half == t:
                        kv_t[p] = jnp.where(keep, acc, 0.0).astype(bf16)
            return update

        s11, s22 = project(pacer, kv_s, c, kv_finish)
        pacer.flush("x")
        put_x(nxt, terms, functools.cache(lambda m: pacer.hold(m / (HT // 16))))

        r = rmax_v[...].reshape(n_chunks * 32, 128)
        tok = rarg_v[...].reshape(n_chunks * 32, 128)
        r_max = jnp.max(r, axis=0, keepdims=True)
        idx = jnp.min(jnp.where(r == r_max, tok, S - 1))
        rows = x_v[pl.ds(pl.multiple_of((idx // 16) * 16, 16), 16), :].astype(f32)
        is_sel = lax.broadcasted_iota(i32, (16, D), 0) == idx % 16
        xcol_v[...] = _lane_bcast_rows(jnp.sum(jnp.where(is_sel, rows, 0.0), axis=0, keepdims=True))
        s11()
        s22()
        pacer.flush("w")
        return idx, r_max

    idx, r_max = lax.fori_loop(1, n_chunks, phase1, (jnp.int32(0), jnp.zeros((1, 128), f32)))
    y_v[...] = jnp.zeros(y_v.shape, f32)
    routed = idx // TS
    idx16 = pl.multiple_of((idx // 16) * 16, 16)
    r_gate = _sigmoid(r_max[:, 0:1])
    wait(whole[4:])

    def chunk_of(i):
        c = routed + i
        return jnp.where(c >= n_chunks, c - n_chunks, c)

    def out_copy(i, t, h, c0, width):
        return pltpu.make_async_copy(
            out_v.at[i, t, h, :, pl.ds(c0, width)],
            out_hbm.at[pl.ds(chunk_of(i) * TS + t * HT, HT), pl.ds(h * HD + c0, width)],
            sem_o.at[jnp.minimum(i, 1)])

    def phase2(i, _):
        pacer = _Pacer(zero)
        c = chunk_of(i)

        def mat_vec(acc, col_ref, blocks, k0, hold):
            for k in range(k0, k0 + KS):
                col = hold(col_ref[8 * k:8 * k + 8, :])
                for a, block in enumerate(blocks):
                    n = block.shape[1] // 128
                    for j0 in range(0, n, 2):
                        j1 = min(j0 + 2, n)
                        w = block[8 * k:8 * k + 8, 128 * j0:128 * j1].astype(f32)
                        for j in range(j0, j1):
                            p = w[:, 128 * (j - j0):128 * (j - j0) + 128] * col
                            acc[a * n + j] = p if acc[a * n + j] is None else acc[a * n + j] + p
            return list(acc)

        def hidden(hold):
            gate, up = (jnp.sum(jnp.concatenate(v, axis=1), axis=0, keepdims=True)
                        for v in (gu[:FS // 128], gu[FS // 128:]))
            hcol_v[...] = _lane_bcast_rows(gate * _sigmoid(gate) * up)
            return [hcol_v[FS - 8:FS, :]]

        gu = [None] * (2 * FS // 128)
        y = [y_v[:, 128 * j:128 * j + 128] for j in range(D // 128)]
        pacer.add("ffn", KS * 43, [lambda hold, k=k: mat_vec(gu, xcol_v, (wg_v.at[i], wu_v.at[i]), k, hold)
                                  for k in range(0, D // 8, KS)])
        pacer.add("ffn", 400, [hidden])
        pacer.add("ffn", KS * 25, [lambda hold, k=k: mat_vec(y, hcol_v, (wd_v.at[i],), k, hold)
                                  for k in range(0, FS // 8, KS)])
        o = {}

        def q_finish(half, t, res):
            features(pacer, (half, t), range(half * HP, half * HP + HP), 2 * t, res)

            def attend():
                pacer.flush((half, t))
                o_t = []
                for p in range(half * HP, half * HP + HP):
                    nd = _dot(kv_t[p], _get(phi_s.at[p, 2 * t:2 * t + 2]), _NN)
                    for h in range(2):
                        inv = _recip(nd[64 + 8 * h:72 + 8 * h] + 1e-6)
                        o_t += [nd[32 * h + 8 * j:32 * h + 8 * j + 8] * inv for j in range(4)]
                o[t, half] = jnp.concatenate(o_t, axis=0)
            return attend

        def o_product(n, o_t):
            return pacer.dot(pltpu.bitcast(o_t.astype(bf16).T, u32), _get(wo_s.at[n]), _NN)

        def mix(t, h, a):
            def piece(m, k0, k1, hold):
                rows = pl.ds(pl.multiple_of(c * TS + t * HT + 16 * m, 16), 16)
                g = g_v[rows, :]
                g = jnp.concatenate([hold(g[:8]), hold(g[8:])], axis=0)
                for k in range(k0, k1):
                    xb = x_v[rows, h * HD + 128 * k:h * HD + 128 * k + 128].astype(f32)
                    out_v[i, t, h, 16 * m:16 * m + 16, 128 * k:128 * k + 128] = (
                        g * a[16 * m:16 * m + 16, 128 * k:128 * k + 128] + (1.0 - g) * xb).astype(bf16)
                return [out_v[i, t, h, 16 * m:16 * m + 16, HD - 128:HD]]

            def send(n=1):
                pacer.flush(("mix", t, h), run=n == 1)
                for k0 in range(0, n_wb, n_wb // n):
                    for m in range(HT // 16 if n > 1 else 0):
                        piece(m, k0, k0 + n_wb // n, lambda v: v)
                    out_copy(i, t, h, 128 * k0, HD // n).start()

            pacer.add(("mix", t, h), 60,
                      [functools.partial(piece, m, 0, n_wb) for m in range(HT // 16)], True)
            return send

        s11, s22 = project(pacer, q_s, c, q_finish)
        m3 = o_product(2, o[1, 0])
        s11()
        m4 = o_product(3, o[0, 1])
        m1 = o_product(0, o[1, 0] + o[0, 1])
        s22()
        t = m1 + m4
        u = m1 + m3
        m2 = o_product(1, o[0, 0] + o[0, 1])
        send = mix(0, 0, m2 + m4)
        u = u - m2
        m6 = o_product(5, o[0, 0] - o[1, 0])
        send()
        send = mix(0, 1, u + m6)
        m5 = o_product(4, o[1, 0] + o[1, 1])
        send()
        send = mix(1, 1, m3 + m5)
        t = t - m5
        m7 = o_product(6, o[1, 1] - o[0, 1])
        send()

        pacer.flush("ffn")
        y = jnp.concatenate(y, axis=1)
        y_v[...] = y
        staged = jnp.concatenate(
            [out_v[0, idx % TS // HT, h, pl.ds(pl.multiple_of(idx16 % HT, 16), 16), :]
             for h in range(2)], axis=1).astype(f32)
        g = jnp.concatenate([g_v[pl.ds(idx16, 16), :]] * (D // 128), axis=1)
        is_sel = lax.broadcasted_iota(i32, (16, D), 0) == idx % 16
        y = jnp.sum(y, axis=0, keepdims=True) * r_gate
        row_v[...] = (staged + jnp.where(is_sel, (1.0 - g) * y, 0.0)).astype(bf16)
        mix(1, 0, t + m7)(n=2)
        return 0

    lax.fori_loop(0, n_chunks, phase2, 0)
    sent = lambda rows, n: pltpu.make_async_copy(out_v.at[rows], out_v.at[rows], sem_o.at[n])
    sent(slice(0, 1), 0).wait()
    row_copy = pltpu.make_async_copy(row_v, out_hbm.at[pl.ds(idx16, 16)], sem_o.at[0])
    row_copy.start()
    sent(slice(1, n_chunks), 1).wait()
    row_copy.wait()


@jax.jit
def pallas_gated_mix__linear_kernel_hedgehog__moe_arch_mod__prompt_kernel(
    A_x: jax.Array,
    A_wqkv: jax.Array,
    A_w_phi: jax.Array,
    A_wo: jax.Array,
    B_x: jax.Array,
    B_w_r: jax.Array,
    B_w_gate: jax.Array,
    B_w_up: jax.Array,
    B_w_down: jax.Array,
    gate_w: jax.Array,
):
    del B_x
    B, S, D = A_x.shape
    H, Dh, _ = A_w_phi.shape
    F = B_w_gate.shape[1]
    n_chunks = S // TS
    FS = F // n_chunks
    HD, HT = D // 2, TS // 2
    assert B == 1 and Dh == 32 and D == 1024 and H * Dh == D and S == 4 * TS and FS % 128 == 0

    hbm = pl.BlockSpec(memory_space=pl.ANY)
    out = pl.pallas_call(
        _kernel,
        out_shape=jax.ShapeDtypeStruct((S, D), A_x.dtype),
        in_specs=[hbm] * 9,
        out_specs=hbm,
        scratch_shapes=[
            pltpu.VMEM((S, D), bf16),
            pltpu.VMEM((3, D // 128, D, 128), bf16),
            pltpu.VMEM((H * Dh, Dh), bf16),
            pltpu.VMEM((8, 128), bf16),
            pltpu.VMEM((8, 128), bf16),
            pltpu.VMEM((D, D), bf16),
            pltpu.VMEM((n_chunks, D, FS), bf16),
            pltpu.VMEM((n_chunks, D, FS), bf16),
            pltpu.VMEM((n_chunks, FS, D), bf16),
            pltpu.VMEM((2, D // 128, 8, 128), f32),
            pltpu.VMEM((2, 2, HD, D), f32),
            pltpu.VMEM((D // 128, 64, 128), u32),
            pltpu.VMEM((D // 128, TS // 2, 128), u32),
            pltpu.VMEM((D // 128, D // 2, 128), u32),
            pltpu.VMEM((7, HD // 128, D // 2, 128), u32),
            pltpu.VMEM((7, HD // 128, HD // 2, 128), u32),
            pltpu.VMEM((7, HD // 128, HD // 2, 128), u32),
            pltpu.VMEM((n_chunks, 7, HD // 128, HT // 2, 128), u32),
            pltpu.VMEM((H // 2, TS // 128, 64, 128), u32),
            pltpu.VMEM((H // 2, 80, 128), f32),
            pltpu.VMEM((H // 2, 80, 128), bf16),
            pltpu.VMEM((n_chunks, 4, 8, 128), f32),
            pltpu.VMEM((n_chunks, 4, 8, 128), i32),
            pltpu.VMEM((S + 8, 128), f32),
            pltpu.VMEM((n_chunks, 2, 2, HT, HD), bf16),
            pltpu.VMEM((16, D), bf16),
            pltpu.VMEM((D, 128), f32),
            pltpu.VMEM((FS, 128), f32),
            pltpu.VMEM((8, D), f32),
            pltpu.SemaphoreType.DMA((5,)),
            pltpu.SemaphoreType.DMA((3, D // 128)),
            pltpu.SemaphoreType.DMA((4 + 3 * n_chunks,)),
            pltpu.SemaphoreType.DMA((2,)),
        ],
        compiler_params=pltpu.CompilerParams(vmem_limit_bytes=110 * 1024 * 1024),
        name="gated_mix_hedgehog_mod",
    )(A_x.reshape(S, D), A_wqkv, A_w_phi.reshape(H * Dh, Dh), A_wo, B_w_r.reshape(8, 128),
      B_w_gate, B_w_up, B_w_down, gate_w.reshape(8, 128))
    return out.reshape(B, S, D)
```

```python
import functools

import jax
import jax.numpy as jnp
from jax import lax
import jax.experimental.pallas as pl
import jax.experimental.pallas.tpu as pltpu

TS = 512
LOG2E = 1.4426950408889634
RATE0 = 1.0
RATE1 = 0.95
RATEK = 1.0
KS = 2
RATE = 1.35

_NT = (((1,), (1,)), ((), ()))
_NN = (((1,), (0,)), ((), ()))

f32 = jnp.float32
bf16 = jnp.bfloat16
i32 = jnp.int32
u32 = jnp.uint32


def _dot(a, b, dims):
    a, b = (pltpu.bitcast(v, bf16) if v.dtype == u32 else v for v in (a, b))
    return lax.dot_general(a, b, dims, preferred_element_type=f32)


def _tree(op, xs):
    xs = list(xs)
    while len(xs) > 1:
        nxt = [op(xs[i], xs[i + 1]) for i in range(0, len(xs) - 1, 2)]
        if len(xs) % 2:
            nxt.append(xs[-1])
        xs = nxt
    return xs[0]


def _recip(x):
    return pl.reciprocal(x, full_range=False)


def _sigmoid(x):
    return 0.5 + 0.5 * jnp.tanh(0.5 * x)


def _head_reduce(op, tiles):
    r = _tree(op, tiles)
    r = op(r, pltpu.roll(r, 4, 0))
    return op(r, pltpu.roll(r, 2, 0))


def _phi(p, hold):
    tiles = [p[8 * j:8 * j + 8] for j in range(8)]
    out = []
    for op, diff in ((jnp.maximum, lambda t, m: t - m), (jnp.minimum, lambda t, m: m - t)):
        m = hold(_head_reduce(op, tiles))
        e = [jnp.exp2(diff(t, m)) for t in tiles]
        r = _recip(_head_reduce(jnp.add, e))
        out += [jnp.concatenate([e[j] * r, e[j + 1] * r], axis=0).astype(bf16) for j in range(0, 8, 2)]
    return out


def _lane_bcast_rows(row):
    return jnp.broadcast_to(row, (128, row.shape[1])).T


def _lhs_terms(a11, a12, a21, a22):
    return (a11 + a22, a21 + a22, a11, a22, a11 + a12, a21 - a11, a12 - a22)


def _rhs_terms(b11, b12, b21, b22):
    return (b11 + b22, b11, b12 - b22, b21 - b11, b22, b11 + b12, b21 + b22)


def _put_terms(dst, m, terms_fn, load):
    rows = pl.ds(pl.multiple_of(16 * m, 16), 16)
    for k in range(dst.shape[1]):
        terms = terms_fn(*[load(i, j, k) for i in range(2) for j in range(2)])
        for n in range(7):
            dst[n, k, rows, :] = terms[n].astype(bf16)
    return terms[6][8:]


def _get(ref):
    ref = ref.bitcast(u32)
    return jnp.concatenate([ref[k] for k in range(ref.shape[0])], axis=1)


class _Pacer:
    def __init__(self, zero):
        self.zero = zero
        self.previous = None
        self.tick = 0
        self.rate = RATE
        self.queues = ([], [])

    def add(self, tag, cost, pieces, urgent=False):
        self.queues[0 if urgent else 1].extend(
            (tag, cost, max(self.tick + urgent, 1), p) for p in pieces)

    def flush(self, tag, run=True):
        for queue in self.queues:
            for item in [q for q in queue if q[0] == tag]:
                queue[:] = [q for q in queue if q is not item]
                if run:
                    item[3](lambda v: v)

    def _take(self, budget):
        taken = ([], [])
        for queue, out in zip(self.queues, taken):
            while queue and queue[0][2] <= self.tick and budget >= queue[0][1] / 2:
                budget -= queue[0][1]
                out.append(queue.pop(0)[3])
        return taken

    def hold(self, where):
        rows = self.previous.shape[0] // 8
        start = pltpu.bitcast(self.previous[int(where * rows) * 8:][:8], u32) & self.zero
        return lambda v: pltpu.bitcast(
            pltpu.bitcast(v, u32) | jnp.concatenate([start] * (v.shape[0] // 8), axis=0), f32)

    def dot(self, lhs, rhs, dims):
        n = rhs.shape[0] // 64 if dims == _NT else rhs.shape[1] // 128
        out = []
        for j in range(n):
            marks = {}
            urgent, chain = self._take(self.rate * lhs.shape[0] * lhs.shape[1] / 256)
            for pieces, shift in ((urgent, 0.0), (chain, 0.5)):
                for m, piece in enumerate(pieces):
                    where = (m + shift) / len(pieces)
                    done = piece(self.hold(where))
                    if done and (pieces is urgent or m == len(pieces) - 1):
                        marks.setdefault(int(where * lhs.shape[0] / 8) * 8, []).extend(done)
            parts, at = [], 0
            for row, done in sorted(marks.items()):
                bits = _tree(jnp.bitwise_or, [pltpu.bitcast(v, u32) for v in done]) & self.zero
                parts += [lhs[at:row]] if row > at else []
                parts.append(jnp.concatenate(
                    [lhs[row:row + 8, 0:128] | bits, lhs[row:row + 8, 128:]], axis=1))
                at = row + 8
            a = jnp.concatenate(parts + ([lhs[at:]] if at < lhs.shape[0] else []), axis=0)
            out.append(_dot(a, rhs[64 * j:64 * j + 64] if dims == _NT else
                            rhs[:, 128 * j:128 * j + 128], dims))
            self.previous = out[-1]
            self.tick += 1
        return jnp.concatenate(out, axis=1)


def _kernel(x_hbm, wqkv_hbm, wphi_hbm, wo_hbm, wr_hbm, wg_hbm, wu_hbm, wd_hbm, gw_hbm,
            out_hbm,
            x_v, wqkv_v, wphi_v, wr_v, gw_v, wo_v, wg_v, wu_v, wd_v, wrg_v, fold_v, phi_t, x0_v, wv_t, kv_s, q_s,
            wo_s, x_s, phi_s, kv_acc, kv_t, rmax_v, rarg_v, g_v, out_v, row_v, xcol_v, hcol_v, y_v,
            sem_x, sem_w, sem_s, sem_o):
    S, D = x_v.shape
    F = wd_hbm.shape[0]
    n_chunks = S // TS
    n_pairs = D // 64
    FS = hcol_v.shape[0]
    HD, HT = D // 2, TS // 2
    n_wb = HD // 128
    HP = n_pairs // 2

    def x_copy(h0, h1):
        rows = pl.ds(h0 * HT, (h1 - h0) * HT)
        return pltpu.make_async_copy(x_hbm.at[rows], x_v.at[rows], sem_x.at[h0])

    def w_copies(j, b):
        return [pltpu.make_async_copy(wqkv_hbm.at[:, pl.ds(j * D + g * 128, 128)],
                                      wqkv_v.at[j, g], sem_w.at[j, g]) for g in (b, b + n_wb)]

    whole = [pltpu.make_async_copy(src, dst, sem_s.at[n]) for n, (src, dst) in enumerate(
        [(wphi_hbm, wphi_v), (wr_hbm, wr_v), (gw_hbm, gw_v), (wo_hbm, wo_v)]
        + [pair for i in range(n_chunks) for pair in (
            (wg_hbm.at[:, pl.ds(i * FS, FS)], wg_v.at[i]),
            (wu_hbm.at[:, pl.ds(i * FS, FS)], wu_v.at[i]),
            (wd_hbm.at[pl.ds(i * FS, FS)], wd_v.at[i]))])]

    def start(copies):
        for cp in copies:
            cp.start()

    def wait(copies):
        for cp in copies:
            cp.wait()

    start(whole[0:1] + w_copies(1, 0) + [x_copy(0, 1)] + whole[1:3])

    c_i = lax.broadcasted_iota(i32, (128, 32), 0)
    f_i = lax.broadcasted_iota(i32, (128, 32), 1)
    sel = jnp.where(c_i % 64 // 2 == f_i, 1.0, 0.0).astype(bf16)
    r_i = lax.broadcasted_iota(i32, (128, 128), 0)
    l_i = lax.broadcasted_iota(i32, (128, 128), 1)
    same_head = (2 * (r_i // 64) + r_i % 2) == (l_i // 32)

    def fold(j, b):
        for i in range(2):
            g = b + i * n_wb
            fold_v[j, i, 128 * b:128 * b + 128, :] = _dot(
                _get(phi_t.at[g:g + 1]), _get(wqkv_v.at[j, g:g + 1]), _NT) * LOG2E

    def gated(hold, i, j, v):
        return hold(v.astype(f32)) if i == j else v.astype(f32)

    def prep_folded(src, dst, m, hold):
        rows = pl.ds(pl.multiple_of(16 * m, 16), 16)
        return [_put_terms(dst, m, _lhs_terms, lambda i, j, k: gated(
            hold, i, j, fold_v[src, i, rows, j * HD + 128 * k:j * HD + 128 * k + 128]))]

    def fold_k(b):
        fold(1, b)
        pacer.add("kv", 100, [functools.partial(prep_folded, 1, kv_s, 8 * b + m) for m in range(8)])

    def prep_x(c, terms, m, best, hold):
        first = [pl.multiple_of(c * TS + t * HT + 16 * m, 16) for t in range(2)]
        dots, done = {}, []
        for k in range(n_wb):
            quads = []
            for i in range(2):
                col = i * n_wb + k
                for t in range(2):
                    quads.append(gated(hold, i, t, x_v[pl.ds(first[t], 16), 128 * col:128 * col + 128]))
                    for p in range(2):
                        for n in range(2):
                            v = quads[-1][8 * p:8 * p + 8] * wrg_v[n, col]
                            dots[n, t, p] = v + dots[n, t, p] if (n, t, p) in dots else v
            for n, term in enumerate(_rhs_terms(*quads)):
                terms[m, n, k] = term
                if n not in (1, 4):
                    done.append(term[8:])
        for t in range(2):
            for p in range(2):
                g = jnp.broadcast_to(jnp.sum(dots[1, t, p], axis=1, keepdims=True), (8, 128))
                g = _sigmoid(g)
                g_v[pl.ds(pl.multiple_of(first[t] + 8 * p, 8), 8), :] = g
                r = jnp.broadcast_to(jnp.sum(dots[0, t, p], axis=1, keepdims=True), (8, 128))
                r = r.astype(bf16).astype(f32)
                tok = first[t] + 8 * p + lax.broadcasted_iota(i32, (8, 128), 0)
                if m:
                    better = r > best[t, p][0]
                    r = jnp.where(better, r, best[t, p][0])
                    tok = jnp.where(better, tok, best[t, p][1])
                best[t, p] = (r, tok)
                done += [g, tok]
                if m == HT // 16 - 1:
                    rmax_v[c, 2 * t + p], rarg_v[c, 2 * t + p] = r, tok
        return done

    def prep_wo(m, hold):
        return [_put_terms(wo_s, m, _rhs_terms, lambda i, j, k: gated(hold, i, j, wo_v[
            pl.ds(pl.multiple_of(i * HD + 16 * m, 16), 16), j * HD + 128 * k:j * HD + 128 * k + 128]))]

    def prep_v(b):
        for g in (b, b + n_wb):
            strip = wqkv_v[2, g].T
            for k in range(D // 128):
                wv_t[k, 128 * g:128 * g + 128, :] = strip[:, 128 * k:128 * k + 128]
        return [lambda hold, m=m: [_put_terms(kv_s, HD // 16 + m, _lhs_terms, lambda i, j, k: gated(
            hold, i, j, wv_t[j * n_wb + k, i * HD + 16 * m:i * HD + 16 * m + 16, :]))]
            for m in range(8 * b, 8 * b + 8)]

    def put_phi(p, j, logits, hold):
        for n, rows in enumerate(_phi(logits, hold)):
            phi_s[p, j, 16 * n:16 * n + 16, :] = rows
        return [phi_s.at[p, j].bitcast(u32)[56:64, :]]

    def features(pacer, tag, pairs, j0, res):
        pacer.add(tag, 100, [lambda hold, q=q, p=p, j=j: put_phi(
            p, j0 + j, res[64 * q:64 * q + 64, 128 * j:128 * j + 128], hold)
            for q, p in enumerate(pairs) for j in range(res.shape[1] // 128)], urgent=True)

    def with_ones(vt):
        return jnp.concatenate([vt, jnp.ones((16, vt.shape[1]), f32)], axis=0).astype(bf16)

    wait(whole[0:1])
    start(w_copies(1, 1))
    bits = jnp.concatenate([pltpu.bitcast(wphi_v[0:16, :], u32)] * 4, axis=1)
    zero = (bits & 1) * ((bits + 1) & 1)
    pacer = _Pacer(zero)
    pacer.rate = RATEK
    for g in range(D // 128):
        spread = _dot(sel, wphi_v[128 * g:128 * g + 128, :], _NT)
        phi_t[g] = jnp.where(same_head, spread, 0.0).astype(bf16)
    rmax_v[...] = jnp.full(rmax_v.shape, -jnp.inf, f32)
    rarg_v[...] = jnp.zeros(rarg_v.shape, i32)

    def stage_x(t):
        for k in range(D // 128):
            x0_v[k, t * HT:(t + 1) * HT, :] = x_v[t * HT:(t + 1) * HT, 128 * k:128 * k + 128]

    def k_block(b, t0, t1):
        lhs = jnp.concatenate([fold_v[1, i, 128 * b:128 * b + 128, :] for i in range(2)], axis=0)
        lhs = pltpu.bitcast(lhs.astype(bf16), u32)
        pk = pacer.dot(lhs, _get(x0_v.at[:, t0 * HT:t1 * HT]), _NT)
        features(pacer, "k", [2 * b, 2 * b + 1, HP + 2 * b, HP + 2 * b + 1], 2 * t0, pk)

    def v_block(b):
        vt = pacer.dot(_get(wv_t.at[:, 256 * b:256 * b + 256]), _get(x0_v), _NT)
        pacer.flush("k")
        for q in range(4):
            kv_acc[4 * b + q] = _dot(with_ones(vt[64 * q:64 * q + 64]), _get(phi_s.at[4 * b + q]), _NT)

    def put_x(c, terms, hold):
        for (m, n, k), term in sorted(terms.items(), key=lambda item: item[0]):
            term = jnp.concatenate([hold(m)(term[:8]), term[8:]], axis=0)
            x_s[c, n, k, 16 * m:16 * m + 16, :] = term.astype(bf16)

    strips = lambda j, b0, b1: [cp for b in range(b0, b1) for cp in w_copies(j, b)]
    wait(strips(1, 0, 1))
    start([x_copy(1, 2)])
    fold_k(0)
    wait([x_copy(0, 1)])
    start(strips(1, 2, 4))
    stage_x(0)
    k_block(0, 0, 1)
    wait(strips(1, 1, 2))
    start(strips(2, 0, 4))
    fold_k(1)
    k_block(1, 0, 1)
    wait([x_copy(1, 2)])
    start(strips(0, 0, 4) + [x_copy(2, 4)])
    stage_x(1)
    k_block(0, 1, 2)
    k_block(1, 1, 2)
    wait(strips(1, 2, 4))
    start([x_copy(4, 8), whole[3]])
    fold_k(2)
    k_block(2, 0, 2)
    fold_k(3)
    wait(strips(2, 0, 4) + whole[1:3])
    start(whole[4:])
    for n, w in enumerate((wr_v, gw_v)):
        w = w[...].astype(f32)
        for col in range(D // 128):
            wrg_v[n, col] = jnp.broadcast_to(w[col:col + 1], (8, 128))
    pacer.add("kv", 90, prep_v(0) + prep_v(1))
    k_block(3, 0, 2)
    pacer.add("kv", 90, prep_v(2) + prep_v(3))
    v_block(0)
    v_block(2)
    pacer.flush("kv")
    wait(strips(0, 0, 4) + [x_copy(2, 4)])
    for b in range(n_wb):
        fold(0, b)
    best = {}

    def first_x(m, hold):
        terms = {}
        done = prep_x(1, terms, m, best, hold)
        put_x(1, terms, lambda m: lambda v: v)
        return done

    pacer.add("x", 270, [functools.partial(first_x, m) for m in range(HT // 16)])
    pacer.rate = RATE0
    v_block(1)
    v_block(3)
    pacer.flush("x")
    wait([x_copy(4, 8), whole[3]])

    def project(pacer, lhs_s, c, finish):
        product = lambda n: pacer.dot(_get(lhs_s.at[n]), _get(x_s.at[c, n]), _NT)
        m3 = product(2)
        m5 = product(4)
        s12 = finish(0, 1, m3 + m5)
        m4 = product(3)
        t = m4 - m5
        m2 = product(1)
        s12()
        s21 = finish(1, 0, m2 + m4)
        u = m3 - m2
        m1 = product(0)
        t = t + m1
        u = u + m1
        m7 = product(6)
        s21()
        s11 = finish(0, 0, t + m7)
        m6 = product(5)
        return s11, finish(1, 1, u + m6)

    def phase1(c, _):
        pacer = _Pacer(zero)
        pacer.rate = RATE1
        nxt = jnp.where(c + 1 < n_chunks, c + 1, 0)
        best, terms = {}, {}
        pacer.add("x", 290, [functools.partial(prep_x, nxt, terms, m, best) for m in range(HT // 16)])
        share = pl.cdiv(HD // 16, n_chunks - 1)
        for prep in (prep_wo, functools.partial(prep_folded, 0, q_s)):
            pacer.add("w", 120, [functools.partial(
                prep, jnp.minimum((c - 1) * share + j, HD // 16 - 1)) for j in range(share)])
        kr = lax.broadcasted_iota(i32, (80, 128), 0)
        kl = lax.broadcasted_iota(i32, (80, 128), 1)
        keep = jnp.where(kr < 64, kr // 32, (kr - 64) // 8) == kl % 2

        def kv_finish(half, t, res):
            features(pacer, (half, t), range(half * HP, half * HP + HP), 2 * t, res)

            def update():
                pacer.flush((half, t))
                for q in range(HP):
                    p = half * HP + q
                    acc = kv_acc[p] + _dot(with_ones(res[HD + 64 * q:HD + 64 * q + 64]),
                                           _get(phi_s.at[p, 2 * t:2 * t + 2]), _NT)
                    kv_acc[p] = acc
                    if half == t:
                        kv_t[p] = jnp.where(keep, acc, 0.0).astype(bf16)
            return update

        s11, s22 = project(pacer, kv_s, c, kv_finish)
        pacer.flush("x")
        put_x(nxt, terms, functools.cache(lambda m: pacer.hold(m / (HT // 16))))

        r = rmax_v[...].reshape(n_chunks * 32, 128)
        tok = rarg_v[...].reshape(n_chunks * 32, 128)
        r_max = jnp.max(r, axis=0, keepdims=True)
        idx = jnp.min(jnp.where(r == r_max, tok, S - 1))
        rows = x_v[pl.ds(pl.multiple_of((idx // 16) * 16, 16), 16), :].astype(f32)
        is_sel = lax.broadcasted_iota(i32, (16, D), 0) == idx % 16
        xcol_v[...] = _lane_bcast_rows(jnp.sum(jnp.where(is_sel, rows, 0.0), axis=0, keepdims=True))
        s11()
        s22()
        pacer.flush("w")
        return idx, r_max

    idx, r_max = lax.fori_loop(1, n_chunks, phase1, (jnp.int32(0), jnp.zeros((1, 128), f32)))
    y_v[...] = jnp.zeros(y_v.shape, f32)
    routed = idx // TS
    idx16 = pl.multiple_of((idx // 16) * 16, 16)
    r_gate = _sigmoid(r_max[:, 0:1])
    wait(whole[4:])

    def chunk_of(i):
        c = routed + i
        return jnp.where(c >= n_chunks, c - n_chunks, c)

    def out_copy(i, t, h, c0, width):
        return pltpu.make_async_copy(
            out_v.at[i, t, h, :, pl.ds(c0, width)],
            out_hbm.at[pl.ds(chunk_of(i) * TS + t * HT, HT), pl.ds(h * HD + c0, width)],
            sem_o.at[jnp.minimum(i, 1)])

    def phase2(i, _):
        pacer = _Pacer(zero)
        c = chunk_of(i)

        def mat_vec(acc, col_ref, blocks, k0, hold):
            for k in range(k0, k0 + KS):
                col = hold(col_ref[8 * k:8 * k + 8, :])
                for a, block in enumerate(blocks):
                    n = block.shape[1] // 128
                    for j0 in range(0, n, 2):
                        j1 = min(j0 + 2, n)
                        w = block[8 * k:8 * k + 8, 128 * j0:128 * j1].astype(f32)
                        for j in range(j0, j1):
                            p = w[:, 128 * (j - j0):128 * (j - j0) + 128] * col
                            acc[a * n + j] = p if acc[a * n + j] is None else acc[a * n + j] + p
            return list(acc)

        def hidden(hold):
            gate, up = (jnp.sum(jnp.concatenate(v, axis=1), axis=0, keepdims=True)
                        for v in (gu[:FS // 128], gu[FS // 128:]))
            hcol_v[...] = _lane_bcast_rows(gate * _sigmoid(gate) * up)
            return [hcol_v[FS - 8:FS, :]]

        gu = [None] * (2 * FS // 128)
        y = [y_v[:, 128 * j:128 * j + 128] for j in range(D // 128)]
        pacer.add("ffn", KS * 43, [lambda hold, k=k: mat_vec(gu, xcol_v, (wg_v.at[i], wu_v.at[i]), k, hold)
                                  for k in range(0, D // 8, KS)])
        pacer.add("ffn", 400, [hidden])
        pacer.add("ffn", KS * 25, [lambda hold, k=k: mat_vec(y, hcol_v, (wd_v.at[i],), k, hold)
                                  for k in range(0, FS // 8, KS)])
        o = {}

        def q_finish(half, t, res):
            features(pacer, (half, t), range(half * HP, half * HP + HP), 2 * t, res)

            def attend():
                pacer.flush((half, t))
                o_t = []
                for p in range(half * HP, half * HP + HP):
                    nd = _dot(_get(kv_t.at[p:p + 1]), _get(phi_s.at[p, 2 * t:2 * t + 2]), _NN)
                    for h in range(2):
                        inv = _recip(nd[64 + 8 * h:72 + 8 * h] + 1e-6)
                        o_t += [nd[32 * h + 8 * j:32 * h + 8 * j + 8] * inv for j in range(4)]
                o[t, half] = jnp.concatenate(o_t, axis=0)
            return attend

        def o_product(n, o_t):
            return pacer.dot(pltpu.bitcast(o_t.astype(bf16).T, u32), _get(wo_s.at[n]), _NN)

        def mix(t, h, a):
            def piece(m, k0, k1, hold):
                rows = pl.ds(pl.multiple_of(c * TS + t * HT + 16 * m, 16), 16)
                g = hold(g_v[rows, :])
                for k in range(k0, k1):
                    xb = x_v[rows, h * HD + 128 * k:h * HD + 128 * k + 128].astype(f32)
                    out_v[i, t, h, 16 * m:16 * m + 16, 128 * k:128 * k + 128] = (
                        g * a[16 * m:16 * m + 16, 128 * k:128 * k + 128] + (1.0 - g) * xb).astype(bf16)
                return [out_v[i, t, h, 16 * m:16 * m + 16, HD - 128:HD]]

            def send(n=1):
                pacer.flush(("mix", t, h), run=n == 1)
                for k0 in range(0, n_wb, n_wb // n):
                    for m in range(HT // 16 if n > 1 else 0):
                        piece(m, k0, k0 + n_wb // n, lambda v: v)
                    out_copy(i, t, h, 128 * k0, HD // n).start()

            pacer.add(("mix", t, h), 60,
                      [functools.partial(piece, m, 0, n_wb) for m in range(HT // 16)], True)
            return send

        s11, s22 = project(pacer, q_s, c, q_finish)
        m3 = o_product(2, o[1, 0])
        s11()
        m4 = o_product(3, o[0, 1])
        m1 = o_product(0, o[1, 0] + o[0, 1])
        s22()
        t = m1 + m4
        u = m1 + m3
        m2 = o_product(1, o[0, 0] + o[0, 1])
        send = mix(0, 0, m2 + m4)
        u = u - m2
        m6 = o_product(5, o[0, 0] - o[1, 0])
        send()
        send = mix(0, 1, u + m6)
        m5 = o_product(4, o[1, 0] + o[1, 1])
        send()
        send = mix(1, 1, m3 + m5)
        t = t - m5
        m7 = o_product(6, o[1, 1] - o[0, 1])
        send()

        pacer.flush("ffn")
        y = jnp.concatenate(y, axis=1)
        y_v[...] = y
        staged = jnp.concatenate(
            [out_v[0, idx % TS // HT, h, pl.ds(pl.multiple_of(idx16 % HT, 16), 16), :]
             for h in range(2)], axis=1).astype(f32)
        g = jnp.concatenate([g_v[pl.ds(idx16, 16), :]] * (D // 128), axis=1)
        is_sel = lax.broadcasted_iota(i32, (16, D), 0) == idx % 16
        y = jnp.sum(y, axis=0, keepdims=True) * r_gate
        row_v[...] = (staged + jnp.where(is_sel, (1.0 - g) * y, 0.0)).astype(bf16)
        mix(1, 0, t + m7)(n=2)
        return 0

    lax.fori_loop(0, n_chunks, phase2, 0)
    sent = lambda rows, n: pltpu.make_async_copy(out_v.at[rows], out_v.at[rows], sem_o.at[n])
    sent(slice(0, 1), 0).wait()
    row_copy = pltpu.make_async_copy(row_v, out_hbm.at[pl.ds(idx16, 16)], sem_o.at[0])
    row_copy.start()
    sent(slice(1, n_chunks), 1).wait()
    row_copy.wait()


@jax.jit
def pallas_gated_mix__linear_kernel_hedgehog__moe_arch_mod__prompt_kernel(
    A_x: jax.Array,
    A_wqkv: jax.Array,
    A_w_phi: jax.Array,
    A_wo: jax.Array,
    B_x: jax.Array,
    B_w_r: jax.Array,
    B_w_gate: jax.Array,
    B_w_up: jax.Array,
    B_w_down: jax.Array,
    gate_w: jax.Array,
):
    del B_x
    B, S, D = A_x.shape
    H, Dh, _ = A_w_phi.shape
    F = B_w_gate.shape[1]
    n_chunks = S // TS
    FS = F // n_chunks
    HD, HT = D // 2, TS // 2
    assert B == 1 and Dh == 32 and D == 1024 and H * Dh == D and S == 4 * TS and FS % 128 == 0

    hbm = pl.BlockSpec(memory_space=pl.ANY)
    out = pl.pallas_call(
        _kernel,
        out_shape=jax.ShapeDtypeStruct((S, D), A_x.dtype),
        in_specs=[hbm] * 9,
        out_specs=hbm,
        scratch_shapes=[
            pltpu.VMEM((S, D), bf16),
            pltpu.VMEM((3, D // 128, D, 128), bf16),
            pltpu.VMEM((H * Dh, Dh), bf16),
            pltpu.VMEM((8, 128), bf16),
            pltpu.VMEM((8, 128), bf16),
            pltpu.VMEM((D, D), bf16),
            pltpu.VMEM((n_chunks, D, FS), bf16),
            pltpu.VMEM((n_chunks, D, FS), bf16),
            pltpu.VMEM((n_chunks, FS, D), bf16),
            pltpu.VMEM((2, D // 128, 8, 128), f32),
            pltpu.VMEM((2, 2, HD, D), f32),
            pltpu.VMEM((D // 128, 128, 128), bf16),
            pltpu.VMEM((D // 128, TS, 128), bf16),
            pltpu.VMEM((D // 128, D, 128), bf16),
            pltpu.VMEM((7, HD // 128, D, 128), bf16),
            pltpu.VMEM((7, HD // 128, HD, 128), bf16),
            pltpu.VMEM((7, HD // 128, HD, 128), bf16),
            pltpu.VMEM((n_chunks, 7, HD // 128, HT, 128), bf16),
            pltpu.VMEM((H // 2, TS // 128, 128, 128), bf16),
            pltpu.VMEM((H // 2, 80, 128), f32),
            pltpu.VMEM((H // 2, 80, 128), bf16),
            pltpu.VMEM((n_chunks, 4, 8, 128), f32),
            pltpu.VMEM((n_chunks, 4, 8, 128), i32),
            pltpu.VMEM((S, 128), f32),
            pltpu.VMEM((n_chunks, 2, 2, HT, HD), bf16),
            pltpu.VMEM((16, D), bf16),
            pltpu.VMEM((D, 128), f32),
            pltpu.VMEM((FS, 128), f32),
            pltpu.VMEM((8, D), f32),
            pltpu.SemaphoreType.DMA((5,)),
            pltpu.SemaphoreType.DMA((3, D // 128)),
            pltpu.SemaphoreType.DMA((4 + 3 * n_chunks,)),
            pltpu.SemaphoreType.DMA((2,)),
        ],
        compiler_params=pltpu.CompilerParams(vmem_limit_bytes=110 * 1024 * 1024),
        name="gated_mix_hedgehog_mod",
    )(A_x.reshape(S, D), A_wqkv, A_w_phi.reshape(H * Dh, Dh), A_wo, B_w_r.reshape(8, 128),
      B_w_gate, B_w_up, B_w_down, gate_w.reshape(8, 128))
    return out.reshape(B, S, D)
```

```python
import functools

import jax
import jax.numpy as jnp
from jax import lax
import jax.experimental.pallas as pl
import jax.experimental.pallas.tpu as pltpu

TS = 512
LOG2E = 1.4426950408889634
FFN_ROWS = 16
RATE_FIRST, RATE_KEYS, RATE_QUERIES = 1.0, 0.95, 1.35

_NT = (((1,), (1,)), ((), ()))
_NN = (((1,), (0,)), ((), ()))

f32 = jnp.float32
bf16 = jnp.bfloat16
i32 = jnp.int32
u32 = jnp.uint32


def _dot(a, b, dims):
    a, b = (pltpu.bitcast(v, bf16) if v.dtype == u32 else v for v in (a, b))
    return lax.dot_general(a, b, dims, preferred_element_type=f32)


def _tree(op, xs):
    xs = list(xs)
    while len(xs) > 1:
        nxt = [op(xs[i], xs[i + 1]) for i in range(0, len(xs) - 1, 2)]
        if len(xs) % 2:
            nxt.append(xs[-1])
        xs = nxt
    return xs[0]


def _recip(x):
    return pl.reciprocal(x, full_range=False)


def _sigmoid(x):
    return 0.5 + 0.5 * jnp.tanh(0.5 * x)


def _head_reduce(op, tiles):
    r = _tree(op, tiles)
    r = op(r, pltpu.roll(r, 4, 0))
    return op(r, pltpu.roll(r, 2, 0))


def _phi(p, hold):
    tiles = [p[8 * j:8 * j + 8] for j in range(8)]
    out = []
    for op, diff in ((jnp.maximum, lambda t, m: t - m), (jnp.minimum, lambda t, m: m - t)):
        m = hold(_head_reduce(op, tiles))
        e = [jnp.exp2(diff(t, m)) for t in tiles]
        r = _recip(_head_reduce(jnp.add, e))
        out += [jnp.concatenate([e[j] * r, e[j + 1] * r], axis=0) for j in range(0, 8, 2)]
    return out


def _lane_bcast_rows(row):
    return jnp.broadcast_to(row, (128, row.shape[1])).T


def _lhs_terms(a11, a12, a21, a22):
    return (a11 + a22, a21 + a22, a11, a22, a11 + a12, a21 - a11, a12 - a22)


def _rhs_terms(b11, b12, b21, b22):
    return (b11 + b22, b11, b12 - b22, b21 - b11, b22, b11 + b12, b21 + b22)


def _put_terms(dst, m, terms_fn, load):
    rows = pl.ds(pl.multiple_of(16 * m, 16), 16)
    for k in range(dst.shape[1]):
        terms = terms_fn(*[load(i, j, k) for i in range(2) for j in range(2)])
        for n in range(7):
            dst[n, k, rows, :] = terms[n].astype(bf16)
    return terms[6][8:]


def _get(ref):
    return jnp.concatenate([pltpu.bitcast(ref[k], u32) for k in range(ref.shape[0])], axis=1)


class _Pacer:
    def __init__(self, zero, rate):
        self.zero = zero
        self.rate = rate
        self.previous = None
        self.tick = 0
        self.queues = ([], [])

    def add(self, tag, cost, pieces, urgent=False):
        self.queues[0 if urgent else 1].extend(
            (tag, cost, max(self.tick + urgent, 1), p) for p in pieces)

    def flush(self, tag, run=True):
        for queue in self.queues:
            for item in [q for q in queue if q[0] == tag]:
                queue[:] = [q for q in queue if q is not item]
                if run:
                    item[3](lambda v: v)

    def _take(self, budget):
        taken = ([], [])
        for queue, out in zip(self.queues, taken):
            while queue and queue[0][2] <= self.tick and budget >= queue[0][1] / 2:
                budget -= queue[0][1]
                out.append(queue.pop(0)[3])
        return taken

    def hold(self, where):
        rows = self.previous.shape[0] // 8
        start = pltpu.bitcast(self.previous[int(where * rows) * 8:][:8], u32) & self.zero
        return lambda v: pltpu.bitcast(
            pltpu.bitcast(v, u32) | jnp.concatenate([start] * (v.shape[0] // 8), axis=0), f32)

    def dot(self, lhs, rhs, dims):
        n = rhs.shape[0] // 64 if dims == _NT else rhs.shape[1] // 128
        out = []
        for j in range(n):
            marks = {}
            urgent, chain = self._take(self.rate * lhs.shape[0] * lhs.shape[1] / 256)
            for pieces, shift in ((urgent, 0.0), (chain, 0.5)):
                for m, piece in enumerate(pieces):
                    where = (m + shift) / len(pieces)
                    done = piece(self.hold(where))
                    if done and (pieces is urgent or m == len(pieces) - 1):
                        marks.setdefault(int(where * lhs.shape[0] / 8) * 8, []).extend(done)
            parts, at = [], 0
            for row, done in sorted(marks.items()):
                bits = _tree(jnp.bitwise_or, [pltpu.bitcast(v, u32) for v in done]) & self.zero
                parts += [lhs[at:row]] if row > at else []
                parts.append(jnp.concatenate(
                    [lhs[row:row + 8, 0:128] | bits, lhs[row:row + 8, 128:]], axis=1))
                at = row + 8
            a = jnp.concatenate(parts + ([lhs[at:]] if at < lhs.shape[0] else []), axis=0)
            out.append(_dot(a, rhs[64 * j:64 * j + 64] if dims == _NT else
                            rhs[:, 128 * j:128 * j + 128], dims))
            self.previous = out[-1]
            self.tick += 1
        return jnp.concatenate(out, axis=1)


def _kernel(x_hbm, wqkv_hbm, wphi_hbm, wo_hbm, wr_hbm, wg_hbm, wu_hbm, wd_hbm, gw_hbm,
            out_hbm,
            x_v, wqkv_v, wphi_v, wr_v, gw_v, wo_v, wg_v, wu_v, wd_v, wrg_v, fold_v,
            phi_t, x0_v, wv_t, kv_s, q_s, wo_s, x_s, phi_s,
            kv_acc, kv_t, rmax_v, rarg_v, g_v, out_v, row_v, xcol_v, hcol_v, y_v,
            sem_x, sem_w, sem_s, sem_o):
    S, D = x_v.shape
    F = wd_hbm.shape[0]
    n_chunks = S // TS
    n_pairs = D // 64
    FS = hcol_v.shape[0]
    HD, HT = D // 2, TS // 2
    n_wb = HD // 128
    HP = n_pairs // 2

    def x_copy(h0, h1):
        rows = pl.ds(h0 * HT, (h1 - h0) * HT)
        return pltpu.make_async_copy(x_hbm.at[rows], x_v.at[rows], sem_x.at[h0])

    def w_copies(j, b):
        return [pltpu.make_async_copy(wqkv_hbm.at[:, pl.ds(j * D + g * 128, 128)],
                                      wqkv_v.at[j, g], sem_w.at[j, g]) for g in (b, b + n_wb)]

    whole = [pltpu.make_async_copy(src, dst, sem_s.at[n]) for n, (src, dst) in enumerate(
        [(wphi_hbm, wphi_v), (wr_hbm, wr_v), (gw_hbm, gw_v), (wo_hbm, wo_v)]
        + [pair for i in range(n_chunks) for pair in (
            (wg_hbm.at[:, pl.ds(i * FS, FS)], wg_v.at[i]),
            (wu_hbm.at[:, pl.ds(i * FS, FS)], wu_v.at[i]),
            (wd_hbm.at[pl.ds(i * FS, FS)], wd_v.at[i]))])]

    def start(copies):
        for cp in copies:
            cp.start()

    def wait(copies):
        for cp in copies:
            cp.wait()

    start(whole[0:1] + w_copies(1, 0) + [x_copy(0, 1)] + whole[1:3])

    c_i = lax.broadcasted_iota(i32, (128, 32), 0)
    f_i = lax.broadcasted_iota(i32, (128, 32), 1)
    sel = jnp.where(c_i % 64 // 2 == f_i, 1.0, 0.0).astype(bf16)
    r_i = lax.broadcasted_iota(i32, (128, 128), 0)
    l_i = lax.broadcasted_iota(i32, (128, 128), 1)
    same_head = (2 * (r_i // 64) + r_i % 2) == (l_i // 32)

    def fold(j, b):
        for i in range(2):
            g = b + i * n_wb
            fold_v[j, i, 128 * b:128 * b + 128, :] = _dot(
                _get(phi_t.at[g:g + 1]), _get(wqkv_v.at[j, g:g + 1]), _NT) * LOG2E

    def gated(hold, i, j, v):
        return hold(v.astype(f32)) if i == j else v.astype(f32)

    def prep_folded(src, dst, m, hold):
        rows = pl.ds(pl.multiple_of(16 * m, 16), 16)
        return [_put_terms(dst, m, _lhs_terms, lambda i, j, k: gated(
            hold, i, j, fold_v[src, i, rows, j * HD + 128 * k:j * HD + 128 * k + 128]))]

    def fold_k(b):
        fold(1, b)
        pacer.add("kv", 100, [functools.partial(prep_folded, 1, kv_s, 8 * b + m) for m in range(8)])

    def prep_x(c, terms, m, best, hold):
        first = [pl.multiple_of(c * TS + t * HT + 16 * m, 16) for t in range(2)]
        dots, done = {}, []
        for k in range(n_wb):
            quads = []
            for i in range(2):
                col = i * n_wb + k
                for t in range(2):
                    quads.append(gated(hold, i, t, x_v[pl.ds(first[t], 16), 128 * col:128 * col + 128]))
                    for p in range(2):
                        for n in range(2):
                            v = quads[-1][8 * p:8 * p + 8] * wrg_v[n, col]
                            dots[n, t, p] = v + dots[n, t, p] if (n, t, p) in dots else v
            for n, term in enumerate(_rhs_terms(*quads)):
                terms[m, n, k] = term
                if n not in (1, 4):
                    done.append(term[8:])
        for t in range(2):
            for p in range(2):
                g = jnp.broadcast_to(jnp.sum(dots[1, t, p], axis=1, keepdims=True), (8, 128))
                g = _sigmoid(g)
                g_v[pl.ds(pl.multiple_of(first[t] + 8 * p, 8), 8), :] = g
                r = jnp.broadcast_to(jnp.sum(dots[0, t, p], axis=1, keepdims=True), (8, 128))
                r = r.astype(bf16).astype(f32)
                tok = first[t] + 8 * p + lax.broadcasted_iota(i32, (8, 128), 0)
                if m:
                    better = r > best[t, p][0]
                    r = jnp.where(better, r, best[t, p][0])
                    tok = jnp.where(better, tok, best[t, p][1])
                best[t, p] = (r, tok)
                done += [g, tok]
                if m == HT // 16 - 1:
                    rmax_v[c, 2 * t + p], rarg_v[c, 2 * t + p] = r, tok
        return done

    def prep_wo(m, hold):
        return [_put_terms(wo_s, m, _rhs_terms, lambda i, j, k: gated(hold, i, j, wo_v[
            pl.ds(pl.multiple_of(i * HD + 16 * m, 16), 16), j * HD + 128 * k:j * HD + 128 * k + 128]))]

    def prep_v(b):
        for g in (b, b + n_wb):
            strip = wqkv_v[2, g].T
            for k in range(D // 128):
                wv_t[k, 128 * g:128 * g + 128, :] = strip[:, 128 * k:128 * k + 128]
        return [lambda hold, m=m: [_put_terms(kv_s, HD // 16 + m, _lhs_terms, lambda i, j, k: gated(
            hold, i, j, wv_t[j * n_wb + k, i * HD + 16 * m:i * HD + 16 * m + 16, :]))]
            for m in range(8 * b, 8 * b + 8)]

    def put_phi(p, j, logits, hold):
        tiles = _phi(logits, hold)
        for n, rows in enumerate(tiles):
            phi_s[p, j, 16 * n:16 * n + 16, :] = rows.astype(bf16)
        return [tiles[3][8:], tiles[7][8:]]

    def features(pacer, tag, pairs, j0, res):
        pacer.add(tag, 100, [lambda hold, q=q, p=p, j=j: put_phi(
            p, j0 + j, res[64 * q:64 * q + 64, 128 * j:128 * j + 128], hold)
            for q, p in enumerate(pairs) for j in range(res.shape[1] // 128)], urgent=True)

    def with_ones(vt):
        return jnp.concatenate([vt, jnp.ones((16, vt.shape[1]), f32)], axis=0).astype(bf16)

    wait(whole[0:1])
    start(w_copies(1, 1))
    bits = jnp.concatenate([pltpu.bitcast(wphi_v[0:16, :], u32)] * 4, axis=1)
    zero = (bits & 1) * ((bits + 1) & 1)
    pacer = _Pacer(zero, RATE_FIRST)
    for g in range(D // 128):
        spread = _dot(sel, wphi_v[128 * g:128 * g + 128, :], _NT)
        phi_t[g] = jnp.where(same_head, spread, 0.0).astype(bf16)
    rmax_v[...] = jnp.full(rmax_v.shape, -jnp.inf, f32)
    rarg_v[...] = jnp.zeros(rarg_v.shape, i32)

    def stage_x(t):
        for k in range(D // 128):
            x0_v[k, t * HT:(t + 1) * HT, :] = x_v[t * HT:(t + 1) * HT, 128 * k:128 * k + 128]

    def k_block(b, t0, t1):
        lhs = jnp.concatenate([fold_v[1, i, 128 * b:128 * b + 128, :] for i in range(2)], axis=0)
        lhs = pltpu.bitcast(lhs.astype(bf16), u32)
        pk = pacer.dot(lhs, _get(x0_v.at[:, t0 * HT:t1 * HT]), _NT)
        features(pacer, "k", [2 * b, 2 * b + 1, HP + 2 * b, HP + 2 * b + 1], 2 * t0, pk)

    def v_block(b):
        vt = pacer.dot(_get(wv_t.at[:, 256 * b:256 * b + 256]), _get(x0_v), _NT)
        pacer.flush("k")
        for q in range(4):
            kv_acc[4 * b + q] = _dot(with_ones(vt[64 * q:64 * q + 64]), _get(phi_s.at[4 * b + q]), _NT)

    def put_x(c, terms, hold):
        for (m, n, k), term in sorted(terms.items(), key=lambda item: item[0]):
            term = jnp.concatenate([hold(m)(term[:8]), term[8:]], axis=0)
            x_s[c, n, k, 16 * m:16 * m + 16, :] = term.astype(bf16)

    strips = lambda j, b0, b1: [cp for b in range(b0, b1) for cp in w_copies(j, b)]
    wait(strips(1, 0, 1))
    start([x_copy(1, 2)])
    fold_k(0)
    wait([x_copy(0, 1)])
    start(strips(1, 2, 4))
    stage_x(0)
    k_block(0, 0, 1)
    wait(strips(1, 1, 2))
    start(strips(2, 0, 4))
    fold_k(1)
    k_block(1, 0, 1)
    wait([x_copy(1, 2)])
    start(strips(0, 0, 4) + [x_copy(2, 4)])
    stage_x(1)
    k_block(0, 1, 2)
    k_block(1, 1, 2)
    wait(strips(1, 2, 4))
    start([x_copy(4, 8), whole[3]])
    fold_k(2)
    k_block(2, 0, 2)
    fold_k(3)
    wait(strips(2, 0, 4) + whole[1:3])
    start(whole[4:])
    for n, w in enumerate((wr_v, gw_v)):
        w = w[...].astype(f32)
        for col in range(D // 128):
            wrg_v[n, col] = jnp.broadcast_to(w[col:col + 1], (8, 128))
    pacer.add("kv", 90, prep_v(0) + prep_v(1))
    k_block(3, 0, 2)
    pacer.add("kv", 90, prep_v(2) + prep_v(3))
    v_block(0)
    v_block(2)
    pacer.flush("kv")
    wait(strips(0, 0, 4) + [x_copy(2, 4)])
    for b in range(n_wb):
        fold(0, b)
    best = {}

    def first_x(m, hold):
        terms = {}
        done = prep_x(1, terms, m, best, hold)
        put_x(1, terms, lambda m: lambda v: v)
        return done

    pacer.add("x", 270, [functools.partial(first_x, m) for m in range(HT // 16)])
    v_block(1)
    v_block(3)
    pacer.flush("x")
    wait([x_copy(4, 8), whole[3]])

    def project(pacer, lhs_s, c, finish):
        product = lambda n: pacer.dot(_get(lhs_s.at[n]), _get(x_s.at[c, n]), _NT)
        m3 = product(2)
        m5 = product(4)
        s12 = finish(0, 1, m3 + m5)
        m4 = product(3)
        t = m4 - m5
        m2 = product(1)
        s12()
        s21 = finish(1, 0, m2 + m4)
        u = m3 - m2
        m1 = product(0)
        t = t + m1
        u = u + m1
        m7 = product(6)
        s21()
        s11 = finish(0, 0, t + m7)
        m6 = product(5)
        return s11, finish(1, 1, u + m6)

    def phase1(c, _):
        pacer = _Pacer(zero, RATE_KEYS)
        nxt = jnp.where(c + 1 < n_chunks, c + 1, 0)
        best, terms = {}, {}
        pacer.add("x", 290, [functools.partial(prep_x, nxt, terms, m, best) for m in range(HT // 16)])
        share = pl.cdiv(HD // 16, n_chunks - 1)
        for prep in (prep_wo, functools.partial(prep_folded, 0, q_s)):
            pacer.add("w", 120, [functools.partial(
                prep, jnp.minimum((c - 1) * share + j, HD // 16 - 1)) for j in range(share)])
        kr = lax.broadcasted_iota(i32, (80, 128), 0)
        kl = lax.broadcasted_iota(i32, (80, 128), 1)
        keep = jnp.where(kr < 64, kr // 32, (kr - 64) // 8) == kl % 2

        def kv_finish(half, t, res):
            features(pacer, (half, t), range(half * HP, half * HP + HP), 2 * t, res)

            def update():
                pacer.flush((half, t))
                for q in range(HP):
                    p = half * HP + q
                    acc = kv_acc[p] + _dot(with_ones(res[HD + 64 * q:HD + 64 * q + 64]),
                                           _get(phi_s.at[p, 2 * t:2 * t + 2]), _NT)
                    kv_acc[p] = acc
                    if half == t:
                        kv_t[p] = jnp.where(keep, acc, 0.0).astype(bf16)
            return update

        s11, s22 = project(pacer, kv_s, c, kv_finish)
        pacer.flush("x")
        put_x(nxt, terms, functools.cache(lambda m: pacer.hold(m / (HT // 16))))

        r = rmax_v[...].reshape(n_chunks * 32, 128)
        tok = rarg_v[...].reshape(n_chunks * 32, 128)
        r_max = jnp.max(r, axis=0, keepdims=True)
        idx = jnp.min(jnp.where(r == r_max, tok, S - 1))
        rows = x_v[pl.ds(pl.multiple_of((idx // 16) * 16, 16), 16), :].astype(f32)
        is_sel = lax.broadcasted_iota(i32, (16, D), 0) == idx % 16
        xcol_v[...] = _lane_bcast_rows(jnp.sum(jnp.where(is_sel, rows, 0.0), axis=0, keepdims=True))
        s11()
        s22()
        pacer.flush("w")
        return idx, r_max

    idx, r_max = lax.fori_loop(1, n_chunks, phase1, (jnp.int32(0), jnp.zeros((1, 128), f32)))
    y_v[...] = jnp.zeros(y_v.shape, f32)
    routed = idx // TS
    idx16 = pl.multiple_of((idx // 16) * 16, 16)
    r_gate = _sigmoid(r_max[:, 0:1])
    wait(whole[4:])

    def chunk_of(i):
        c = routed + i
        return jnp.where(c >= n_chunks, c - n_chunks, c)

    def out_copy(i, t, h, c0, width):
        return pltpu.make_async_copy(
            out_v.at[i, t, h, :, pl.ds(c0, width)],
            out_hbm.at[pl.ds(chunk_of(i) * TS + t * HT, HT), pl.ds(h * HD + c0, width)],
            sem_o.at[jnp.minimum(i, 1)])

    def phase2(i, _):
        pacer = _Pacer(zero, RATE_QUERIES)
        c = chunk_of(i)
        step = FFN_ROWS // 8

        def mat_vec(acc, col_ref, blocks, k0, hold):
            for k in range(k0, k0 + step):
                col = hold(col_ref[8 * k:8 * k + 8, :])
                for a, block in enumerate(blocks):
                    n = block.shape[1] // 128
                    for j0 in range(0, n, 2):
                        j1 = min(j0 + 2, n)
                        w = block[8 * k:8 * k + 8, 128 * j0:128 * j1].astype(f32)
                        for j in range(j0, j1):
                            p = w[:, 128 * (j - j0):128 * (j - j0) + 128] * col
                            acc[a * n + j] = p if acc[a * n + j] is None else acc[a * n + j] + p
            return list(acc)

        def hidden(hold):
            gate, up = (jnp.sum(jnp.concatenate(v, axis=1), axis=0, keepdims=True)
                        for v in (gu[:FS // 128], gu[FS // 128:]))
            hcol_v[...] = _lane_bcast_rows(gate * _sigmoid(gate) * up)
            return [hcol_v[FS - 8:FS, :]]

        gu = [None] * (2 * FS // 128)
        y = [y_v[:, 128 * j:128 * j + 128] for j in range(D // 128)]
        pacer.add("ffn", step * 43, [functools.partial(mat_vec, gu, xcol_v, (wg_v.at[i], wu_v.at[i]), k)
                                    for k in range(0, D // 8, step)])
        pacer.add("ffn", 400, [hidden])
        pacer.add("ffn", step * 25, [functools.partial(mat_vec, y, hcol_v, (wd_v.at[i],), k)
                                    for k in range(0, FS // 8, step)])
        o = {}

        def q_finish(half, t, res):
            features(pacer, (half, t), range(half * HP, half * HP + HP), 2 * t, res)

            def attend():
                pacer.flush((half, t))
                o_t = []
                for p in range(half * HP, half * HP + HP):
                    nd = _dot(_get(kv_t.at[p:p + 1]), _get(phi_s.at[p, 2 * t:2 * t + 2]), _NN)
                    for h in range(2):
                        inv = _recip(nd[64 + 8 * h:72 + 8 * h] + 1e-6)
                        o_t += [nd[32 * h + 8 * j:32 * h + 8 * j + 8] * inv for j in range(4)]
                o[t, half] = jnp.concatenate(o_t, axis=0)
            return attend

        def o_product(n, o_t):
            return pacer.dot(pltpu.bitcast(o_t.astype(bf16).T, u32), _get(wo_s.at[n]), _NN)

        def mix(t, h, a):
            def piece(m, k0, k1, hold):
                rows = pl.ds(pl.multiple_of(c * TS + t * HT + 16 * m, 16), 16)
                g = hold(g_v[rows, :])
                for k in range(k0, k1):
                    xb = x_v[rows, h * HD + 128 * k:h * HD + 128 * k + 128].astype(f32)
                    out_v[i, t, h, 16 * m:16 * m + 16, 128 * k:128 * k + 128] = (
                        g * a[16 * m:16 * m + 16, 128 * k:128 * k + 128] + (1.0 - g) * xb).astype(bf16)
                return [out_v[i, t, h, 16 * m:16 * m + 16, HD - 128:HD]]

            def send(n=1):
                pacer.flush(("mix", t, h), run=n == 1)
                for k0 in range(0, n_wb, n_wb // n):
                    for m in range(HT // 16 if n > 1 else 0):
                        piece(m, k0, k0 + n_wb // n, lambda v: v)
                    out_copy(i, t, h, 128 * k0, HD // n).start()

            pacer.add(("mix", t, h), 60,
                      [functools.partial(piece, m, 0, n_wb) for m in range(HT // 16)], True)
            return send

        s11, s22 = project(pacer, q_s, c, q_finish)
        m3 = o_product(2, o[1, 0])
        s11()
        m4 = o_product(3, o[0, 1])
        m1 = o_product(0, o[1, 0] + o[0, 1])
        s22()
        t = m1 + m4
        u = m1 + m3
        m2 = o_product(1, o[0, 0] + o[0, 1])
        send = mix(0, 0, m2 + m4)
        u = u - m2
        m6 = o_product(5, o[0, 0] - o[1, 0])
        send()
        send = mix(0, 1, u + m6)
        m5 = o_product(4, o[1, 0] + o[1, 1])
        send()
        send = mix(1, 1, m3 + m5)
        t = t - m5
        m7 = o_product(6, o[1, 1] - o[0, 1])
        send()

        pacer.flush("ffn")
        y = jnp.concatenate(y, axis=1)
        y_v[...] = y
        staged = jnp.concatenate(
            [out_v[0, idx % TS // HT, h, pl.ds(pl.multiple_of(idx16 % HT, 16), 16), :]
             for h in range(2)], axis=1).astype(f32)
        g = jnp.concatenate([g_v[pl.ds(idx16, 16), :]] * (D // 128), axis=1)
        is_sel = lax.broadcasted_iota(i32, (16, D), 0) == idx % 16
        y = jnp.sum(y, axis=0, keepdims=True) * r_gate
        row_v[...] = (staged + jnp.where(is_sel, (1.0 - g) * y, 0.0)).astype(bf16)
        mix(1, 0, t + m7)(n=2)
        return 0

    lax.fori_loop(0, n_chunks, phase2, 0)

    sent = lambda rows, n: pltpu.make_async_copy(out_v.at[rows], out_v.at[rows], sem_o.at[n])
    sent(slice(0, 1), 0).wait()
    row_copy = pltpu.make_async_copy(row_v, out_hbm.at[pl.ds(idx16, 16)], sem_o.at[0])
    row_copy.start()
    sent(slice(1, n_chunks), 1).wait()
    row_copy.wait()


@jax.jit
def pallas_gated_mix__linear_kernel_hedgehog__moe_arch_mod__prompt_kernel(
    A_x: jax.Array,
    A_wqkv: jax.Array,
    A_w_phi: jax.Array,
    A_wo: jax.Array,
    B_x: jax.Array,
    B_w_r: jax.Array,
    B_w_gate: jax.Array,
    B_w_up: jax.Array,
    B_w_down: jax.Array,
    gate_w: jax.Array,
):
    del B_x
    B, S, D = A_x.shape
    H, Dh, _ = A_w_phi.shape
    F = B_w_gate.shape[1]
    n_chunks = S // TS
    FS = F // n_chunks
    HD, HT = D // 2, TS // 2
    assert B == 1 and Dh == 32 and D == 1024 and H * Dh == D and S == 4 * TS and FS % 128 == 0

    hbm = pl.BlockSpec(memory_space=pl.ANY)
    out = pl.pallas_call(
        _kernel,
        out_shape=jax.ShapeDtypeStruct((S, D), A_x.dtype),
        in_specs=[hbm] * 9,
        out_specs=hbm,
        scratch_shapes=[
            pltpu.VMEM((S, D), bf16),
            pltpu.VMEM((3, D // 128, D, 128), bf16),
            pltpu.VMEM((H * Dh, Dh), bf16),
            pltpu.VMEM((8, 128), bf16),
            pltpu.VMEM((8, 128), bf16),
            pltpu.VMEM((D, D), bf16),
            pltpu.VMEM((n_chunks, D, FS), bf16),
            pltpu.VMEM((n_chunks, D, FS), bf16),
            pltpu.VMEM((n_chunks, FS, D), bf16),
            pltpu.VMEM((2, D // 128, 8, 128), f32),
            pltpu.VMEM((2, 2, HD, D), f32),
            pltpu.VMEM((D // 128, 128, 128), bf16),
            pltpu.VMEM((D // 128, TS, 128), bf16),
            pltpu.VMEM((D // 128, D, 128), bf16),
            pltpu.VMEM((7, HD // 128, D, 128), bf16),
            pltpu.VMEM((7, HD // 128, HD, 128), bf16),
            pltpu.VMEM((7, HD // 128, HD, 128), bf16),
            pltpu.VMEM((n_chunks, 7, HD // 128, HT, 128), bf16),
            pltpu.VMEM((H // 2, TS // 128, 128, 128), bf16),
            pltpu.VMEM((H // 2, 80, 128), f32),
            pltpu.VMEM((H // 2, 80, 128), bf16),
            pltpu.VMEM((n_chunks, 4, 8, 128), f32),
            pltpu.VMEM((n_chunks, 4, 8, 128), i32),
            pltpu.VMEM((S, 128), f32),
            pltpu.VMEM((n_chunks, 2, 2, HT, HD), bf16),
            pltpu.VMEM((16, D), bf16),
            pltpu.VMEM((D, 128), f32),
            pltpu.VMEM((FS, 128), f32),
            pltpu.VMEM((8, D), f32),
            pltpu.SemaphoreType.DMA((5,)),
            pltpu.SemaphoreType.DMA((3, D // 128)),
            pltpu.SemaphoreType.DMA((4 + 3 * n_chunks,)),
            pltpu.SemaphoreType.DMA((2,)),
        ],
        compiler_params=pltpu.CompilerParams(vmem_limit_bytes=110 * 1024 * 1024),
        name="gated_mix_hedgehog_mod",
    )(A_x.reshape(S, D), A_wqkv, A_w_phi.reshape(H * Dh, Dh), A_wo, B_w_r.reshape(8, 128),
      B_w_gate, B_w_up, B_w_down, gate_w.reshape(8, 128))
    return out.reshape(B, S, D)
```
